```python
import jax
import jax.numpy as jnp

def _softmax(x, axis=-1):
    return jax.nn.softmax(x, axis=axis)
def _gelu(x):
    return jax.nn.gelu(x, approximate=True)
def _silu(x):
    return jax.nn.silu(x)
def _sigmoid(x):
    return jax.nn.sigmoid(x)
def _layernorm(x, axis=-1, eps=1e-5):
    m = jnp.mean(x, axis=axis, keepdims=True)
    v = jnp.var(x, axis=axis, keepdims=True)
    return (x - m) / jnp.sqrt(v + eps)
def _scatter_add(tgt, idx, src, axis=0):
    return tgt.at[idx].add(src)
def _segment_sum(src, seg, n):
    return jax.ops.segment_sum(src, seg, n)
class _Rng:
    def __init__(self, key):
        self._k = key
    def _next(self):
        self._k, sub = jax.random.split(self._k)
        return sub
    def normal(self, shape):
        return jax.random.normal(self._next(), shape, dtype=jnp.bfloat16)
    def randint(self, lo, hi, shape):
        return jax.random.randint(self._next(), shape, lo, hi, dtype=jnp.int32)
    def uniform(self, shape, lo=0.0, hi=1.0):
        return jax.random.uniform(self._next(), shape, jnp.bfloat16, lo, hi)
    def permutation(self, n):
        return jax.random.permutation(self._next(), n)


kernel_name = 'interleave_layers__compressed_kv_cla__moe_arch_mod__decode'

def setup_inputs():
    _rng = _Rng(jax.random.key(int.from_bytes(__import__("os").urandom(4), "little")))
    _w = (lambda a: (lambda t: t.astype(jnp.bfloat16) if jnp.issubdtype(t.dtype, jnp.floating) else t)(jnp.asarray(a)))
    def _A_setup():
        B, H, Sq, Sk, D, M = 1, 32, 1, 4096, 128, 640
        Dc = 4 * D
        return {
            "x": _w((lambda *s: _rng.normal(s) * 0.05)(B, Sq, M)),
            "c_kv": _w((lambda *s: _rng.normal(s) * 0.05)(B, Sk, Dc)),
            "w_q": _w((lambda *s: _rng.normal(s) * 0.05)(M, H, D) * (M ** -0.5)),
            "w_uk": _w((lambda *s: _rng.normal(s) * 0.05)(Dc, H, D) * (Dc ** -0.5)),
            "w_uv": _w((lambda *s: _rng.normal(s) * 0.05)(Dc, H, D) * (Dc ** -0.5)),
            "w_o": _w((lambda *s: _rng.normal(s) * 0.05)(H, D, M) * ((H * D) ** -0.5)),
        }
    _A_in = _A_setup()

    def _B_setup():
        B, S, D, F, C = 1, 1, 640, 1728, 1
        return {
            "x": _w((lambda *s: _rng.normal(s) * 0.05)(B, S, D)),
            "w_r": _w((lambda *s: _rng.normal(s) * 0.05)(D)),
            "w_gate": _w((lambda *s: _rng.normal(s) * 0.05)(D, F)),
            "w_up": _w((lambda *s: _rng.normal(s) * 0.05)(D, F)),
            "w_down": _w((lambda *s: _rng.normal(s) * 0.05)(F, D)),
        }
    _B_in = _B_setup()

    return {
        "A_x": _A_in["x"],
        "A_c_kv": _A_in["c_kv"],
        "A_w_q": _A_in["w_q"],
        "A_w_uk": _A_in["w_uk"],
        "A_w_uv": _A_in["w_uv"],
        "A_w_o": _A_in["w_o"],
        "B_x": _B_in["x"],
        "B_w_r": _B_in["w_r"],
        "B_w_gate": _B_in["w_gate"],
        "B_w_up": _B_in["w_up"],
        "B_w_down": _B_in["w_down"],
    }

def reference(A_x, A_c_kv, A_w_q, A_w_uk, A_w_uv, A_w_o, B_x, B_w_r, B_w_gate, B_w_up, B_w_down):
    def _A_ref(x, c_kv, w_q, w_uk, w_uv, w_o):
        B, Sq, M = x.shape[0], x.shape[1], x.shape[2]
        Sk = c_kv.shape[1]
        H, D = w_q.shape[1], w_q.shape[2]
        q = jnp.einsum("bqm,mhd->bhqd", x, w_q)
        k = jnp.einsum("bkc,chd->bhkd", c_kv, w_uk)
        v = jnp.einsum("bkc,chd->bhkd", c_kv, w_uv)
        scores = jnp.einsum("bhqd,bhkd->bhqk", q, k) * (D ** -0.5)
        off = Sk - Sq
        qi = jnp.arange(Sq)[:, None]
        kj = jnp.arange(Sk)[None, :]
        cmask = kj <= (qi + off)
        scores = jnp.where(cmask[None, None], scores, -1e9)
        p = _softmax(scores, axis=-1)
        ctx = jnp.einsum("bhqk,bhkd->bhqd", p, v)
        return jnp.einsum("bhqd,hdm->bqm", ctx, w_o)

    def _B_ref(x, w_r, w_gate, w_up, w_down):
        B, S, D = x.shape
        C = 1
        r = x @ w_r
        idx = jnp.argsort(-r, axis=-1)[:, :C]
        idx_e = jnp.repeat(idx.reshape(B, C, 1), D, axis=2)
        x_sel = jnp.take_along_axis(x, idx_e, axis=1)
        g = _silu(x_sel @ w_gate)
        u = x_sel @ w_up
        y = (g * u) @ w_down
        r_sel = _sigmoid(jnp.take_along_axis(r, idx, axis=1))
        y = y * r_sel.reshape(B, C, 1)
        b_off = (jnp.arange(B) * S).reshape(B, 1)
        flat_idx = (idx + b_off).reshape(B * C)
        zero = (x * 0.0).reshape(B * S, D)
        upd = _scatter_add(zero, flat_idx, y.reshape(B * C, D), axis=0)
        return x + upd.reshape(B, S, D)

    x = A_x
    x = x + _A_ref(_layernorm(x, axis=-1), A_c_kv, A_w_q, A_w_uk, A_w_uv, A_w_o)
    x = x + _B_ref(_layernorm(x, axis=-1), B_w_r, B_w_gate, B_w_up, B_w_down)
    x = x + _A_ref(_layernorm(x, axis=-1), A_c_kv, A_w_q, A_w_uk, A_w_uv, A_w_o)
    x = x + _B_ref(_layernorm(x, axis=-1), B_w_r, B_w_gate, B_w_up, B_w_down)
    return x
```

```python
import functools
import jax
import jax.numpy as jnp
from jax import lax
import jax.experimental.pallas as pl
import jax.experimental.pallas.tpu as pltpu

F32 = jnp.float32
BF16 = jnp.bfloat16
U32 = jnp.uint32
M = 640
H = 32
D = 128
DC = 512
SK = 4096
FF = 1728
EPS = 1e-5

NT = (((1,), (1,)), ((), ()))


def _iota(shape, dim):
    return lax.broadcasted_iota(jnp.int32, shape, dim)


def _ln(x):
    mean = jnp.sum(x, axis=1, keepdims=True) * (1.0 / M)
    xc = x - mean
    var = jnp.sum(xc * xc, axis=1, keepdims=True) * (1.0 / M)
    return xc * lax.rsqrt(var + EPS)


def _kernel(x_hbm, ckv_hbm, wq_hbm, wuk_hbm, wuv_hbm, wo_hbm, wr_hbm, wg_hbm, wu_hbm, wd_hbm,
            o_ref,
            x_s, wr_s, wq_s, wuk_s, ckv_s, wuv_s, wo_s, wg_s, wu_s, wd_s,
            v_s, s_s, sems):
    WD_CH = [(0, 768), (768, 640), (1408, 320)]
    cps = {}
    k = 0
    def mk(name, src, dst):
        nonlocal k
        cps[name] = pltpu.make_async_copy(src, dst, sems.at[k])
        k += 1
    mk("x", x_hbm, x_s)
    mk("wr", wr_hbm, wr_s)
    mk("wq", wq_hbm, wq_s)
    mk("wuk", wuk_hbm, wuk_s)
    mk("ckv", ckv_hbm.at[0], ckv_s)
    mk("wuv", wuv_hbm, wuv_s)
    mk("wo", wo_hbm, wo_s)
    mk("wg", wg_hbm, wg_s)
    mk("wu", wu_hbm, wu_s)
    for i, (a, n) in enumerate(WD_CH):
        mk(f"wd{i}", wd_hbm.at[pl.ds(a, n)], wd_s.at[pl.ds(a, n)])
    for c in cps.values():
        c.start()

    def wait(name, first):
        if first:
            cps[name].wait()

    lane = _iota((128, 128), 1)
    row = _iota((128, 128), 0)
    E4 = jnp.where(row % 4 == lane // 32, 1.0, 0.0).astype(BF16)
    A_mask = _iota((32, 128), 1) // 4 == _iota((32, 128), 0)
    ls = _iota((16, 128), 0)
    lj = _iota((16, 128), 1) % 32
    M32 = jnp.where(lj == 2 * ls, jnp.uint32(0x0000FFFF), jnp.where(lj == 2 * ls + 1, jnp.uint32(0xFFFF0000), jnp.uint32(0)))

    def dup_bf16(v):
        u = pltpu.bitcast(v.astype(BF16).astype(F32), U32)
        return u | (u >> 16)

    def masked_lhs_matmul(nrows, get_tile):
        acc = None
        G = 8
        for t0 in range(0, nrows, G):
            lhs = []
            rhs = []
            for t in range(t0, t0 + G):
                vrow = jnp.broadcast_to(v_s[pl.ds(t, 1), :], (16, 128))
                lhs.append(pltpu.bitcast(vrow & M32, BF16))
                rhs.append(get_tile(t))
            o = jnp.dot(jnp.concatenate(lhs, axis=1), jnp.concatenate(rhs, axis=0), preferred_element_type=F32)
            acc = o if acc is None else acc + o
        return acc

    def attn(x, first):
        xn = _ln(x)
        xb = xn.astype(BF16)
        for kt in range(5):
            xr = jnp.broadcast_to(xn[0:1, 128 * kt:128 * (kt + 1)], (32, 128))
            A = jnp.where(A_mask, xr, 0.0).astype(BF16)
            V = jnp.dot(A, E4, preferred_element_type=F32)
            v_s[pl.ds(32 * kt, 32), :] = dup_bf16(V)
        wait("wq", first)
        q = masked_lhs_matmul(160, lambda t: wq_s[pl.ds(4 * t, 4)].reshape(128, 128))
        qb = q.astype(BF16)
        wait("wuk", first)
        hsel = (_iota((8, 128), 1) % 32) // 8
        rsel = _iota((8, 128), 1) % 8
        srow = _iota((8, 128), 0)
        vblocks = []
        for b0 in range(0, 128, 8):
            rhs = []
            for b in range(b0, b0 + 8):
                for cl in range(4):
                    rhs.append(wuk_s[128 * cl + b])
            o = lax.dot_general(qb, jnp.concatenate(rhs, axis=0), NT, preferred_element_type=F32)
            vb = None
            for i in range(8):
                ob = o[:, 128 * i:128 * (i + 1)]
                u = jnp.where(hsel == 0, ob[0:8], jnp.where(hsel == 1, ob[8:16], jnp.where(hsel == 2, ob[16:24], ob[24:32])))
                u = jnp.where(srow == rsel, u, 0.0)
                r_ = jnp.sum(u, axis=0, keepdims=True)
                r_ = jnp.broadcast_to(r_, (8, 128))
                vb = r_ if vb is None else jnp.where(srow == i, r_, vb)
            vblocks.append(vb)
        Vq = jnp.concatenate(vblocks, axis=0)
        Qt = Vq.T
        scale = D ** -0.5
        qa = jnp.concatenate([Qt[32 * cl:32 * (cl + 1)] for cl in range(4)], axis=1)
        qab = qa.astype(BF16)
        wait("ckv", first)
        KC = 512
        mx = None
        for kc in range(SK // KC):
            s = lax.dot_general(qab, ckv_s[pl.ds(kc * KC, KC), :], NT, preferred_element_type=F32) * scale
            s_s[:, pl.ds(kc * KC, KC)] = s
            for j in range(KC // 128):
                sj = s[:, 128 * j:128 * (j + 1)]
                mx = sj if mx is None else jnp.maximum(mx, sj)
        mx = jnp.max(mx, axis=1, keepdims=True)
        l = None
        o = None
        for kc in range(SK // KC):
            p = jnp.exp(s_s[:, pl.ds(kc * KC, KC)] - mx)
            for j in range(KC // 128):
                pj = p[:, 128 * j:128 * (j + 1)]
                l = pj if l is None else l + pj
            oc = jnp.dot(p.astype(BF16), ckv_s[pl.ds(kc * KC, KC), :], preferred_element_type=F32)
            o = oc if o is None else o + oc
        l = jnp.sum(l, axis=1, keepdims=True)
        o = o * (1.0 / l)
        Obig = jnp.concatenate([o[:, 128 * cl:128 * (cl + 1)] for cl in range(4)], axis=0)
        v_s[pl.ds(0, 128), :] = dup_bf16(Obig.T)
        wait("wuv", first)
        ctx = masked_lhs_matmul(128, lambda b: jnp.concatenate([wuv_s[128 * cl + b] for cl in range(4)], axis=0))
        ctxb = ctx.astype(BF16)
        wait("wo", first)
        r16 = _iota((16, 128), 0)
        acc = None
        for g in range(2):
            cg = ctxb[16 * g:16 * (g + 1)]
            for h0 in range(0, 16, 4):
                lhs = [jnp.where(r16 == h, cg, jnp.zeros_like(cg)) for h in range(h0, h0 + 4)]
                rhs = wo_s[pl.ds(16 * g + h0, 4)].reshape(512, M)
                oo = jnp.dot(jnp.concatenate(lhs, axis=1), rhs, preferred_element_type=F32)
                acc = oo if acc is None else acc + oo
        out = jnp.sum(acc, axis=0, keepdims=True)
        return x + out

    def ffn(x, first):
        xn = _ln(x)
        wr = wr_s[...].astype(F32).reshape(1, M)
        r = jnp.sum(xn * wr, axis=1, keepdims=True)
        rs = jax.nn.sigmoid(r)
        xb = jnp.broadcast_to(xn[0:1], (16, M)).astype(BF16)
        wait("wg", first)
        g = lax.dot_general(xb, wg_s[...], NT, preferred_element_type=F32)[0:8]
        wait("wu", first)
        u = lax.dot_general(xb, wu_s[...], NT, preferred_element_type=F32)[0:8]
        hh = (g * jax.nn.sigmoid(g) * u)
        hb = jnp.broadcast_to(hh[0:1], (16, FF)).astype(BF16)
        y = None
        for i, (a, n) in enumerate(WD_CH):
            wait(f"wd{i}", first)
            yc = jnp.dot(hb[:, a:a + n], wd_s[pl.ds(a, n), :], preferred_element_type=F32)[0:8]
            y = yc if y is None else y + yc
        upd = xn * 0.0 + y * rs
        return x + (xn + upd)

    cps["x"].wait()
    cps["wr"].wait()
    x = jnp.broadcast_to(x_s[0].astype(F32), (8, M))
    x = attn(x, True)
    x = ffn(x, True)
    x = attn(x, False)
    x = ffn(x, False)
    o_ref[0] = x[0:1].astype(BF16)


@jax.jit
def pallas_interleave_layers__compressed_kv_cla__moe_arch_mod__decode_kernel(A_x, A_c_kv, A_w_q, A_w_uk, A_w_uv, A_w_o, B_x, B_w_r, B_w_gate, B_w_up, B_w_down):
    anyspec = pl.BlockSpec(memory_space=pl.ANY)
    vm = pl.BlockSpec(memory_space=pltpu.VMEM)
    return pl.pallas_call(
        _kernel,
        out_shape=jax.ShapeDtypeStruct((1, 1, M), BF16),
        in_specs=[anyspec] * 10,
        out_specs=vm,
        scratch_shapes=[
            pltpu.VMEM((1, 1, M), BF16), pltpu.VMEM((M,), BF16),
            pltpu.VMEM((M, H, D), BF16), pltpu.VMEM((DC, H, D), BF16), pltpu.VMEM((SK, DC), BF16),
            pltpu.VMEM((DC, H, D), BF16), pltpu.VMEM((H, D, M), BF16),
            pltpu.VMEM((FF, M), BF16), pltpu.VMEM((FF, M), BF16), pltpu.VMEM((FF, M), BF16),
            pltpu.VMEM((160, 128), U32), pltpu.VMEM((H, SK), F32),
            pltpu.SemaphoreType.DMA((16,)),
        ],
        compiler_params=pltpu.CompilerParams(vmem_limit_bytes=100 * 1024 * 1024),
        name="fused_v1",
    )(A_x, A_c_kv, A_w_q, A_w_uk, A_w_uv, A_w_o, B_w_r, B_w_gate.T, B_w_up.T, B_w_down)
```

```python
import functools
import math
import jax
import jax.numpy as jnp
from jax import lax
import jax.experimental.pallas as pl
import jax.experimental.pallas.tpu as pltpu

F32 = jnp.float32
BF16 = jnp.bfloat16
U32 = jnp.uint32
M = 640
H = 32
D = 128
DC = 512
SK = 4096
FF = 1728
EPS = 1e-5
LOG2E = math.log2(math.e)

NT = (((1,), (1,)), ((), ()))


def _iota(shape, dim):
    return lax.broadcasted_iota(jnp.int32, shape, dim)


def _dot(a, b):
    return jnp.dot(a, b, preferred_element_type=F32)


def _lo(u):
    return pltpu.bitcast(u << 16, F32)


def _hi(u):
    return pltpu.bitcast(u & jnp.uint32(0xFFFF0000), F32)


def _pack16(v):
    return jnp.concatenate([v, v], axis=0).astype(BF16)


def _as_bf16(u):
    return pltpu.bitcast(u, BF16)


def _xsum(v):
    return jnp.sum(v, axis=1, keepdims=True)


def _interleave(*streams):
    items = []
    for si, s in enumerate(streams):
        n = len(s)
        for i, th in enumerate(s):
            items.append(((i + 0.5) / n, si, th))
    items.sort(key=lambda t: (t[0], t[1]))
    for _, _, th in items:
        th()


def _interleave(*streams):
    items = []
    for si, s in enumerate(streams):
        n = len(s)
        for i, th in enumerate(s):
            items.append(((i + 0.5) / n, si, th))
    items.sort(key=lambda t: (t[0], t[1]))
    for _, _, th in items:
        th()

def ln_parts(x):
    mean = _xsum(x) * (1.0 / M)
    xc = x - mean
    var = _xsum(xc * xc) * (1.0 / M)
    return xc, lax.rsqrt(var + EPS)

def two_step(NV, nmult, first, second, opt, fin):
    st = {}
    dstep = opt.get("dstep", 8); doff = opt.get("doff", 29)
    zneed = set(s - doff for s in range(0, NV * 16, dstep))
    def fA(i, db):
        def f():
            s = i * 16 + db
            if db % dstep == 0:
                base = first["mult"](i)
                key = ("z", s - doff)
                if key in st:
                    z = st.pop(key)
                    st[("m", i)] = [v + z for v in base]
                else:
                    st[("m", i)] = base
            xx = st[("m", i)]
            a = None
            for k in range(len(xx)):
                p = first["w"](i, k, db) * xx[k]
                a = p if a is None else a + p
            st[("b", s)] = _xsum(a)
        return f
    def fB(i, db):
        def f():
            s = i * 16 + db
            b = st.pop(("b", s))
            n = second["n"]
            for k in range(n):
                p = second["w"](i, k, db) * b
                key = second["acc"](i, k)
                st[key] = p if key not in st else st[key] + p
            if s in zneed:
                st[("z", s)] = st[second["acc"](i, n - 1)] * 0.0
            if db == 15:
                fin(i, st)
        return f
    vs = []
    for i in range(NV + 1):
        for db in range(16):
            if i < NV: vs.append(fA(i, db))
            if i >= 1: vs.append(fB(i - 1, db))
    return vs, st

def stage_BC(xc, W, qa_s, NV, opt):
    NM = H - NV
    WQm, WKm, WQv, WKv = W["WQm"], W["WKm"], W["WQv"], W["WKv"]
    xv = [xc[:, 128 * mt:128 * (mt + 1)] for mt in range(5)]
    XL = [_pack16(v) for v in xv]
    st = {}
    ms = []
    def mB(j, mt):
        def f():
            o = _dot(XL[mt], _as_bf16(WQm[j, mt]))[0:8]
            st[("q", j)] = o if mt == 0 else st[("q", j)] + o
            if mt == 4:
                st[("qL", j)] = _pack16(st.pop(("q", j)))
        return f
    def mC(j, ct):
        def f():
            o = _dot(st[("qL", j)], _as_bf16(WKm[j, ct]))
            qa_s[pl.ds(NV + j, 1), pl.ds(128 * ct, 128)] = o[0:1]
        return f
    lag = opt.get("lag", 2)
    for j in range(NM + lag):
        if j < NM: ms += [mB(j, mt) for mt in range(5)]
        if j >= lag: ms += [mC(j - lag, ct) for ct in range(4)]
    if NV == 0:
        _interleave(ms); return
    def fin(i, s):
        for ct in range(4):
            qa_s[pl.ds(i, 1), pl.ds(128 * ct, 128)] = jnp.sum(s.pop(("c", i, ct)), axis=0, keepdims=True)
    vs, _ = two_step(NV, 5,
        dict(mult=lambda i: xv, w=lambda i, k, db: WQv[i, k, pl.ds(8 * db, 8), :]),
        dict(n=4, w=lambda i, k, db: WKv[i, k, pl.ds(8 * db, 8), :], acc=lambda i, k: ("c", i, k)), opt, fin)
    _interleave(ms, vs)

def stage_DF(qa_s, scale, W, s_s, opt):
    ckvT, ckvN = W["ckvT"], W["ckvN"]
    QL = (qa_s[...] * scale).astype(BF16)
    NH = opt.get("nh", 16)
    mx = [None, None]
    for kt in range(32):
        sc = _dot(QL, _as_bf16(ckvT[kt]))
        s_s[:, pl.ds(128 * kt, 128)] = sc
        hf = int(kt >= NH)
        mx[hf] = sc if mx[hf] is None else jnp.maximum(mx[hf], sc)
    m0 = jnp.max(mx[0], axis=1, keepdims=True)
    m1 = jnp.maximum(m0, jnp.max(mx[1], axis=1, keepdims=True))
    alpha = jnp.exp2(m0 - m1)
    l = None; O = None
    for kt in range(32):
        mm = m0 if kt < NH else m1
        p = jnp.exp2(s_s[:, pl.ds(128 * kt, 128)] - mm)
        if kt == NH:
            l = l * alpha
            O = [o * alpha for o in O]
        l = p if l is None else l + p
        oc = _dot(p.astype(BF16), jnp.concatenate([_as_bf16(ckvN[kt, ct]) for ct in range(4)], axis=1))
        O = [oc[:, 128 * ct:128 * (ct + 1)] if kt == 0 else O[ct] + oc[:, 128 * ct:128 * (ct + 1)] for ct in range(4)]
    ls = _xsum(l)
    r0 = pl.reciprocal(ls, approx=True)
    inv = r0 * (2.0 - ls * r0)
    return [o * inv for o in O]

def stage_GH(O, W, NV, opt):
    NM = H - NV
    WVm, WOm, WVv, WOv = W["WVm"], W["WOm"], W["WVv"], W["WOv"]
    st = {}
    ms = []
    def mG(j, ct):
        def f():
            h = NV + j
            OL = jnp.broadcast_to(O[ct][h:h + 1], (16, 128)).astype(BF16)
            o = _dot(OL, _as_bf16(WVm[j, ct]))[0:8]
            st[("x", j)] = o if ct == 0 else st[("x", j)] + o
            if ct == 3:
                st[("cL", j)] = _pack16(st.pop(("x", j)))
        return f
    def mH(j, mt):
        def f():
            o = _dot(st[("cL", j)], _as_bf16(WOm[j, mt]))[0:8]
            st[("hm", mt)] = o if j == 0 else st[("hm", mt)] + o
        return f
    lag = opt.get("lag", 2)
    for j in range(NM + lag):
        if j < NM: ms += [mG(j, ct) for ct in range(4)]
        if j >= lag: ms += [mH(j - lag, mt) for mt in range(5)]
    vs, sv = two_step(NV, 4,
        dict(mult=lambda i: [jnp.broadcast_to(O[ct][i:i + 1], (8, 128)) for ct in range(4)],
             w=lambda i, k, db: WVv[i, k, pl.ds(8 * db, 8), :]),
        dict(n=5, w=lambda i, k, db: WOv[i, k, pl.ds(8 * db, 8), :], acc=lambda i, k: ("hv", k)), opt, lambda i, s: None)
    _interleave(ms, vs)
    return [st[("hm", mt)] + jnp.sum(sv[("hv", mt)], axis=0, keepdims=True) for mt in range(5)]

def stage_IJ(xc, rstd, W, FT, opt):
    FV = FF - 128 * FT
    WGm, WUm, WDm, WGv, WUv, WDv = (W[k] for k in ("WGm", "WUm", "WDm", "WGv", "WUv", "WDv"))
    xv = [xc[:, 128 * mt:128 * (mt + 1)] for mt in range(5)]
    XL = [_pack16(v) for v in xv]
    hs = jnp.broadcast_to(0.5 * rstd, (8, 128))
    st = {}
    ms = []
    def mI(ft, which, mt):
        def f():
            Wm = WGm if which == 0 else WUm
            o = _dot(XL[mt], _as_bf16(Wm[ft, mt]))[0:8]
            st[("g", ft, which)] = o if mt == 0 else st[("g", ft, which)] + o
            if which == 1 and mt == 4:
                t = st.pop(("g", ft, 0)) * hs
                hh = (t * st.pop(("g", ft, 1))) * (1.0 + jnp.tanh(t))
                st[("hL", ft)] = _pack16(hh)
        return f
    def mJ(ft, mt):
        def f():
            o = _dot(st[("hL", ft)], _as_bf16(WDm[ft, mt]))[0:8]
            st[("ym", mt)] = o if ft == 0 else st[("ym", mt)] + o
        return f
    lag = opt.get("lag", 1)
    for ft in range(FT + lag):
        if ft < FT: ms += [mI(ft, w, mt) for w in range(2) for mt in range(5)]
        if ft >= lag: ms += [mJ(ft - lag, mt) for mt in range(5)]
    vs = []
    NB = FV // 8
    dstep = opt.get("dstep", 8); doff = opt.get("doff", 16)
    LAG = opt.get("vlag", 8)
    zneed = set(s - doff for s in range(0, NB, dstep))
    def vI(fb, which):
        def f():
            if which == 0 and fb % dstep == 0:
                key = ("z", fb - doff)
                if key in st:
                    z = st.pop(key)
                    st["xv"] = [v + z for v in xv]
                else:
                    st["xv"] = xv
            Wv = WGv if which == 0 else WUv
            a = None
            for mt in range(5):
                p = Wv[mt, pl.ds(8 * fb, 8), :] * st["xv"][mt]
                a = p if a is None else a + p
            st[("gb", fb, which)] = jnp.broadcast_to(_xsum(a), (8, 128))
        return f
    def vJ(fb):
        def f():
            t = st.pop(("gb", fb, 0)) * hs
            hh = (t * st.pop(("gb", fb, 1))) * (1.0 + jnp.tanh(t))
            for mt in range(5):
                p = WDv[mt, pl.ds(8 * fb, 8), :] * hh
                st[("yv", mt)] = p if fb == 0 else st[("yv", mt)] + p
            if fb in zneed:
                st[("z", fb)] = st[("yv", 4)] * 0.0
        return f
    for fb in range(NB + LAG):
        if fb < NB: vs += [vI(fb, 0), vI(fb, 1)]
        if fb >= LAG: vs.append(vJ(fb - LAG))
    _interleave(ms, vs)
    return [st[("ym", mt)] + jnp.sum(st[("yv", mt)], axis=0, keepdims=True) for mt in range(5)]


def make_kernel(NV1, NV2, FT, opt, flags=None, tag=''):
    FM = 128 * FT
    FV = FF - FM
    WD_CH = [(0, FV), (FV, FM - 256), (FF - 256, 256)]

    def _kernel(x_hbm, ckv_hbm, wq_hbm, wuk_hbm, wuv_hbm, wo_hbm, wr_hbm, wg_hbm, wu_hbm, wd_hbm,
                o_ref,
                x_s, wr_s, wq_s, wuk_s, ckv_s, wuv_s, wo_s, wg_s, wu_s, wd_s,
                v_s, s_s, qa_s,
                WQm, WKm, WVm, WOm, WQv, WKv, WVv, WOv, ckvT, ckvN, WGm, WUm, WDm, WGv, WUv, WDv,
                sems):
        cps = {}
        k = 0

        def mk(name, src, dst):
            nonlocal k
            cps[name] = pltpu.make_async_copy(src, dst, sems.at[k])
            k += 1
        mk("x", x_hbm, x_s)
        mk("wr", wr_hbm, wr_s)
        mk("wq", wq_hbm, wq_s)
        mk("wuk", wuk_hbm, wuk_s)
        mk("ckv", ckv_hbm.at[0], ckv_s)
        mk("wuv", wuv_hbm, wuv_s)
        mk("wo", wo_hbm, wo_s)
        mk("wg", wg_hbm, wg_s)
        mk("wu", wu_hbm, wu_s)
        for i, (a, n) in enumerate(WD_CH):
            mk(f"wd{i}", wd_hbm.at[pl.ds(a, n)], wd_s.at[pl.ds(a, n)])
        for c in cps.values():
            c.start()

        def wait(name):
            cps[name].wait()

        wq_u = wq_s.bitcast(U32)
        wuk_u = wuk_s.bitcast(U32)
        wuv_u = wuv_s.bitcast(U32)

        lane = _iota((128, 128), 1)
        row = _iota((128, 128), 0)
        E4 = jnp.where(row % 4 == lane // 32, 1.0, 0.0).astype(BF16)
        A_mask = _iota((32, 128), 1) // 4 == _iota((32, 128), 0)
        ls = _iota((16, 128), 0)
        lj = _iota((16, 128), 1) % 32
        M32 = jnp.where(lj == 2 * ls, jnp.uint32(0x0000FFFF), jnp.where(lj == 2 * ls + 1, jnp.uint32(0xFFFF0000), jnp.uint32(0)))

        def ln_parts(x):
            mean = _xsum(x) * (1.0 / M)
            xc = x - mean
            var = _xsum(xc * xc) * (1.0 / M)
            return xc, lax.rsqrt(var + EPS)

        def dup_bf16(v):
            u = pltpu.bitcast(v.astype(BF16).astype(F32), U32)
            return u | (u >> 16)

        def masked_lhs_matmul(nrows, get_tile):
            acc = None
            G = 8
            for t0 in range(0, nrows, G):
                lhs = []
                rhs = []
                for t in range(t0, t0 + G):
                    vrow = jnp.broadcast_to(v_s[pl.ds(t, 1), :], (16, 128))
                    lhs.append(pltpu.bitcast(vrow & M32, BF16))
                    rhs.append(get_tile(t))
                o = _dot(jnp.concatenate(lhs, axis=1), jnp.concatenate(rhs, axis=0))
                acc = o if acc is None else acc + o
            return acc

        def gather(wu, hp, x0, n):
            return jnp.concatenate([wu[pl.ds((x0 + 8 * r) * 16 + hp, 8, stride=16), :] for r in range(n // 8)], axis=0)

        def gather_b(blk, hp):
            return jnp.concatenate([blk[pl.ds(128 * r + hp, 8, stride=16), :] for r in range(16)], axis=0)

        def prep_heads(wu, nt, Wv, Wm, m_transposed, NV):
            def body(t, c):
                blk = wu.at[pl.ds(pl.multiple_of(t * 2048, 2048), 2048)]
                for hp in range(16):
                    g = gather_b(blk, hp)
                    tt = g.T if (2 * hp < NV or m_transposed) else None
                    for half, f in ((0, _lo), (1, _hi)):
                        h = 2 * hp + half
                        if h < NV:
                            Wv[h, t] = f(tt)
                        else:
                            Wm[h - NV, t] = pltpu.bitcast(f(tt if m_transposed else g).astype(BF16), U32)
                return c
            lax.fori_loop(0, nt, body, 0)

        def attn1(x):
            xc, rstd = ln_parts(x)
            xn = xc * rstd
            for kt in range(5):
                xr = jnp.broadcast_to(xn[0:1, 128 * kt:128 * (kt + 1)], (32, 128))
                A = jnp.where(A_mask, xr, 0.0).astype(BF16)
                V = _dot(A, E4)
                v_s[pl.ds(32 * kt, 32), :] = dup_bf16(V)
            wait("wq")
            q = masked_lhs_matmul(160, lambda t: wq_s[pl.ds(128 * t, 128), :])
            qb = q.astype(BF16)
            prep_heads(wq_u, 5, WQv, WQm, False, NV1)
            wait("wuk")
            hsel = (_iota((8, 128), 1) % 32) // 8
            rsel = _iota((8, 128), 1) % 8
            srow = _iota((8, 128), 0)
            vblocks = []
            for b0 in range(0, 128, 8):
                rhs = []
                for b in range(b0, b0 + 8):
                    for cl in range(4):
                        rhs.append(wuk_s[pl.ds(32 * (128 * cl + b), 32), :])
                o = lax.dot_general(qb, jnp.concatenate(rhs, axis=0), NT, preferred_element_type=F32)
                vb = None
                for i in range(8):
                    ob = o[:, 128 * i:128 * (i + 1)]
                    u = jnp.where(hsel == 0, ob[0:8], jnp.where(hsel == 1, ob[8:16], jnp.where(hsel == 2, ob[16:24], ob[24:32])))
                    u = jnp.where(srow == rsel, u, 0.0)
                    r_ = jnp.broadcast_to(jnp.sum(u, axis=0, keepdims=True), (8, 128))
                    vb = r_ if vb is None else jnp.where(srow == i, r_, vb)
                vblocks.append(vb)
            Qt = jnp.concatenate(vblocks, axis=0).T
            qa = jnp.concatenate([Qt[32 * cl:32 * (cl + 1)] for cl in range(4)], axis=1)
            qab = qa.astype(BF16)
            prep_heads(wuk_u, 4, WKv, WKm, True, NV1)
            scale = D ** -0.5
            wait("ckv")
            KC = 512
            mx = None
            for kc in range(SK // KC):
                s = lax.dot_general(qab, ckv_s[pl.ds(kc * KC, KC), :], NT, preferred_element_type=F32) * scale
                s_s[:, pl.ds(kc * KC, KC)] = s
                for j in range(KC // 128):
                    sj = s[:, 128 * j:128 * (j + 1)]
                    mx = sj if mx is None else jnp.maximum(mx, sj)
            mx = jnp.max(mx, axis=1, keepdims=True)
            l = None
            o = None
            for kc in range(SK // KC):
                p = jnp.exp(s_s[:, pl.ds(kc * KC, KC)] - mx)
                for j in range(KC // 128):
                    pj = p[:, 128 * j:128 * (j + 1)]
                    l = pj if l is None else l + pj
                oc = _dot(p.astype(BF16), ckv_s[pl.ds(kc * KC, KC), :])
                o = oc if o is None else o + oc
            l = _xsum(l)
            o = o * (1.0 / l)
            def ckv_body(i, c):
                for j in range(2):
                    kt = 2 * i + j
                    for ct in range(4):
                        t = ckv_s[pl.ds(pl.multiple_of(128 * kt, 128), 128), pl.ds(128 * ct, 128)]
                        ckvT[kt, pl.ds(64 * ct, 64), :] = pltpu.bitcast(t.T, U32)
                        ckvN[kt, ct] = pltpu.bitcast(t, U32)
                return c
            lax.fori_loop(0, 16, ckv_body, 0)
            Obig = jnp.concatenate([o[:, 128 * cl:128 * (cl + 1)] for cl in range(4)], axis=0)
            v_s[pl.ds(0, 128), :] = dup_bf16(Obig.T)
            wait("wuv")
            ctx = masked_lhs_matmul(128, lambda b: jnp.concatenate([wuv_s[pl.ds(32 * (128 * cl + b), 32), :] for cl in range(4)], axis=0))
            ctxb = ctx.astype(BF16)
            prep_heads(wuv_u, 4, WVv, WVm, False, NV2)
            wait("wo")
            r16 = _iota((16, 128), 0)
            acc = None
            for g in range(2):
                cg = ctxb[16 * g:16 * (g + 1)]
                for h0 in range(0, 16, 4):
                    lhs = [jnp.where(r16 == h, cg, jnp.zeros_like(cg)) for h in range(h0, h0 + 4)]
                    rhs = wo_s[pl.ds(128 * (16 * g + h0), 512), :]
                    oo = _dot(jnp.concatenate(lhs, axis=1), rhs)
                    acc = oo if acc is None else acc + oo
            out = jnp.sum(acc, axis=0, keepdims=True)
            xo = x + out

            def wo_v(h, c):
                for mt in range(5):
                    WOv[h, mt] = wo_s[pl.ds(pl.multiple_of(128 * h, 128), 128), pl.ds(128 * mt, 128)].astype(F32)
                return c
            lax.fori_loop(0, NV2, wo_v, 0)

            def wo_m(j, c):
                for mt in range(5):
                    WOm[j, mt] = pltpu.bitcast(wo_s[pl.ds(pl.multiple_of(128 * (j + NV2), 128), 128), pl.ds(128 * mt, 128)], U32)
                return c
            lax.fori_loop(0, H - NV2, wo_m, 0)
            return xo

        def prep_gu(w_s, Wm, Wv):
            def body(ft, c):
                for mt in range(5):
                    t = w_s[pl.ds(pl.multiple_of(FV + 128 * ft, 16), 128), pl.ds(128 * mt, 128)]
                    Wm[ft, mt] = pltpu.bitcast(t.T, U32)
                return c
            lax.fori_loop(0, FT, body, 0)
            prep_v(w_s, Wv)

        def prep_v(w_s, Wv):
            def body(i, c):
                f0 = pl.multiple_of(64 * i, 64)
                for mt in range(5):
                    Wv[mt, pl.ds(f0, 64), :] = w_s[pl.ds(f0, 64), pl.ds(128 * mt, 128)].astype(F32)
                return c
            lax.fori_loop(0, FV // 64, body, 0)

        def router(xn):
            wr = wr_s[...].astype(F32).reshape(1, M)
            return jax.nn.sigmoid(_xsum(xn * wr))

        def ffn1(x):
            xc, rstd = ln_parts(x)
            xn = xc * rstd
            rs = router(xn)
            xb = jnp.broadcast_to(xn[0:1], (16, M)).astype(BF16)
            wait("wg")
            g = [lax.dot_general(xb, wg_s[pl.ds(a, n), :], NT, preferred_element_type=F32)[0:8] for a, n in ((0, FV), (FV, FM))]
            prep_gu(wg_s, WGm, WGv)
            wait("wu")
            u = [lax.dot_general(xb, wu_s[pl.ds(a, n), :], NT, preferred_element_type=F32)[0:8] for a, n in ((0, FV), (FV, FM))]
            hb = []
            for gg, uu in zip(g, u):
                hh = gg * jax.nn.sigmoid(gg) * uu
                hb.append(jnp.broadcast_to(hh[0:1], (16, hh.shape[1])).astype(BF16))
            prep_gu(wu_s, WUm, WUv)
            y = None
            for i, (a, n) in enumerate(WD_CH):
                wait(f"wd{i}")
                if i == 0:
                    lhs = hb[0]
                else:
                    lhs = hb[1][:, a - FV:a - FV + n]
                yc = _dot(lhs, wd_s[pl.ds(a, n), :])[0:8]
                y = yc if y is None else y + yc
                if i == 0:
                    prep_v(wd_s, WDv)
            upd = xn * 0.0 + y * rs
            return x + (xn + upd)

        W = dict(WQm=WQm, WKm=WKm, WVm=WVm, WOm=WOm, WQv=WQv, WKv=WKv, WVv=WVv, WOv=WOv, ckvT=ckvT, ckvN=ckvN,
                 WGm=WGm, WUm=WUm, WDm=WDm, WGv=WGv, WUv=WUv, WDv=WDv)

        def attn2(x):
            xc, rstd = ln_parts(x)
            stage_BC(xc, W, qa_s, NV1, opt["BC"])
            for ft in range(FT):
                for mt in range(5):
                    WDm[ft, mt] = pltpu.bitcast(wd_s[pl.ds(FV + 128 * ft, 128), pl.ds(128 * mt, 128)], U32)
            O = stage_DF(qa_s, rstd[0:1] * (D ** -0.5 * LOG2E), W, s_s, opt["DF"])
            out = stage_GH(O, W, NV2, opt["GH"])
            return x + jnp.concatenate(out, axis=1)

        def ffn2(x):
            xc, rstd = ln_parts(x)
            xn = xc * rstd
            rs = router(xn)
            out = stage_IJ(xc, rstd, W, FT, opt["IJ"])
            upd = xn * 0.0 + jnp.concatenate(out, axis=1) * (rs * rstd)
            return x + (xn + upd)

        wait("x")
        wait("wr")
        x = jnp.broadcast_to(x_s[0].astype(F32), (8, M))
        x = attn1(x)
        x = ffn1(x)
        x = attn2(x)
        x = ffn2(x)
        o_ref[0] = x[0:1].astype(BF16)

    def run(A_x, A_c_kv, A_w_q, A_w_uk, A_w_uv, A_w_o, B_x, B_w_r, B_w_gate, B_w_up, B_w_down):
        anyspec = pl.BlockSpec(memory_space=pl.ANY)
        vm = pl.BlockSpec(memory_space=pltpu.VMEM)
        return pl.pallas_call(
            _kernel,
            out_shape=jax.ShapeDtypeStruct((1, 1, M), BF16),
            in_specs=[anyspec] * 10,
            out_specs=vm,
            scratch_shapes=[
                pltpu.VMEM((1, 1, M), BF16), pltpu.VMEM((M,), BF16),
                pltpu.VMEM((M * H, D), BF16), pltpu.VMEM((DC * H, D), BF16), pltpu.VMEM((SK, DC), BF16),
                pltpu.VMEM((DC * H, D), BF16), pltpu.VMEM((H * D, M), BF16),
                pltpu.VMEM((FF, M), BF16), pltpu.VMEM((FF, M), BF16), pltpu.VMEM((FF, M), BF16),
                pltpu.VMEM((160, 128), U32), pltpu.VMEM((H, SK), F32), pltpu.VMEM((H, DC), F32),
                pltpu.VMEM((H - NV1, 5, 64, 128), U32), pltpu.VMEM((H - NV1, 4, 64, 128), U32),
                pltpu.VMEM((H - NV2, 4, 64, 128), U32), pltpu.VMEM((H - NV2, 5, 64, 128), U32),
                pltpu.VMEM((NV1, 5, 128, 128), F32), pltpu.VMEM((NV1, 4, 128, 128), F32),
                pltpu.VMEM((NV2, 4, 128, 128), F32), pltpu.VMEM((NV2, 5, 128, 128), F32),
                pltpu.VMEM((32, 256, 128), U32), pltpu.VMEM((32, 4, 64, 128), U32),
                pltpu.VMEM((FT, 5, 64, 128), U32), pltpu.VMEM((FT, 5, 64, 128), U32), pltpu.VMEM((FT, 5, 64, 128), U32),
                pltpu.VMEM((5, FV, 128), F32), pltpu.VMEM((5, FV, 128), F32), pltpu.VMEM((5, FV, 128), F32),
                pltpu.SemaphoreType.DMA((16,)),
            ],
            compiler_params=pltpu.CompilerParams(vmem_limit_bytes=110 * 1024 * 1024, flags=flags),
            name=f"fused_v4_{NV1}_{NV2}_{FT}{tag}",
        )(A_x, A_c_kv, A_w_q.reshape(M * H, D), A_w_uk.reshape(DC * H, D), A_w_uv.reshape(DC * H, D),
          A_w_o.reshape(H * D, M), B_w_r, B_w_gate.T, B_w_up.T, B_w_down)
    return run


OPT = dict(BC=dict(lag=3, dstep=8, doff=29), DF=dict(nh=16), GH=dict(lag=3, dstep=16, doff=25), IJ=dict(lag=3, dstep=8, doff=20, vlag=12))
_run = make_kernel(15, 15, 7, OPT)


@jax.jit
def pallas_interleave_layers__compressed_kv_cla__moe_arch_mod__decode_kernel(
    A_x, A_c_kv, A_w_q, A_w_uk, A_w_uv, A_w_o, B_x, B_w_r, B_w_gate, B_w_up, B_w_down):
    return _run(A_x, A_c_kv, A_w_q, A_w_uk, A_w_uv, A_w_o, B_x, B_w_r, B_w_gate, B_w_up, B_w_down)
```

```python
import functools
import math
import jax
import jax.numpy as jnp
from jax import lax
import jax.experimental.pallas as pl
import jax.experimental.pallas.tpu as pltpu

F32 = jnp.float32
BF16 = jnp.bfloat16
U32 = jnp.uint32
M = 640
H = 32
D = 128
DC = 512
SK = 4096
FF = 1728
EPS = 1e-5
LOG2E = math.log2(math.e)

NT = (((1,), (1,)), ((), ()))


def _iota(shape, dim):
    return lax.broadcasted_iota(jnp.int32, shape, dim)


def _dot(a, b):
    return jnp.dot(a, b, preferred_element_type=F32)


def _lo(u):
    return pltpu.bitcast(u << 16, F32)


def _hi(u):
    return pltpu.bitcast(u & jnp.uint32(0xFFFF0000), F32)


def _pack16(v):
    return jnp.concatenate([v, v], axis=0).astype(BF16)


def _as_bf16(u):
    return pltpu.bitcast(u, BF16)


def _xsum(v):
    return jnp.sum(v, axis=1, keepdims=True)


def _interleave(*streams):
    items = []
    for si, s in enumerate(streams):
        n = len(s)
        for i, th in enumerate(s):
            items.append(((i + 0.5) / n, si, th))
    items.sort(key=lambda t: (t[0], t[1]))
    for _, _, th in items:
        th()


PHI = 1.0
def _interleave(*streams):
    items = []
    for si, s in enumerate(streams):
        n = len(s)
        for i, th in enumerate(s):
            items.append(((i + 0.5) / n * (PHI if si == 1 else 1.0), si, th))
    items.sort(key=lambda t: (t[0], t[1]))
    for _, _, th in items:
        th()

def ln_parts(x):
    mean = _xsum(x) * (1.0 / M)
    xc = x - mean
    var = _xsum(xc * xc) * (1.0 / M)
    return xc, lax.rsqrt(var + EPS)

def two_step(NV, nmult, first, second, opt, fin):
    st = {}
    dstep = opt.get("dstep", 8); doff = opt.get("doff", 29)
    s0 = opt.get("s0", 0)
    zneed = set(s - doff for s in range(0, NV * 16, dstep) if s >= s0)
    def fA(i, db):
        def f():
            s = i * 16 + db
            if db % dstep == 0:
                if first.get("shared"):
                    base = st.get("m", first["mult"](i))
                else:
                    base = first["mult"](i) if db == 0 else st["m"]
                key = ("z", s - doff)
                if key in st:
                    z = st.pop(key)
                    st["m"] = [v + z for v in base]
                else:
                    st["m"] = base
            xx = st["m"]
            a = None
            for k in range(len(xx)):
                p = first["w"](i, k, db) * xx[k]
                a = p if a is None else a + p
            st[("b", s)] = _xsum(a)
        return f
    def fB(i, db):
        def f():
            s = i * 16 + db
            b = st.pop(("b", s))
            n = second["n"]
            for k in range(n):
                p = second["w"](i, k, db) * b
                key = second["acc"](i, k)
                st[key] = p if key not in st else st[key] + p
            if s in zneed:
                st[("z", s)] = st[second["acc"](i, n - 1)] * 0.0
            if db == 15:
                fin(i, st)
        return f
    vs = []
    for i in range(NV + 1):
        for db in range(16):
            if i < NV: vs.append(fA(i, db))
            if i >= 1: vs.append(fB(i - 1, db))
    return vs, st

def stage_BC(xc, W, qa_s, NV, opt):
    NM = H - NV
    WQm, WKm, WQv, WKv = W["WQm"], W["WKm"], W["WQv"], W["WKv"]
    xv = [xc[:, 128 * mt:128 * (mt + 1)] for mt in range(5)]
    XL = [_pack16(v) for v in xv]
    st = {}
    ms = []
    def mB(j, mt):
        def f():
            o = _dot(XL[mt], _as_bf16(WQm[j, mt]))[0:8]
            st[("q", j)] = o if mt == 0 else st[("q", j)] + o
            if mt == 4:
                st[("qL", j)] = _pack16(st.pop(("q", j)))
        return f
    def mC(j, ct):
        def f():
            o = _dot(st[("qL", j)], _as_bf16(WKm[j, ct]))
            qa_s[pl.ds(NV + j, 1), pl.ds(128 * ct, 128)] = o[0:1]
        return f
    lag = opt.get("lag", 2)
    if lag == "sweep":
        for j in range(NM): ms += [mB(j, mt) for mt in range(5)]
        for ct in range(4): ms += [mC(j, ct) for j in range(NM)]
    else:
        for j in range(NM + lag):
            if j < NM: ms += [mB(j, mt) for mt in range(5)]
            if j >= lag: ms += [mC(j - lag, ct) for ct in range(4)]
    if NV == 0:
        _interleave(ms); return
    def fin(i, s):
        for ct in range(4):
            qa_s[pl.ds(i, 1), pl.ds(128 * ct, 128)] = jnp.sum(s.pop(("c", i, ct)), axis=0, keepdims=True)
    vs, _ = two_step(NV, 5,
        dict(shared=1, mult=lambda i: xv, w=lambda i, k, db: WQv[i, k, pl.ds(8 * db, 8), :]),
        dict(n=4, w=lambda i, k, db: WKv[i, k, pl.ds(8 * db, 8), :], acc=lambda i, k: ("c", i, k)), opt, fin)
    if opt.get("nomxu"): ms = []
    if opt.get("novpu"): vs = []
    _interleave(*[s for s in (ms, vs) if s])

def stage_DF(qa_s, scale, W, s_s, opt):
    ckvT, ckvN = W["ckvT"], W["ckvN"]
    QL = [(qa_s[:, pl.ds(128 * ct, 128)] * scale).astype(BF16) for ct in range(4)]
    NH = opt.get("nh", 16)
    NA = opt.get("na", 0)
    def Dt(kt, ct):
        return _dot(QL[ct], _as_bf16(ckvT[kt, pl.ds(64 * ct, 64), :]))
    for kt in range(NA):
        s_s[:, pl.ds(128 * kt, 128)] = Dt(kt, 0)
    mx = [None, None]
    for kt in range(32):
        if kt < NA:
            sc = s_s[:, pl.ds(128 * kt, 128)]
            for ct in range(1, 4): sc = sc + Dt(kt, ct)
        else:
            sc = Dt(kt, 0)
            for ct in range(1, 4): sc = sc + Dt(kt, ct)
        s_s[:, pl.ds(128 * kt, 128)] = sc
        hf = int(kt >= NH)
        mx[hf] = sc if mx[hf] is None else jnp.maximum(mx[hf], sc)
    m0 = jnp.max(mx[0], axis=1, keepdims=True)
    m1 = jnp.maximum(m0, jnp.max(mx[1], axis=1, keepdims=True))
    alpha = jnp.exp2(m0 - m1)
    l = None; O = [None] * 4
    def Ft(pb, kt, ct):
        o = _dot(pb, _as_bf16(ckvN[kt, ct]))
        O[ct] = o if O[ct] is None else O[ct] + o
    for kt in range(NH):
        p = jnp.exp2(s_s[:, pl.ds(128 * kt, 128)] - m0)
        l = p if l is None else l + p
        pb = p.astype(BF16)
        for ct in range(4): Ft(pb, kt, ct)
    l = l * alpha
    if opt.get("sweep", 0):
        P = {}
        for ct in range(4):
            O[ct] = O[ct] * alpha
            for kt in range(NH, 32):
                if ct == 0:
                    p = jnp.exp2(s_s[:, pl.ds(128 * kt, 128)] - m1)
                    l = l + p
                    P[kt] = p.astype(BF16)
                Ft(P[kt], kt, ct)
    else:
        O = [o * alpha for o in O]
        for kt in range(NH, 32):
            p = jnp.exp2(s_s[:, pl.ds(128 * kt, 128)] - m1)
            l = l + p
            pb = p.astype(BF16)
            for ct in range(4): Ft(pb, kt, ct)
    ls = _xsum(l)
    r0 = pl.reciprocal(ls, approx=True)
    inv = r0 * (2.0 - ls * r0)
    return [o * inv for o in O]

def stage_GH(O, W, NV, opt):
    NM = H - NV
    WVm, WOm, WVv, WOv = W["WVm"], W["WOm"], W["WVv"], W["WOv"]
    st = {}
    ms = []
    def mG(j, ct):
        def f():
            h = NV + j
            OL = jnp.broadcast_to(O[ct][h:h + 1], (16, 128)).astype(BF16)
            o = _dot(OL, _as_bf16(WVm[j, ct]))[0:8]
            st[("x", j)] = o if ct == 0 else st[("x", j)] + o
            if ct == 3:
                st[("cL", j)] = _pack16(st.pop(("x", j)))
        return f
    def mH(j, mt):
        def f():
            o = _dot(st[("cL", j)], _as_bf16(WOm[j, mt]))[0:8]
            st[("hm", mt)] = o if j == 0 else st[("hm", mt)] + o
        return f
    lag = opt.get("lag", 2)
    if lag == "sweep":
        for ct in range(4): ms += [mG(j, ct) for j in range(NM)]
        for j in range(NM): ms += [mH(j, mt) for mt in range(5)]
    else:
        for j in range(NM + lag):
            if j < NM: ms += [mG(j, ct) for ct in range(4)]
            if j >= lag: ms += [mH(j - lag, mt) for mt in range(5)]
    vs, sv = two_step(NV, 4,
        dict(mult=lambda i: [jnp.broadcast_to(O[ct][i:i + 1], (8, 128)) for ct in range(4)],
             w=lambda i, k, db: WVv[i, k, pl.ds(8 * db, 8), :]),
        dict(n=5, w=lambda i, k, db: WOv[i, k, pl.ds(8 * db, 8), :], acc=lambda i, k: ("hv", k)), opt, lambda i, s: None)
    _interleave(ms, vs)
    return [st[("hm", mt)] + jnp.sum(sv[("hv", mt)], axis=0, keepdims=True) for mt in range(5)]

def stage_IJ(xc, rstd, W, FT, opt):
    FV = FF - 128 * FT
    _tanh = (lambda t: t * t) if opt.get("notanh") else jnp.tanh
    WGm, WUm, WDm, WGv, WUv, WDv = (W[k] for k in ("WGm", "WUm", "WDm", "WGv", "WUv", "WDv"))
    xv = [xc[:, 128 * mt:128 * (mt + 1)] for mt in range(5)]
    XL = [_pack16(v) for v in xv]
    hs = jnp.broadcast_to(0.5 * rstd, (8, 128))
    st = {}
    ms = []
    def mI(ft, which, mt):
        def f():
            Wm = WGm if which == 0 else WUm
            o = _dot(XL[mt], _as_bf16(Wm[ft, mt]))[0:8]
            st[("g", ft, which)] = o if mt == 0 else st[("g", ft, which)] + o
            if which == 1 and mt == 4:
                t = st.pop(("g", ft, 0)) * hs
                hh = (t * st.pop(("g", ft, 1))) * (1.0 + _tanh(t))
                st[("hL", ft)] = _pack16(hh)
        return f
    def mJ(ft, mt):
        def f():
            o = _dot(st[("hL", ft)], _as_bf16(WDm[ft, mt]))[0:8]
            st[("ym", mt)] = o if ft == 0 else st[("ym", mt)] + o
        return f
    lag = opt.get("lag", 1)
    for ft in range(FT + lag):
        if ft < FT: ms += [mI(ft, w, mt) for w in range(2) for mt in range(5)]
        if ft >= lag: ms += [mJ(ft - lag, mt) for mt in range(5)]
    vs = []
    NB = FV // 8
    dstep = opt.get("dstep", 8); doff = opt.get("doff", 16)
    LAG = opt.get("vlag", 8)
    zneed = set(s - doff for s in range(0, NB, dstep))
    def vI(fb, which):
        def f():
            if which == 0 and fb % dstep == 0:
                key = ("z", fb - doff)
                if key in st:
                    z = st.pop(key)
                    st["xv"] = [v + z for v in st.get("xv", xv)]
                else:
                    st["xv"] = st.get("xv", xv)
            Wv = WGv if which == 0 else WUv
            a = None
            for mt in range(5):
                p = Wv[mt, pl.ds(8 * fb, 8), :] * st["xv"][mt]
                a = p if a is None else a + p
            st[("gb", fb, which)] = jnp.broadcast_to(_xsum(a), (8, 128))
        return f
    def vJ(fb):
        def f():
            t = st.pop(("gb", fb, 0)) * hs
            hh = (t * st.pop(("gb", fb, 1))) * (1.0 + _tanh(t))
            for mt in range(5):
                p = WDv[mt, pl.ds(8 * fb, 8), :] * hh
                st[("yv", mt)] = p if fb == 0 else st[("yv", mt)] + p
            if fb in zneed:
                st[("z", fb)] = st[("yv", 4)] * 0.0
        return f
    for fb in range(NB + LAG):
        if fb < NB: vs += [vI(fb, 0), vI(fb, 1)]
        if fb >= LAG: vs.append(vJ(fb - LAG))
    if opt.get("nomxu"):
        _interleave(vs)
        return [jnp.broadcast_to(jnp.sum(st[("yv", mt)], axis=0, keepdims=True), (8, 128)) for mt in range(5)]
    if opt.get("novpu"):
        _interleave(ms)
        return [st[("ym", mt)] for mt in range(5)]
    _interleave(ms, vs)
    return [st[("ym", mt)] + jnp.sum(st[("yv", mt)], axis=0, keepdims=True) for mt in range(5)]


def make_kernel(NV1, NV2, FT, opt, flags=None, tag=''):
    FM = 128 * FT
    FV = FF - FM
    WD_CH = [(0, FV), (FV, FM - 256), (FF - 256, 256)]

    def _kernel(x_hbm, ckv_hbm, wq_hbm, wuk_hbm, wuv_hbm, wo_hbm, wr_hbm, wg_hbm, wu_hbm, wd_hbm,
                o_ref,
                x_s, wr_s, wq_s, wuk_s, ckv_s, wuv_s, wo_s, wg_s, wu_s, wd_s,
                v_s, s_s, qa_s,
                WQm, WKm, WVm, WOm, WQv, WKv, WVv, WOv, ckvT, ckvN, WGm, WUm, WDm, WGv, WUv, WDv,
                sems):
        cps = {}
        k = 0

        def mk(name, src, dst):
            nonlocal k
            cps[name] = pltpu.make_async_copy(src, dst, sems.at[k])
            k += 1
        mk("x", x_hbm, x_s)
        mk("wr", wr_hbm, wr_s)
        mk("wq", wq_hbm, wq_s)
        mk("wuk", wuk_hbm, wuk_s)
        mk("ckv", ckv_hbm.at[0], ckv_s)
        mk("wuv", wuv_hbm, wuv_s)
        mk("wo", wo_hbm, wo_s)
        mk("wg", wg_hbm, wg_s)
        mk("wu", wu_hbm, wu_s)
        for i, (a, n) in enumerate(WD_CH):
            mk(f"wd{i}", wd_hbm.at[pl.ds(a, n)], wd_s.at[pl.ds(a, n)])
        for c in cps.values():
            c.start()

        def wait(name):
            cps[name].wait()

        wq_u = wq_s.bitcast(U32)
        wuk_u = wuk_s.bitcast(U32)
        wuv_u = wuv_s.bitcast(U32)

        lane = _iota((128, 128), 1)
        row = _iota((128, 128), 0)
        E4 = jnp.where(row % 4 == lane // 32, 1.0, 0.0).astype(BF16)
        A_mask = _iota((32, 128), 1) // 4 == _iota((32, 128), 0)
        ls = _iota((16, 128), 0)
        lj = _iota((16, 128), 1) % 32
        M32 = jnp.where(lj == 2 * ls, jnp.uint32(0x0000FFFF), jnp.where(lj == 2 * ls + 1, jnp.uint32(0xFFFF0000), jnp.uint32(0)))

        def ln_parts(x):
            mean = _xsum(x) * (1.0 / M)
            xc = x - mean
            var = _xsum(xc * xc) * (1.0 / M)
            return xc, lax.rsqrt(var + EPS)

        def dup_bf16(v):
            u = pltpu.bitcast(v.astype(BF16).astype(F32), U32)
            return u | (u >> 16)

        def masked_lhs_matmul(nrows, get_tile):
            acc = None
            G = 8
            for t0 in range(0, nrows, G):
                lhs = []
                rhs = []
                for t in range(t0, t0 + G):
                    vrow = jnp.broadcast_to(v_s[pl.ds(t, 1), :], (16, 128))
                    lhs.append(pltpu.bitcast(vrow & M32, BF16))
                    rhs.append(get_tile(t))
                o = _dot(jnp.concatenate(lhs, axis=1), jnp.concatenate(rhs, axis=0))
                acc = o if acc is None else acc + o
            return acc

        def gather(wu, hp, x0, n):
            return jnp.concatenate([wu[pl.ds((x0 + 8 * r) * 16 + hp, 8, stride=16), :] for r in range(n // 8)], axis=0)

        def gather_b(blk, hp):
            return jnp.concatenate([blk[pl.ds(128 * r + hp, 8, stride=16), :] for r in range(16)], axis=0)

        def prep_heads(wu, nt, Wv, Wm, m_transposed, NV):
            def body(t, c):
                blk = wu.at[pl.ds(pl.multiple_of(t * 2048, 2048), 2048)]
                for hp in range(16):
                    g = gather_b(blk, hp)
                    tt = g.T if (2 * hp < NV or m_transposed) else None
                    for half, f in ((0, _lo), (1, _hi)):
                        h = 2 * hp + half
                        if h < NV:
                            Wv[h, t] = f(tt)
                        else:
                            Wm[h - NV, t] = pltpu.bitcast(f(tt if m_transposed else g).astype(BF16), U32)
                return c
            lax.fori_loop(0, nt, body, 0)

        def attn1(x):
            xc, rstd = ln_parts(x)
            xn = xc * rstd
            for kt in range(5):
                xr = jnp.broadcast_to(xn[0:1, 128 * kt:128 * (kt + 1)], (32, 128))
                A = jnp.where(A_mask, xr, 0.0).astype(BF16)
                V = _dot(A, E4)
                v_s[pl.ds(32 * kt, 32), :] = dup_bf16(V)
            wait("wq")
            q = masked_lhs_matmul(160, lambda t: wq_s[pl.ds(128 * t, 128), :])
            qb = q.astype(BF16)
            if not opt.get("noprep"): prep_heads(wq_u, 5, WQv, WQm, False, NV1)
            wait("wuk")
            hsel = (_iota((8, 128), 1) % 32) // 8
            rsel = _iota((8, 128), 1) % 8
            srow = _iota((8, 128), 0)
            vblocks = []
            for b0 in range(0, 128, 8):
                rhs = []
                for b in range(b0, b0 + 8):
                    for cl in range(4):
                        rhs.append(wuk_s[pl.ds(32 * (128 * cl + b), 32), :])
                o = lax.dot_general(qb, jnp.concatenate(rhs, axis=0), NT, preferred_element_type=F32)
                vb = None
                for i in range(8):
                    ob = o[:, 128 * i:128 * (i + 1)]
                    u = jnp.where(hsel == 0, ob[0:8], jnp.where(hsel == 1, ob[8:16], jnp.where(hsel == 2, ob[16:24], ob[24:32])))
                    u = jnp.where(srow == rsel, u, 0.0)
                    r_ = jnp.broadcast_to(jnp.sum(u, axis=0, keepdims=True), (8, 128))
                    vb = r_ if vb is None else jnp.where(srow == i, r_, vb)
                vblocks.append(vb)
            Qt = jnp.concatenate(vblocks, axis=0).T
            qa = jnp.concatenate([Qt[32 * cl:32 * (cl + 1)] for cl in range(4)], axis=1)
            qab = qa.astype(BF16)
            if not opt.get("noprep"): prep_heads(wuk_u, 4, WKv, WKm, True, NV1)
            scale = D ** -0.5
            wait("ckv")
            KC = 512
            mx = None
            for kc in range(SK // KC):
                s = lax.dot_general(qab, ckv_s[pl.ds(kc * KC, KC), :], NT, preferred_element_type=F32) * scale
                s_s[:, pl.ds(kc * KC, KC)] = s
                for j in range(KC // 128):
                    sj = s[:, 128 * j:128 * (j + 1)]
                    mx = sj if mx is None else jnp.maximum(mx, sj)
            mx = jnp.max(mx, axis=1, keepdims=True)
            l = None
            o = None
            for kc in range(SK // KC):
                p = jnp.exp(s_s[:, pl.ds(kc * KC, KC)] - mx)
                for j in range(KC // 128):
                    pj = p[:, 128 * j:128 * (j + 1)]
                    l = pj if l is None else l + pj
                oc = _dot(p.astype(BF16), ckv_s[pl.ds(kc * KC, KC), :])
                o = oc if o is None else o + oc
            l = _xsum(l)
            o = o * (1.0 / l)
            def ckv_body(i, c):
                for j in range(2):
                    kt = 2 * i + j
                    for ct in range(4):
                        t = ckv_s[pl.ds(pl.multiple_of(128 * kt, 128), 128), pl.ds(128 * ct, 128)]
                        ckvT[kt, pl.ds(64 * ct, 64), :] = pltpu.bitcast(t.T, U32)
                        ckvN[kt, ct] = pltpu.bitcast(t, U32)
                return c
            if not opt.get("noprep"): lax.fori_loop(0, 16, ckv_body, 0)
            Obig = jnp.concatenate([o[:, 128 * cl:128 * (cl + 1)] for cl in range(4)], axis=0)
            v_s[pl.ds(0, 128), :] = dup_bf16(Obig.T)
            wait("wuv")
            ctx = masked_lhs_matmul(128, lambda b: jnp.concatenate([wuv_s[pl.ds(32 * (128 * cl + b), 32), :] for cl in range(4)], axis=0))
            ctxb = ctx.astype(BF16)
            if not opt.get("noprep"): prep_heads(wuv_u, 4, WVv, WVm, False, NV2)
            wait("wo")
            r16 = _iota((16, 128), 0)
            acc = None
            for g in range(2):
                cg = ctxb[16 * g:16 * (g + 1)]
                for h0 in range(0, 16, 4):
                    lhs = [jnp.where(r16 == h, cg, jnp.zeros_like(cg)) for h in range(h0, h0 + 4)]
                    rhs = wo_s[pl.ds(128 * (16 * g + h0), 512), :]
                    oo = _dot(jnp.concatenate(lhs, axis=1), rhs)
                    acc = oo if acc is None else acc + oo
            out = jnp.sum(acc, axis=0, keepdims=True)
            xo = x + out

            def wo_v(h, c):
                for mt in range(5):
                    WOv[h, mt] = wo_s[pl.ds(pl.multiple_of(128 * h, 128), 128), pl.ds(128 * mt, 128)].astype(F32)
                return c
            if not opt.get("noprep"): lax.fori_loop(0, NV2, wo_v, 0)

            def wo_m(j, c):
                for mt in range(5):
                    WOm[j, mt] = pltpu.bitcast(wo_s[pl.ds(pl.multiple_of(128 * (j + NV2), 128), 128), pl.ds(128 * mt, 128)], U32)
                return c
            if not opt.get("noprep"): lax.fori_loop(0, H - NV2, wo_m, 0)
            return xo

        def prep_gu(w_s, Wm, Wv):
            if opt.get("noprep"): return
            nb = FV // 32
            for ft in range(FT):
                for mt in range(5):
                    t = w_s[pl.ds(FV + 128 * ft, 128), pl.ds(128 * mt, 128)]
                    Wm[ft, mt] = pltpu.bitcast(t.T, U32)
                for b in range(ft * nb // FT, (ft + 1) * nb // FT):
                    for mt in range(5):
                        Wv[mt, pl.ds(32 * b, 32), :] = w_s[pl.ds(32 * b, 32), pl.ds(128 * mt, 128)].astype(F32)

        def prep_v(w_s, Wv):
            if opt.get("noprep"): return
            def body(i, c):
                for j in range(2):
                    f0 = pl.multiple_of(FV // 2 * i + FV // 4 * j, 16)
                    for mt in range(5):
                        Wv[mt, pl.ds(f0, FV // 4), :] = w_s[pl.ds(f0, FV // 4), pl.ds(128 * mt, 128)].astype(F32)
                return c
            lax.fori_loop(0, 2, body, 0)

        def router(xn):
            wr = wr_s[...].astype(F32).reshape(1, M)
            return jax.nn.sigmoid(_xsum(xn * wr))

        def ffn1(x):
            xc, rstd = ln_parts(x)
            xn = xc * rstd
            rs = router(xn)
            xb = jnp.broadcast_to(xn[0:1], (16, M)).astype(BF16)
            wait("wg")
            g = [lax.dot_general(xb, wg_s[pl.ds(a, n), :], NT, preferred_element_type=F32)[0:8] for a, n in ((0, FV), (FV, FM))]
            prep_gu(wg_s, WGm, WGv)
            wait("wu")
            u = [lax.dot_general(xb, wu_s[pl.ds(a, n), :], NT, preferred_element_type=F32)[0:8] for a, n in ((0, FV), (FV, FM))]
            hb = []
            for gg, uu in zip(g, u):
                hh = gg * jax.nn.sigmoid(gg) * uu
                hb.append(jnp.broadcast_to(hh[0:1], (16, hh.shape[1])).astype(BF16))
            prep_gu(wu_s, WUm, WUv)
            y = None
            for i, (a, n) in enumerate(WD_CH):
                wait(f"wd{i}")
                if i == 0:
                    lhs = hb[0]
                else:
                    lhs = hb[1][:, a - FV:a - FV + n]
                yc = _dot(lhs, wd_s[pl.ds(a, n), :])[0:8]
                y = yc if y is None else y + yc
                if i == 0:
                    prep_v(wd_s, WDv)
            upd = xn * 0.0 + y * rs
            return x + (xn + upd)

        W = dict(WQm=WQm, WKm=WKm, WVm=WVm, WOm=WOm, WQv=WQv, WKv=WKv, WVv=WVv, WOv=WOv, ckvT=ckvT, ckvN=ckvN,
                 WGm=WGm, WUm=WUm, WDm=WDm, WGv=WGv, WUv=WUv, WDv=WDv)

        def attn2(x):
            xc, rstd = ln_parts(x)
            stage_BC(xc, W, qa_s, NV1, opt["BC"])
            if opt.get("stop") == "BC":
                return x + jnp.concatenate([qa_s[0:8, :], qa_s[8:16, 0:128]], axis=1)
            for ft in range(FT):
                for mt in range(5):
                    WDm[ft, mt] = pltpu.bitcast(wd_s[pl.ds(FV + 128 * ft, 128), pl.ds(128 * mt, 128)], U32)
            O = stage_DF(qa_s, rstd[0:1] * (D ** -0.5 * LOG2E), W, s_s, opt["DF"])
            if opt.get("stop") == "DF":
                return x + jnp.concatenate([O[0][0:8], O[1][0:8], O[2][0:8], O[3][0:8], O[0][8:16] + O[1][8:16] + O[2][8:16] + O[3][8:16]
                    + O[0][16:24] + O[1][16:24] + O[2][16:24] + O[3][16:24] + O[0][24:32] + O[1][24:32] + O[2][24:32] + O[3][24:32]], axis=1)
            out = stage_GH(O, W, NV2, opt["GH"])
            return x + jnp.concatenate(out, axis=1)

        def ffn2(x):
            xc, rstd = ln_parts(x)
            xn = xc * rstd
            rs = router(xn)
            out = stage_IJ(xc, rstd, W, FT, opt["IJ"])
            upd = xn * 0.0 + jnp.concatenate(out, axis=1) * (rs * rstd)
            return x + (xn + upd)

        wait("x")
        wait("wr")
        x = jnp.broadcast_to(x_s[0].astype(F32), (8, M))
        x = attn1(x)
        x = ffn1(x)
        if not opt.get("skip2"):
            x = attn2(x)
            if not opt.get("stop"): x = ffn2(x)
        o_ref[0] = x[0:1].astype(BF16)

    def run(A_x, A_c_kv, A_w_q, A_w_uk, A_w_uv, A_w_o, B_x, B_w_r, B_w_gate, B_w_up, B_w_down):
        anyspec = pl.BlockSpec(memory_space=pl.ANY)
        vm = pl.BlockSpec(memory_space=pltpu.VMEM)
        return pl.pallas_call(
            _kernel,
            out_shape=jax.ShapeDtypeStruct((1, 1, M), BF16),
            in_specs=[anyspec] * 10,
            out_specs=vm,
            scratch_shapes=[
                pltpu.VMEM((1, 1, M), BF16), pltpu.VMEM((M,), BF16),
                pltpu.VMEM((M * H, D), BF16), pltpu.VMEM((DC * H, D), BF16), pltpu.VMEM((SK, DC), BF16),
                pltpu.VMEM((DC * H, D), BF16), pltpu.VMEM((H * D, M), BF16),
                pltpu.VMEM((FF, M), BF16), pltpu.VMEM((FF, M), BF16), pltpu.VMEM((FF, M), BF16),
                pltpu.VMEM((160, 128), U32), pltpu.VMEM((H, SK), F32), pltpu.VMEM((H, DC), F32),
                pltpu.VMEM((H - NV1, 5, 64, 128), U32), pltpu.VMEM((H - NV1, 4, 64, 128), U32),
                pltpu.VMEM((H - NV2, 4, 64, 128), U32), pltpu.VMEM((H - NV2, 5, 64, 128), U32),
                pltpu.VMEM((NV1, 5, 128, 128), F32), pltpu.VMEM((NV1, 4, 128, 128), F32),
                pltpu.VMEM((NV2, 4, 128, 128), F32), pltpu.VMEM((NV2, 5, 128, 128), F32),
                pltpu.VMEM((32, 256, 128), U32), pltpu.VMEM((32, 4, 64, 128), U32),
                pltpu.VMEM((FT, 5, 64, 128), U32), pltpu.VMEM((FT, 5, 64, 128), U32), pltpu.VMEM((FT, 5, 64, 128), U32),
                pltpu.VMEM((5, FV, 128), F32), pltpu.VMEM((5, FV, 128), F32), pltpu.VMEM((5, FV, 128), F32),
                pltpu.SemaphoreType.DMA((16,)),
            ],
            compiler_params=pltpu.CompilerParams(vmem_limit_bytes=110 * 1024 * 1024, flags=flags),
            name=f"fused_v5_{NV1}_{NV2}_{FT}{tag}",
        )(A_x, A_c_kv, A_w_q.reshape(M * H, D), A_w_uk.reshape(DC * H, D), A_w_uv.reshape(DC * H, D),
          A_w_o.reshape(H * D, M), B_w_r, B_w_gate.T, B_w_up.T, B_w_down)
    return run


OPT = dict(BC=dict(lag=3, dstep=8, doff=29), DF=dict(nh=16), GH=dict(lag=3, dstep=16, doff=25), IJ=dict(lag=3, dstep=8, doff=20, vlag=12))
_run = make_kernel(15, 15, 7, OPT)


@jax.jit
def pallas_interleave_layers__compressed_kv_cla__moe_arch_mod__decode_kernel(
    A_x, A_c_kv, A_w_q, A_w_uk, A_w_uv, A_w_o, B_x, B_w_r, B_w_gate, B_w_up, B_w_down):
    return _run(A_x, A_c_kv, A_w_q, A_w_uk, A_w_uv, A_w_o, B_x, B_w_r, B_w_gate, B_w_up, B_w_down)
```

```python
import functools
import math
import jax
import jax.numpy as jnp
from jax import lax
import jax.experimental.pallas as pl
import jax.experimental.pallas.tpu as pltpu

F32 = jnp.float32
BF16 = jnp.bfloat16
U32 = jnp.uint32
M = 640
H = 32
D = 128
DC = 512
SK = 4096
FF = 1728
EPS = 1e-5
LOG2E = math.log2(math.e)

NT = (((1,), (1,)), ((), ()))


def _iota(shape, dim):
    return lax.broadcasted_iota(jnp.int32, shape, dim)


def _dot(a, b):
    return jnp.dot(a, b, preferred_element_type=F32)


def _lo(u):
    return pltpu.bitcast(u << 16, F32)


def _hi(u):
    return pltpu.bitcast(u & jnp.uint32(0xFFFF0000), F32)


def _pack16(v):
    return jnp.concatenate([v, v], axis=0).astype(BF16)


def _as_bf16(u):
    return pltpu.bitcast(u, BF16)


def _xsum(v):
    return jnp.sum(v, axis=1, keepdims=True)


def _interleave(*streams):
    items = []
    for si, s in enumerate(streams):
        n = len(s)
        for i, th in enumerate(s):
            items.append(((i + 0.5) / n, si, th))
    items.sort(key=lambda t: (t[0], t[1]))
    for _, _, th in items:
        th()


PHI = 1.0
def _interleave(*streams):
    items = []
    for si, s in enumerate(streams):
        n = len(s)
        for i, th in enumerate(s):
            items.append(((i + 0.5) / n * (PHI if si == 1 else 1.0), si, th))
    items.sort(key=lambda t: (t[0], t[1]))
    for _, _, th in items:
        th()

def ln_parts(x):
    mean = _xsum(x) * (1.0 / M)
    xc = x - mean
    var = _xsum(xc * xc) * (1.0 / M)
    return xc, lax.rsqrt(var + EPS)

def two_step(NV, nmult, first, second, opt, fin):
    st = {}
    dstep = opt.get("dstep", 8); doff = opt.get("doff", 29)
    s0 = opt.get("s0", 0)
    zneed = set(s - doff for s in range(0, NV * 16, dstep) if s >= s0)
    def fA(i, db):
        def f():
            s = i * 16 + db
            if db % dstep == 0:
                if first.get("shared"):
                    base = st.get("m", first["mult"](i))
                else:
                    base = first["mult"](i) if db == 0 else st["m"]
                key = ("z", s - doff)
                if key in st:
                    z = st.pop(key)
                    st["m"] = [v + z for v in base]
                else:
                    st["m"] = base
            xx = st["m"]
            a = None
            for k in range(len(xx)):
                p = first["w"](i, k, db) * xx[k]
                a = p if a is None else a + p
            st[("b", s)] = _xsum(a)
        return f
    def fB(i, db):
        def f():
            s = i * 16 + db
            b = st.pop(("b", s))
            n = second["n"]
            for k in range(n):
                p = second["w"](i, k, db) * b
                key = second["acc"](i, k)
                st[key] = p if key not in st else st[key] + p
            if s in zneed:
                st[("z", s)] = st[second["acc"](i, n - 1)] * 0.0
            if db == 15:
                fin(i, st)
        return f
    vs = []
    for i in range(NV + 1):
        for db in range(16):
            if i < NV: vs.append(fA(i, db))
            if i >= 1: vs.append(fB(i - 1, db))
    return vs, st

def stage_BC(xc, W, qa_s, NV, opt):
    NM = H - NV
    WQm, WKm, WQv, WKv = W["WQm"], W["WKm"], W["WQv"], W["WKv"]
    xv = [xc[:, 128 * mt:128 * (mt + 1)] for mt in range(5)]
    XL = [_pack16(v) for v in xv]
    st = {}
    ms = []
    def mB(j, mt):
        def f():
            o = _dot(XL[mt], _as_bf16(WQm[j, mt]))[0:8]
            st[("q", j)] = o if mt == 0 else st[("q", j)] + o
            if mt == 4:
                st[("qL", j)] = _pack16(st.pop(("q", j)))
        return f
    def mC(j, ct):
        def f():
            o = _dot(st[("qL", j)], _as_bf16(WKm[j, ct]))
            qa_s[pl.ds(NV + j, 1), pl.ds(128 * ct, 128)] = o[0:1]
        return f
    lag = opt.get("lag", 2)
    if lag == "sweep":
        for j in range(NM): ms += [mB(j, mt) for mt in range(5)]
        for ct in range(4): ms += [mC(j, ct) for j in range(NM)]
    else:
        for j in range(NM + lag):
            if j < NM: ms += [mB(j, mt) for mt in range(5)]
            if j >= lag: ms += [mC(j - lag, ct) for ct in range(4)]
    if NV == 0:
        _interleave(ms); return
    def fin(i, s):
        for ct in range(4):
            qa_s[pl.ds(i, 1), pl.ds(128 * ct, 128)] = jnp.sum(s.pop(("c", i, ct)), axis=0, keepdims=True)
    vs, _ = two_step(NV, 5,
        dict(shared=1, mult=lambda i: xv, w=lambda i, k, db: WQv[i, k, pl.ds(8 * db, 8), :]),
        dict(n=4, w=lambda i, k, db: WKv[i, k, pl.ds(8 * db, 8), :], acc=lambda i, k: ("c", i, k)), opt, fin)
    if opt.get("nomxu"): ms = []
    if opt.get("novpu"): vs = []
    _interleave(*[s for s in (ms, vs) if s])

def stage_DF(qa_s, scale, W, s_s, opt):
    ckvT, ckvN = W["ckvT"], W["ckvN"]
    QL = [(qa_s[:, pl.ds(128 * ct, 128)] * scale).astype(BF16) for ct in range(4)]
    NH = opt.get("nh", 16)
    NA = opt.get("na", 0)
    def Dt(kt, ct):
        return _dot(QL[ct], _as_bf16(ckvT[kt, pl.ds(64 * ct, 64), :]))
    for kt in range(NA):
        s_s[:, pl.ds(128 * kt, 128)] = Dt(kt, 0)
    mx = [None, None]
    for kt in range(32):
        if kt < NA:
            sc = s_s[:, pl.ds(128 * kt, 128)]
            for ct in range(1, 4): sc = sc + Dt(kt, ct)
        else:
            sc = Dt(kt, 0)
            for ct in range(1, 4): sc = sc + Dt(kt, ct)
        s_s[:, pl.ds(128 * kt, 128)] = sc
        hf = int(kt >= NH)
        mx[hf] = sc if mx[hf] is None else jnp.maximum(mx[hf], sc)
    m0 = jnp.max(mx[0], axis=1, keepdims=True)
    m1 = jnp.maximum(m0, jnp.max(mx[1], axis=1, keepdims=True))
    alpha = jnp.exp2(m0 - m1)
    l = None; O = [None] * 4
    def Ft(pb, kt, ct):
        o = _dot(pb, _as_bf16(ckvN[kt, ct]))
        O[ct] = o if O[ct] is None else O[ct] + o
    for kt in range(NH):
        p = jnp.exp2(s_s[:, pl.ds(128 * kt, 128)] - m0)
        l = p if l is None else l + p
        pb = p.astype(BF16)
        for ct in range(4): Ft(pb, kt, ct)
    l = l * alpha
    if opt.get("sweep", 0):
        P = {}
        for ct in range(4):
            O[ct] = O[ct] * alpha
            for kt in range(NH, 32):
                if ct == 0:
                    p = jnp.exp2(s_s[:, pl.ds(128 * kt, 128)] - m1)
                    l = l + p
                    P[kt] = p.astype(BF16)
                Ft(P[kt], kt, ct)
    else:
        O = [o * alpha for o in O]
        for kt in range(NH, 32):
            p = jnp.exp2(s_s[:, pl.ds(128 * kt, 128)] - m1)
            l = l + p
            pb = p.astype(BF16)
            for ct in range(4): Ft(pb, kt, ct)
    ls = _xsum(l)
    r0 = pl.reciprocal(ls, approx=True)
    inv = r0 * (2.0 - ls * r0)
    return [o * inv for o in O]

def stage_GH(O, W, NV, opt):
    NM = H - NV
    WVm, WOm, WVv, WOv = W["WVm"], W["WOm"], W["WVv"], W["WOv"]
    st = {}
    ms = []
    def mG(j, ct):
        def f():
            h = NV + j
            OL = jnp.broadcast_to(O[ct][h:h + 1], (16, 128)).astype(BF16)
            o = _dot(OL, _as_bf16(WVm[j, ct]))[0:8]
            st[("x", j)] = o if ct == 0 else st[("x", j)] + o
            if ct == 3:
                st[("cL", j)] = _pack16(st.pop(("x", j)))
        return f
    def mH(j, mt):
        def f():
            o = _dot(st[("cL", j)], _as_bf16(WOm[j, mt]))[0:8]
            st[("hm", mt)] = o if j == 0 else st[("hm", mt)] + o
        return f
    lag = opt.get("lag", 2)
    if lag == "sweep":
        for ct in range(4): ms += [mG(j, ct) for j in range(NM)]
        for j in range(NM): ms += [mH(j, mt) for mt in range(5)]
    else:
        for j in range(NM + lag):
            if j < NM: ms += [mG(j, ct) for ct in range(4)]
            if j >= lag: ms += [mH(j - lag, mt) for mt in range(5)]
    vs, sv = two_step(NV, 4,
        dict(mult=lambda i: [jnp.broadcast_to(O[ct][i:i + 1], (8, 128)) for ct in range(4)],
             w=lambda i, k, db: WVv[i, k, pl.ds(8 * db, 8), :]),
        dict(n=5, w=lambda i, k, db: WOv[i, k, pl.ds(8 * db, 8), :], acc=lambda i, k: ("hv", k)), opt, lambda i, s: None)
    _interleave(ms, vs)
    return [st[("hm", mt)] + jnp.sum(sv[("hv", mt)], axis=0, keepdims=True) for mt in range(5)]

def stage_IJ(xc, rstd, W, FT, opt):
    FV = FF - 128 * FT
    _tanh = (lambda t: t * t) if opt.get("notanh") else jnp.tanh
    WGm, WUm, WDm, WGv, WUv, WDv = (W[k] for k in ("WGm", "WUm", "WDm", "WGv", "WUv", "WDv"))
    xv = [xc[:, 128 * mt:128 * (mt + 1)] for mt in range(5)]
    XL = [_pack16(v) for v in xv]
    hs = jnp.broadcast_to(0.5 * rstd, (8, 128))
    st = {}
    ms = []
    def mI(ft, which, mt):
        def f():
            Wm = WGm if which == 0 else WUm
            o = _dot(XL[mt], _as_bf16(Wm[ft, mt]))[0:8]
            st[("g", ft, which)] = o if mt == 0 else st[("g", ft, which)] + o
            if which == 1 and mt == 4:
                t = st.pop(("g", ft, 0)) * hs
                hh = (t * st.pop(("g", ft, 1))) * (1.0 + _tanh(t))
                st[("hL", ft)] = _pack16(hh)
        return f
    def mJ(ft, mt):
        def f():
            o = _dot(st[("hL", ft)], _as_bf16(WDm[ft, mt]))[0:8]
            st[("ym", mt)] = o if ft == 0 else st[("ym", mt)] + o
        return f
    lag = opt.get("lag", 1)
    for ft in range(FT + lag):
        if ft < FT: ms += [mI(ft, w, mt) for w in range(2) for mt in range(5)]
        if ft >= lag: ms += [mJ(ft - lag, mt) for mt in range(5)]
    vs = []
    NB = FV // 8
    dstep = opt.get("dstep", 8); doff = opt.get("doff", 16)
    LAG = opt.get("vlag", 8)
    zneed = set(s - doff for s in range(0, NB, dstep) if s >= opt.get("s0", 0))
    def vI(fb, which):
        def f():
            if which == 0 and fb % dstep == 0:
                key = ("z", fb - doff)
                if key in st:
                    z = st.pop(key)
                    st["xv"] = [v + z for v in st.get("xv", xv)]
                else:
                    st["xv"] = st.get("xv", xv)
            Wv = WGv if which == 0 else WUv
            a = None
            for mt in range(5):
                p = Wv[mt, pl.ds(8 * fb, 8), :] * st["xv"][mt]
                a = p if a is None else a + p
            st[("gb", fb, which)] = jnp.broadcast_to(_xsum(a), (8, 128))
        return f
    def vJ(fb):
        def f():
            t = st.pop(("gb", fb, 0)) * hs
            hh = (t * st.pop(("gb", fb, 1))) * (1.0 + _tanh(t))
            for mt in range(5):
                p = WDv[mt, pl.ds(8 * fb, 8), :] * hh
                st[("yv", mt)] = p if fb == 0 else st[("yv", mt)] + p
            if fb in zneed:
                st[("z", fb)] = st[("yv", 4)] * 0.0
        return f
    for fb in range(NB + LAG):
        if fb < NB: vs += [vI(fb, 0), vI(fb, 1)]
        if fb >= LAG: vs.append(vJ(fb - LAG))
    if opt.get("nomxu"):
        _interleave(vs)
        return [jnp.broadcast_to(jnp.sum(st[("yv", mt)], axis=0, keepdims=True), (8, 128)) for mt in range(5)]
    if opt.get("novpu"):
        _interleave(ms)
        return [st[("ym", mt)] for mt in range(5)]
    _interleave(ms, vs)
    return [st[("ym", mt)] + jnp.sum(st[("yv", mt)], axis=0, keepdims=True) for mt in range(5)]


def make_kernel(NV1, NV2, FT, opt, flags=None, tag=''):
    FM = 128 * FT
    FV = FF - FM
    WD_CH = [(0, FV), (FV, FM - 256), (FF - 256, 256)]

    def _kernel(x_hbm, ckv_hbm, wq_hbm, wuk_hbm, wuv_hbm, wo_hbm, wr_hbm, wg_hbm, wu_hbm, wd_hbm,
                o_ref,
                x_s, wr_s, wq_s, wuk_s, ckv_s, wuv_s, wo_s, wg_s, wu_s, wd_s,
                v_s, s_s, qa_s,
                WQm, WKm, WVm, WOm, WQv, WKv, WVv, WOv, ckvT, ckvN, WGm, WUm, WDm, WGv, WUv, WDv,
                sems):
        cps = {}
        k = 0

        def mk(name, src, dst):
            nonlocal k
            cps[name] = pltpu.make_async_copy(src, dst, sems.at[k])
            k += 1
        mk("x", x_hbm, x_s)
        mk("wr", wr_hbm, wr_s)
        mk("wq", wq_hbm, wq_s)
        mk("wuk", wuk_hbm, wuk_s)
        mk("ckv", ckv_hbm.at[0], ckv_s)
        mk("wuv", wuv_hbm, wuv_s)
        mk("wo", wo_hbm, wo_s)
        mk("wg", wg_hbm, wg_s)
        mk("wu", wu_hbm, wu_s)
        for i, (a, n) in enumerate(WD_CH):
            mk(f"wd{i}", wd_hbm.at[pl.ds(a, n)], wd_s.at[pl.ds(a, n)])
        for c in cps.values():
            c.start()

        def wait(name):
            cps[name].wait()

        wq_u = wq_s.bitcast(U32)
        wuk_u = wuk_s.bitcast(U32)
        wuv_u = wuv_s.bitcast(U32)

        lane = _iota((128, 128), 1)
        row = _iota((128, 128), 0)
        E4 = jnp.where(row % 4 == lane // 32, 1.0, 0.0).astype(BF16)
        A_mask = _iota((32, 128), 1) // 4 == _iota((32, 128), 0)
        ls = _iota((16, 128), 0)
        lj = _iota((16, 128), 1) % 32
        M32 = jnp.where(lj == 2 * ls, jnp.uint32(0x0000FFFF), jnp.where(lj == 2 * ls + 1, jnp.uint32(0xFFFF0000), jnp.uint32(0)))

        def ln_parts(x):
            mean = _xsum(x) * (1.0 / M)
            xc = x - mean
            var = _xsum(xc * xc) * (1.0 / M)
            return xc, lax.rsqrt(var + EPS)

        def dup_bf16(v):
            u = pltpu.bitcast(v.astype(BF16).astype(F32), U32)
            return u | (u >> 16)

        def masked_lhs_matmul(nrows, get_tile):
            acc = None
            G = 8
            for t0 in range(0, nrows, G):
                lhs = []
                rhs = []
                for t in range(t0, t0 + G):
                    vrow = jnp.broadcast_to(v_s[pl.ds(t, 1), :], (16, 128))
                    lhs.append(pltpu.bitcast(vrow & M32, BF16))
                    rhs.append(get_tile(t))
                o = _dot(jnp.concatenate(lhs, axis=1), jnp.concatenate(rhs, axis=0))
                acc = o if acc is None else acc + o
            return acc

        def gather(wu, hp, x0, n):
            return jnp.concatenate([wu[pl.ds((x0 + 8 * r) * 16 + hp, 8, stride=16), :] for r in range(n // 8)], axis=0)

        def gather_b(blk, hp):
            return jnp.concatenate([blk[pl.ds(128 * r + hp, 8, stride=16), :] for r in range(16)], axis=0)

        def prep_heads(wu, nt, Wv, Wm, m_transposed, NV):
            def body(t, c):
                blk = wu.at[pl.ds(pl.multiple_of(t * 2048, 2048), 2048)]
                for hp in range(16):
                    g = gather_b(blk, hp)
                    tt = g.T if (2 * hp < NV or m_transposed) else None
                    for half, f in ((0, _lo), (1, _hi)):
                        h = 2 * hp + half
                        if h < NV:
                            Wv[h, t] = f(tt)
                        else:
                            Wm[h - NV, t] = pltpu.bitcast(f(tt if m_transposed else g).astype(BF16), U32)
                return c
            lax.fori_loop(0, nt, body, 0)

        def attn1(x):
            xc, rstd = ln_parts(x)
            xn = xc * rstd
            for kt in range(5):
                xr = jnp.broadcast_to(xn[0:1, 128 * kt:128 * (kt + 1)], (32, 128))
                A = jnp.where(A_mask, xr, 0.0).astype(BF16)
                V = _dot(A, E4)
                v_s[pl.ds(32 * kt, 32), :] = dup_bf16(V)
            wait("wq")
            q = masked_lhs_matmul(160, lambda t: wq_s[pl.ds(128 * t, 128), :])
            qb = q.astype(BF16)
            if not opt.get("noprep"): prep_heads(wq_u, 5, WQv, WQm, False, NV1)
            wait("wuk")
            hsel = (_iota((8, 128), 1) % 32) // 8
            rsel = _iota((8, 128), 1) % 8
            srow = _iota((8, 128), 0)
            vblocks = []
            for b0 in range(0, 128, 8):
                rhs = []
                for b in range(b0, b0 + 8):
                    for cl in range(4):
                        rhs.append(wuk_s[pl.ds(32 * (128 * cl + b), 32), :])
                o = lax.dot_general(qb, jnp.concatenate(rhs, axis=0), NT, preferred_element_type=F32)
                vb = None
                for i in range(8):
                    ob = o[:, 128 * i:128 * (i + 1)]
                    u = jnp.where(hsel == 0, ob[0:8], jnp.where(hsel == 1, ob[8:16], jnp.where(hsel == 2, ob[16:24], ob[24:32])))
                    u = jnp.where(srow == rsel, u, 0.0)
                    r_ = jnp.broadcast_to(jnp.sum(u, axis=0, keepdims=True), (8, 128))
                    vb = r_ if vb is None else jnp.where(srow == i, r_, vb)
                vblocks.append(vb)
            Qt = jnp.concatenate(vblocks, axis=0).T
            qa = jnp.concatenate([Qt[32 * cl:32 * (cl + 1)] for cl in range(4)], axis=1)
            qab = qa.astype(BF16)
            if not opt.get("noprep"): prep_heads(wuk_u, 4, WKv, WKm, True, NV1)
            scale = D ** -0.5
            wait("ckv")
            KC = 512
            mx = None
            for kc in range(SK // KC):
                s = lax.dot_general(qab, ckv_s[pl.ds(kc * KC, KC), :], NT, preferred_element_type=F32) * scale
                s_s[:, pl.ds(kc * KC, KC)] = s
                for j in range(KC // 128):
                    sj = s[:, 128 * j:128 * (j + 1)]
                    mx = sj if mx is None else jnp.maximum(mx, sj)
            mx = jnp.max(mx, axis=1, keepdims=True)
            l = None
            o = None
            for kc in range(SK // KC):
                p = jnp.exp(s_s[:, pl.ds(kc * KC, KC)] - mx)
                for j in range(KC // 128):
                    pj = p[:, 128 * j:128 * (j + 1)]
                    l = pj if l is None else l + pj
                oc = _dot(p.astype(BF16), ckv_s[pl.ds(kc * KC, KC), :])
                o = oc if o is None else o + oc
            l = _xsum(l)
            o = o * (1.0 / l)
            def ckv_body(i, c):
                for j in range(2):
                    kt = 2 * i + j
                    for ct in range(4):
                        t = ckv_s[pl.ds(pl.multiple_of(128 * kt, 128), 128), pl.ds(128 * ct, 128)]
                        ckvT[kt, pl.ds(64 * ct, 64), :] = pltpu.bitcast(t.T, U32)
                        ckvN[kt, ct] = pltpu.bitcast(t, U32)
                return c
            if not opt.get("noprep"): lax.fori_loop(0, 16, ckv_body, 0)
            Obig = jnp.concatenate([o[:, 128 * cl:128 * (cl + 1)] for cl in range(4)], axis=0)
            v_s[pl.ds(0, 128), :] = dup_bf16(Obig.T)
            wait("wuv")
            ctx = masked_lhs_matmul(128, lambda b: jnp.concatenate([wuv_s[pl.ds(32 * (128 * cl + b), 32), :] for cl in range(4)], axis=0))
            ctxb = ctx.astype(BF16)
            if not opt.get("noprep"): prep_heads(wuv_u, 4, WVv, WVm, False, NV2)
            wait("wo")
            r16 = _iota((16, 128), 0)
            acc = None
            for g in range(2):
                cg = ctxb[16 * g:16 * (g + 1)]
                for h0 in range(0, 16, 4):
                    lhs = [jnp.where(r16 == h, cg, jnp.zeros_like(cg)) for h in range(h0, h0 + 4)]
                    rhs = wo_s[pl.ds(128 * (16 * g + h0), 512), :]
                    oo = _dot(jnp.concatenate(lhs, axis=1), rhs)
                    acc = oo if acc is None else acc + oo
            out = jnp.sum(acc, axis=0, keepdims=True)
            xo = x + out

            def wo_v(h, c):
                for mt in range(5):
                    WOv[h, mt] = wo_s[pl.ds(pl.multiple_of(128 * h, 128), 128), pl.ds(128 * mt, 128)].astype(F32)
                return c
            if not opt.get("noprep"): lax.fori_loop(0, NV2, wo_v, 0)

            def wo_m(j, c):
                for mt in range(5):
                    WOm[j, mt] = pltpu.bitcast(wo_s[pl.ds(pl.multiple_of(128 * (j + NV2), 128), 128), pl.ds(128 * mt, 128)], U32)
                return c
            if not opt.get("noprep"): lax.fori_loop(0, H - NV2, wo_m, 0)
            return xo

        def prep_gu(w_s, Wm, Wv):
            if opt.get("noprep"): return
            nb = FV // 32
            for ft in range(FT):
                for mt in range(5):
                    t = w_s[pl.ds(FV + 128 * ft, 128), pl.ds(128 * mt, 128)]
                    Wm[ft, mt] = pltpu.bitcast(t.T, U32)
                for b in range(ft * nb // FT, (ft + 1) * nb // FT):
                    for mt in range(5):
                        Wv[mt, pl.ds(32 * b, 32), :] = w_s[pl.ds(32 * b, 32), pl.ds(128 * mt, 128)].astype(F32)

        def prep_v(w_s, Wv):
            if opt.get("noprep"): return
            def body(i, c):
                for j in range(2):
                    f0 = pl.multiple_of(FV // 2 * i + FV // 4 * j, 16)
                    for mt in range(5):
                        Wv[mt, pl.ds(f0, FV // 4), :] = w_s[pl.ds(f0, FV // 4), pl.ds(128 * mt, 128)].astype(F32)
                return c
            lax.fori_loop(0, 2, body, 0)

        def router(xn):
            wr = wr_s[...].astype(F32).reshape(1, M)
            return jax.nn.sigmoid(_xsum(xn * wr))

        def ffn1(x):
            xc, rstd = ln_parts(x)
            xn = xc * rstd
            rs = router(xn)
            xb = jnp.broadcast_to(xn[0:1], (16, M)).astype(BF16)
            wait("wg")
            g = [lax.dot_general(xb, wg_s[pl.ds(a, n), :], NT, preferred_element_type=F32)[0:8] for a, n in ((0, FV), (FV, FM))]
            prep_gu(wg_s, WGm, WGv)
            wait("wu")
            u = [lax.dot_general(xb, wu_s[pl.ds(a, n), :], NT, preferred_element_type=F32)[0:8] for a, n in ((0, FV), (FV, FM))]
            hb = []
            for gg, uu in zip(g, u):
                hh = gg * jax.nn.sigmoid(gg) * uu
                hb.append(jnp.broadcast_to(hh[0:1], (16, hh.shape[1])).astype(BF16))
            prep_gu(wu_s, WUm, WUv)
            y = None
            for i, (a, n) in enumerate(WD_CH):
                wait(f"wd{i}")
                if i == 0:
                    lhs = hb[0]
                else:
                    lhs = hb[1][:, a - FV:a - FV + n]
                yc = _dot(lhs, wd_s[pl.ds(a, n), :])[0:8]
                y = yc if y is None else y + yc
                if i == 0:
                    prep_v(wd_s, WDv)
            upd = xn * 0.0 + y * rs
            return x + (xn + upd)

        W = dict(WQm=WQm, WKm=WKm, WVm=WVm, WOm=WOm, WQv=WQv, WKv=WKv, WVv=WVv, WOv=WOv, ckvT=ckvT, ckvN=ckvN,
                 WGm=WGm, WUm=WUm, WDm=WDm, WGv=WGv, WUv=WUv, WDv=WDv)

        def attn2(x):
            xc, rstd = ln_parts(x)
            if opt.get("fake3"):
                mu = _xsum(x) * (1.0 / M); rstd = lax.rsqrt(_xsum(x * x) * (1.0 / M) - mu * mu + EPS); xc = x
            stage_BC(xc, W, qa_s, NV1, opt["BC"])
            if opt.get("stop") == "BC":
                return x + jnp.concatenate([qa_s[0:8, :], qa_s[8:16, 0:128]], axis=1)
            for ft in range(FT):
                for mt in range(5):
                    WDm[ft, mt] = pltpu.bitcast(wd_s[pl.ds(FV + 128 * ft, 128), pl.ds(128 * mt, 128)], U32)
            O = stage_DF(qa_s, rstd[0:1] * (D ** -0.5 * LOG2E), W, s_s, opt["DF"])
            if opt.get("stop") == "DF":
                return x + jnp.concatenate([O[0][0:8], O[1][0:8], O[2][0:8], O[3][0:8], O[0][8:16] + O[1][8:16] + O[2][8:16] + O[3][8:16]
                    + O[0][16:24] + O[1][16:24] + O[2][16:24] + O[3][16:24] + O[0][24:32] + O[1][24:32] + O[2][24:32] + O[3][24:32]], axis=1)
            out = stage_GH(O, W, NV2, opt["GH"])
            return x + jnp.concatenate(out, axis=1)

        def ffn2(x):
            xc, rstd = ln_parts(x)
            xn = xc * rstd
            if opt.get("fake4"):
                mu = _xsum(x) * (1.0 / M); rstd = lax.rsqrt(_xsum(x * x) * (1.0 / M) - mu * mu + EPS); xc = x
                xn = (x - mu) * rstd
            rs = router(xn)
            out = stage_IJ(xc, rstd, W, FT, opt["IJ"])
            upd = xn * 0.0 + jnp.concatenate(out, axis=1) * (rs * rstd)
            return x + (xn + upd)

        wait("x")
        wait("wr")
        x = jnp.broadcast_to(x_s[0].astype(F32), (8, M))
        x = attn1(x)
        x = ffn1(x)
        if not opt.get("skip2"):
            x = attn2(x)
            if not opt.get("stop"): x = ffn2(x)
        o_ref[0] = x[0:1].astype(BF16)

    def run(A_x, A_c_kv, A_w_q, A_w_uk, A_w_uv, A_w_o, B_x, B_w_r, B_w_gate, B_w_up, B_w_down):
        anyspec = pl.BlockSpec(memory_space=pl.ANY)
        vm = pl.BlockSpec(memory_space=pltpu.VMEM)
        return pl.pallas_call(
            _kernel,
            out_shape=jax.ShapeDtypeStruct((1, 1, M), BF16),
            in_specs=[anyspec] * 10,
            out_specs=vm,
            scratch_shapes=[
                pltpu.VMEM((1, 1, M), BF16), pltpu.VMEM((M,), BF16),
                pltpu.VMEM((M * H, D), BF16), pltpu.VMEM((DC * H, D), BF16), pltpu.VMEM((SK, DC), BF16),
                pltpu.VMEM((DC * H, D), BF16), pltpu.VMEM((H * D, M), BF16),
                pltpu.VMEM((FF, M), BF16), pltpu.VMEM((FF, M), BF16), pltpu.VMEM((FF, M), BF16),
                pltpu.VMEM((160, 128), U32), pltpu.VMEM((H, SK), F32), pltpu.VMEM((H, DC), F32),
                pltpu.VMEM((H - NV1, 5, 64, 128), U32), pltpu.VMEM((H - NV1, 4, 64, 128), U32),
                pltpu.VMEM((H - NV2, 4, 64, 128), U32), pltpu.VMEM((H - NV2, 5, 64, 128), U32),
                pltpu.VMEM((NV1, 5, 128, 128), F32), pltpu.VMEM((NV1, 4, 128, 128), F32),
                pltpu.VMEM((NV2, 4, 128, 128), F32), pltpu.VMEM((NV2, 5, 128, 128), F32),
                pltpu.VMEM((32, 256, 128), U32), pltpu.VMEM((32, 4, 64, 128), U32),
                pltpu.VMEM((FT, 5, 64, 128), U32), pltpu.VMEM((FT, 5, 64, 128), U32), pltpu.VMEM((FT, 5, 64, 128), U32),
                pltpu.VMEM((5, FV, 128), F32), pltpu.VMEM((5, FV, 128), F32), pltpu.VMEM((5, FV, 128), F32),
                pltpu.SemaphoreType.DMA((12,)),
            ],
            compiler_params=pltpu.CompilerParams(vmem_limit_bytes=110 * 1024 * 1024, flags=flags, disable_semaphore_checks=bool(opt.get('nosemchk'))),
            name=f"fused_v5_{NV1}_{NV2}_{FT}{tag}",
        )(A_x, A_c_kv, A_w_q.reshape(M * H, D), A_w_uk.reshape(DC * H, D), A_w_uv.reshape(DC * H, D),
          A_w_o.reshape(H * D, M), B_w_r, B_w_gate.T, B_w_up.T, B_w_down)
    return run


OPT = dict(nosemchk=1, BC=dict(lag="sweep", dstep=8, doff=33, s0=48), DF=dict(nh=16, sweep=1, na=16),
           GH=dict(lag="sweep", dstep=8, doff=29, s0=48), IJ=dict(lag=3, dstep=8, doff=16, vlag=10, s0=24))
_run = make_kernel(15, 15, 8, OPT)


@jax.jit
def pallas_interleave_layers__compressed_kv_cla__moe_arch_mod__decode_kernel(
    A_x, A_c_kv, A_w_q, A_w_uk, A_w_uv, A_w_o, B_x, B_w_r, B_w_gate, B_w_up, B_w_down):
    return _run(A_x, A_c_kv, A_w_q, A_w_uk, A_w_uv, A_w_o, B_x, B_w_r, B_w_gate, B_w_up, B_w_down)
```

```python
import functools
import math
import jax
import jax.numpy as jnp
from jax import lax
import jax.experimental.pallas as pl
import jax.experimental.pallas.tpu as pltpu

F32 = jnp.float32
BF16 = jnp.bfloat16
U32 = jnp.uint32
M = 640
H = 32
D = 128
DC = 512
SK = 4096
FF = 1728
EPS = 1e-5
LOG2E = math.log2(math.e)

NT = (((1,), (1,)), ((), ()))


def _iota(shape, dim):
    return lax.broadcasted_iota(jnp.int32, shape, dim)


def _dot(a, b):
    return jnp.dot(a, b, preferred_element_type=F32)


def _lo(u):
    return pltpu.bitcast(u << 16, F32)


def _hi(u):
    return pltpu.bitcast(u & jnp.uint32(0xFFFF0000), F32)


def _pack16(v):
    return jnp.concatenate([v, v], axis=0).astype(BF16)


def _as_bf16(u):
    return pltpu.bitcast(u, BF16)


def _xsum(v):
    return jnp.sum(v, axis=1, keepdims=True)


def _interleave(*streams):
    items = []
    for si, s in enumerate(streams):
        n = len(s)
        for i, th in enumerate(s):
            items.append(((i + 0.5) / n, si, th))
    items.sort(key=lambda t: (t[0], t[1]))
    for _, _, th in items:
        th()


def _interleave(*streams, phi=1.0):
    items = []
    for si, s in enumerate(streams):
        n = len(s)
        for i, th in enumerate(s):
            items.append(((i + 0.5) / n * (phi if si == 1 else 1.0), si, th))
    items.sort(key=lambda t: (t[0], t[1]))
    for _, _, th in items:
        th()


def ln_parts(x):
    mean = _xsum(x) * (1.0 / M)
    xc = x - mean
    var = _xsum(xc * xc) * (1.0 / M)
    return xc, lax.rsqrt(var + EPS)

def two_step(NV, nmult, first, second, opt, fin):
    st = {}
    dstep = opt.get("dstep", 8); doff = opt.get("doff", 29)
    s0 = opt.get("s0", 0)
    zneed = set(s - doff for s in range(0, NV * 16, dstep) if s >= s0)
    def fA(i, db):
        def f():
            s = i * 16 + db
            if db % dstep == 0:
                if first.get("shared"):
                    base = st.get("m", first["mult"](i))
                else:
                    base = first["mult"](i) if db == 0 else st["m"]
                key = ("z", s - doff)
                if key in st:
                    z = st.pop(key)
                    st["m"] = [v + z for v in base]
                else:
                    st["m"] = base
            xx = st["m"]
            a = first["init"](i, db) if "init" in first else None
            for k in range(len(xx)):
                p = first["w"](i, k, db) * xx[k]
                a = p if a is None else a + p
            st[("b", s)] = _xsum(a)
            if "keep" in first:
                first["keep"](s, st[("b", s)])
        return f
    def fB(i, db):
        def f():
            s = i * 16 + db
            b = st.pop(("b", s))
            n = second["n"]
            for k in range(n):
                p = second["w"](i, k, db) * b
                key = second["acc"](i, k)
                st[key] = p if key not in st else st[key] + p
            if s in zneed:
                st[("z", s)] = st[second["acc"](i, n - 1)] * 0.0
            if db == 15:
                fin(i, st)
        return f
    vs = []
    for i in range(NV + 1):
        for db in range(16):
            if i < NV: vs.append(fA(i, db))
            if i >= 1: vs.append(fB(i - 1, db))
    return vs, st

def stage_BC(xc, W, qa_s, NV, opt, qb_s=None, dyn=None):
    NM = H - NV
    WQm, WKm, WQv, WKv = W["WQm"], W["WKm"], W["WQv"], W["WKv"]
    xv = [xc[:, 128 * mt:128 * (mt + 1)] for mt in range(5)]
    XL = [_pack16(v) for v in xv]
    st = {}
    ms = []
    def mB(j, mt):
        def f():
            o = _dot(XL[mt], _as_bf16(WQm[j, mt]))[0:8]
            st[("q", j)] = o if mt == 0 else st[("q", j)] + o
            if mt == 4:
                st[("qL", j)] = _pack16(st.pop(("q", j)))
        return f
    def mC(j, ct):
        def f():
            o = _dot(st[("qL", j)], _as_bf16(WKm[j, ct]))
            qa_s[pl.ds(NV + j, 1), pl.ds(128 * ct, 128)] = o[0:1]
        return f
    lag = opt.get("lag", 2)
    if lag == "sweep":
        for j in range(NM): ms += [mB(j, mt) for mt in range(5)]
        for ct in range(4): ms += [mC(j, ct) for j in range(NM)]
    elif opt.get("nsw"):
        n0 = NM - opt["nsw"]
        for j in range(NM):
            ms += [mB(j, mt) for mt in range(5)]
            if j >= lag and j - lag < n0: ms += [mC(j - lag, ct) for ct in range(4)]
        for j in range(max(NM - lag, 0), n0): ms += [mC(j, ct) for ct in range(4)]
        for ct in range(4): ms += [mC(j, ct) for j in range(n0, NM)]
    else:
        for j in range(NM + lag):
            if j < NM: ms += [mB(j, mt) for mt in range(5)]
            if j >= lag: ms += [mC(j - lag, ct) for ct in range(4)]
    if NV == 0:
        _interleave(ms); return
    NC = 2 if opt.get("split") else 4

    def fin(i, s):
        for ct in range(NC):
            qa_s[pl.ds(i, 1), pl.ds(128 * ct, 128)] = jnp.sum(s.pop(("c", i, ct)), axis=0, keepdims=True)
    first = dict(shared=1, mult=lambda i: xv, w=lambda i, k, db: WQv[i, k, pl.ds(8 * db, 8), :])
    if NC < 4:
        def keep(s, b):
            qb_s[pl.ds(dyn(8 * s, 8), 8), :] = jnp.broadcast_to(b, (8, 128))
        first["keep"] = keep
    vs, _ = two_step(NV, 5, first,
        dict(n=NC, w=lambda i, k, db: WKv[i, k, pl.ds(8 * db, 8), :], acc=lambda i, k: ("c", i, k)), opt, fin)
    _interleave(ms, vs)
    if NC == 4:
        return []
    sd = {}

    def late(i, db):
        def f():
            qb = qb_s[pl.ds(8 * (16 * i + db), 8), :]
            for ct in range(NC, 4):
                p = WKv[i, ct, pl.ds(8 * db, 8), :] * qb
                sd[ct] = p if db == 0 else sd[ct] + p
            if db == 15:
                for ct in range(NC, 4):
                    qa_s[pl.ds(i, 1), pl.ds(128 * ct, 128)] = jnp.sum(sd[ct], axis=0, keepdims=True)
        return f
    return [late(i, db) for i in range(NV) for db in range(16)]

def stage_DF(qa_s, scale, W, s_s, opt, corr=None, late=(), early_g=None, pin=None):
    ckvT, ckvN = W["ckvT"], W["ckvN"]
    u_s, mu = corr
    ms_ = mu * scale

    def QLf(ct):
        return (qa_s[:, pl.ds(128 * ct, 128)] * scale - u_s[:, pl.ds(128 * ct, 128)] * ms_).astype(BF16)
    NH = opt.get("nh", 16)

    def Dt(q, kt, ct):
        return _dot(q, _as_bf16(ckvT[kt, pl.ds(64 * ct, 64), :]))
    mx = [None, None]
    if late:
        QL = [QLf(0), QLf(1)]

        def dA(kt):
            def f():
                sa = Dt(QL[0], kt, 0) + Dt(QL[1], kt, 1)
                s_s[:, pl.ds(128 * kt, 128)] = sa
                if kt % opt.get("pin", 1) == 0:
                    pin(sa[0:8])
            return f
        _interleave([dA(kt) for kt in range(32)], list(late), phi=opt.get("phid", 0.8))
        QL += [QLf(2), QLf(3)]
        for kt in range(32):
            sc = s_s[:, pl.ds(128 * kt, 128)] + Dt(QL[2], kt, 2) + Dt(QL[3], kt, 3)
            s_s[:, pl.ds(128 * kt, 128)] = sc
            hf = int(kt >= NH)
            mx[hf] = sc if mx[hf] is None else jnp.maximum(mx[hf], sc)
    else:
        QL = [QLf(ct) for ct in range(4)]
        NA = opt.get("na", 0)
        for kt in range(NA):
            s_s[:, pl.ds(128 * kt, 128)] = Dt(QL[0], kt, 0)
        for kt in range(32):
            if kt < NA:
                sc = s_s[:, pl.ds(128 * kt, 128)]
                for ct in range(1, 4): sc = sc + Dt(QL[ct], kt, ct)
            else:
                sc = Dt(QL[0], kt, 0)
                for ct in range(1, 4): sc = sc + Dt(QL[ct], kt, ct)
            s_s[:, pl.ds(128 * kt, 128)] = sc
            hf = int(kt >= NH)
            mx[hf] = sc if mx[hf] is None else jnp.maximum(mx[hf], sc)
    m0 = jnp.max(mx[0], axis=1, keepdims=True)
    m1 = jnp.maximum(m0, jnp.max(mx[1], axis=1, keepdims=True))
    alpha = jnp.exp2(m0 - m1)
    l = None; O = [None] * 4

    def Ft(pb, kt, ct):
        o = _dot(pb, _as_bf16(ckvN[kt, ct]))
        O[ct] = o if O[ct] is None else O[ct] + o
    P = {}

    def mkP(kt, m):
        nonlocal l
        p = jnp.exp2(s_s[:, pl.ds(128 * kt, 128)] - m)
        l = p if l is None else l + p
        P[kt] = p.astype(BF16)
    if early_g is None:
        for kt in range(NH):
            mkP(kt, m0)
            for ct in range(4): Ft(P[kt], kt, ct)
        l = l * alpha
        for ct in range(4):
            O[ct] = O[ct] * alpha
            for kt in range(NH, 32):
                if ct == 0: mkP(kt, m1)
                Ft(P[kt], kt, ct)
        ls = _xsum(l)
        r0 = pl.reciprocal(ls, approx=True)
        inv = r0 * (2.0 - ls * r0)
        return [o * inv for o in O]
    for kt in range(NH):
        mkP(kt, m0)
        for ct in (0, 1): Ft(P[kt], kt, ct)
    l = l * alpha
    for ct in (0, 1): O[ct] = O[ct] * alpha
    for kt in range(NH, 32):
        mkP(kt, m1)
        for ct in (0, 1): Ft(P[kt], kt, ct)
    ls = _xsum(l)
    r0 = pl.reciprocal(ls, approx=True)
    inv = r0 * (2.0 - ls * r0)
    O[0] = O[0] * inv
    O[1] = O[1] * inv

    def f2(kt):
        def f():
            if kt == NH:
                for ct in (2, 3): O[ct] = O[ct] * alpha
            for ct in (2, 3): Ft(P[kt], kt, ct)
        return f
    _interleave([f2(kt) for kt in range(32)], early_g(O[0], O[1]), phi=opt.get("phif", 0.9))
    O[2] = O[2] * inv
    O[3] = O[3] * inv
    return O


def early_g_thunks(O0, O1, W, NV, a_s, dyn):
    WVv = W["WVv"]
    sd = {}

    def step(i, db):
        def f():
            if db == 0:
                sd["r"] = [jnp.broadcast_to(O[i:i + 1], (8, 128)) for O in (O0, O1)]
            a_s[pl.ds(dyn(8 * (16 * i + db), 8), 8), :] = (WVv[i, 0, pl.ds(8 * db, 8), :] * sd["r"][0]
                                                    + WVv[i, 1, pl.ds(8 * db, 8), :] * sd["r"][1])
        return f
    return [step(i, db) for i in range(NV) for db in range(16)]


def stage_GH(O, W, NV, opt, a_s=None):
    NM = H - NV
    WVm, WOm, WVv, WOv = W["WVm"], W["WOm"], W["WVv"], W["WOv"]
    st = {}
    ms = []
    def mG(j, ct):
        def f():
            h = NV + j
            OL = jnp.broadcast_to(O[ct][h:h + 1], (16, 128)).astype(BF16)
            o = _dot(OL, _as_bf16(WVm[j, ct]))[0:8]
            st[("x", j)] = o if ct == 0 else st[("x", j)] + o
            if ct == 3:
                st[("cL", j)] = _pack16(st.pop(("x", j)))
        return f
    def mH(j, mt):
        def f():
            o = _dot(st[("cL", j)], _as_bf16(WOm[j, mt]))[0:8]
            st[("hm", mt)] = o if j == 0 else st[("hm", mt)] + o
        return f
    lag = opt.get("lag", 2)
    if lag == "sweep":
        for ct in range(4): ms += [mG(j, ct) for j in range(NM)]
        for j in range(NM): ms += [mH(j, mt) for mt in range(5)]
    elif opt.get("nsw"):
        n0 = opt["nsw"]
        for ct in range(4): ms += [mG(j, ct) for j in range(n0)]
        hq = list(range(NM)); hi = 0
        for j in range(n0, NM):
            ms += [mG(j, ct) for ct in range(4)]
            if j - n0 >= lag:
                ms += [mH(hq[hi], mt) for mt in range(5)]; hi += 1
        for j in hq[hi:]: ms += [mH(j, mt) for mt in range(5)]
    else:
        for j in range(NM + lag):
            if j < NM: ms += [mG(j, ct) for ct in range(4)]
            if j >= lag: ms += [mH(j - lag, mt) for mt in range(5)]
    if a_s is None:
        first = dict(mult=lambda i: [jnp.broadcast_to(O[ct][i:i + 1], (8, 128)) for ct in range(4)],
                     w=lambda i, k, db: WVv[i, k, pl.ds(8 * db, 8), :])
    else:
        first = dict(mult=lambda i: [jnp.broadcast_to(O[ct][i:i + 1], (8, 128)) for ct in (2, 3)],
                     w=lambda i, k, db: WVv[i, k + 2, pl.ds(8 * db, 8), :],
                     init=lambda i, db: a_s[pl.ds(8 * (16 * i + db), 8), :])
    vs, sv = two_step(NV, 4, first,
        dict(n=5, w=lambda i, k, db: WOv[i, k, pl.ds(8 * db, 8), :], acc=lambda i, k: ("hv", k)), opt, lambda i, s: None)
    _interleave(ms, vs)
    return [st[("hm", mt)] + jnp.sum(sv[("hv", mt)], axis=0, keepdims=True) for mt in range(5)]

def stage_IJ(xc, rstd, W, FT, opt, defer=None):
    FV = FF - 128 * FT
    _tanh = (lambda t: t * t) if opt.get("notanh") else jnp.tanh
    WGm, WUm, WDm, WGv, WUv, WDv = (W[k] for k in ("WGm", "WUm", "WDm", "WGv", "WUv", "WDv"))
    xv = [xc[:, 128 * mt:128 * (mt + 1)] for mt in range(5)]
    XL = [_pack16(v) for v in xv]
    hs = jnp.broadcast_to(0.5 * rstd, (8, 128))
    if defer is not None:
        mu, csm_s, csv_s, LB = defer
        mub = jnp.broadcast_to(mu, (8, 128))
    st = {}
    ms = []
    def mI(ft, which, mt):
        def f():
            Wm = WGm if which == 0 else WUm
            o = _dot(XL[mt], _as_bf16(Wm[ft, mt]))[0:8]
            st[("g", ft, which)] = o if mt == 0 else st[("g", ft, which)] + o
            if which == 1 and mt == 4:
                g, u = st.pop(("g", ft, 0)), st.pop(("g", ft, 1))
                if defer is not None:
                    g = g - mub * csm_s[0, ft]
                    u = u - mub * csm_s[1, ft]
                t = g * hs
                hh = (t * u) * (1.0 + _tanh(t))
                st[("hL", ft)] = _pack16(hh)
        return f
    def mJ(ft, mt):
        def f():
            o = _dot(st[("hL", ft)], _as_bf16(WDm[ft, mt]))[0:8]
            st[("ym", mt)] = o if ft == 0 else st[("ym", mt)] + o
        return f
    lag = opt.get("lag", 1)
    for ft in range(FT + lag):
        if ft < FT: ms += [mI(ft, w, mt) for w in range(2) for mt in range(5)]
        if ft >= lag: ms += [mJ(ft - lag, mt) for mt in range(5)]
    vs = []
    NB = FV // 8
    dstep = opt.get("dstep", 8); doff = opt.get("doff", 16)
    LAG = opt.get("vlag", 8)
    zneed = set(s - doff for s in range(0, NB, dstep) if s >= opt.get("s0", 0))
    def vI(fb, which):
        def f():
            if defer is not None and which == 0 and fb == LB:
                st["xv"] = [v - mub for v in st.get("xv", xv)]
            if which == 0 and fb % dstep == 0:
                key = ("z", fb - doff)
                if key in st:
                    z = st.pop(key)
                    st["xv"] = [v + z for v in st.get("xv", xv)]
                else:
                    st["xv"] = st.get("xv", xv)
            Wv = WGv if which == 0 else WUv
            a = None
            for mt in range(5):
                p = Wv[mt, pl.ds(8 * fb, 8), :] * st["xv"][mt]
                a = p if a is None else a + p
            st[("gb", fb, which)] = jnp.broadcast_to(_xsum(a), (8, 128))
        return f
    def vJ(fb):
        def f():
            g, u = st.pop(("gb", fb, 0)), st.pop(("gb", fb, 1))
            if defer is not None and fb < LB:
                g = g - mub * csv_s[0, pl.ds(8 * fb, 8), :]
                u = u - mub * csv_s[1, pl.ds(8 * fb, 8), :]
            t = g * hs
            hh = (t * u) * (1.0 + _tanh(t))
            for mt in range(5):
                p = WDv[mt, pl.ds(8 * fb, 8), :] * hh
                st[("yv", mt)] = p if fb == 0 else st[("yv", mt)] + p
            if fb in zneed:
                st[("z", fb)] = st[("yv", 4)] * 0.0
        return f
    for fb in range(NB + LAG):
        if fb < NB: vs += [vI(fb, 0), vI(fb, 1)]
        if fb >= LAG: vs.append(vJ(fb - LAG))
    if opt.get("nomxu"):
        _interleave(vs)
        return [jnp.broadcast_to(jnp.sum(st[("yv", mt)], axis=0, keepdims=True), (8, 128)) for mt in range(5)]
    if opt.get("novpu"):
        _interleave(ms)
        return [st[("ym", mt)] for mt in range(5)]
    _interleave(ms, vs)
    return [st[("ym", mt)] + jnp.sum(st[("yv", mt)], axis=0, keepdims=True) for mt in range(5)]


def make_kernel(NV1, NV2, FT, opt, flags=None, tag=''):
    FM = 128 * FT
    FV = FF - FM
    TV = opt.get("tailv", 0)
    if TV:
        nb = opt.get("tailb", 1)
        c1b = opt.get("c1b", 0)
        WD_CH = [(0, FV), (FV, FM - 128 - c1b)] + ([(FF - 128 - c1b, c1b)] if c1b else [])
        NMX = len(WD_CH)
        WD_CH += [(FF - 128 + j * (128 // nb), 128 // nb) for j in range(nb)]
    else:
        WD_CH = [(0, FV), (FV, FM - 256), (FF - 256, 256)]
    LB = opt.get("lb", 0)

    def _kernel(x_hbm, ckv_hbm, wq_hbm, wuk_hbm, wuv_hbm, wo_hbm, wr_hbm, wg_hbm, wu_hbm, wd_hbm,
                o_ref,
                x_s, wr_s, wq_s, wuk_s, ckv_s, wuv_s, wo_s, wg_s, wu_s, wd_s,
                v_s, s_s, qa_s, u_s, csm_s, csv_s, hb_s, qb_s, a_s,
                WQm, WKm, WVm, WOm, WQv, WKv, WVv, WOv, ckvT, ckvN, WGm, WUm, WDm, WGv, WUv, WDv,
                sems):
        cps = {}
        k = 0

        def mk(name, src, dst):
            nonlocal k
            cps[name] = pltpu.make_async_copy(src, dst, sems.at[k])
            k += 1
        mk("x", x_hbm, x_s)
        mk("wr", wr_hbm, wr_s)
        mk("wq", wq_hbm, wq_s)
        mk("wuk", wuk_hbm, wuk_s)
        mk("ckv", ckv_hbm.at[0], ckv_s)
        mk("wuv", wuv_hbm, wuv_s)
        mk("wo", wo_hbm, wo_s)
        mk("wg", wg_hbm, wg_s)
        mk("wu", wu_hbm, wu_s)
        for i, (a, n) in enumerate(WD_CH):
            mk(f"wd{i}", wd_hbm.at[pl.ds(a, n)], wd_s.at[pl.ds(a, n)])
        for c in cps.values():
            c.start()

        def wait(name):
            cps[name].wait()

        wq_u = wq_s.bitcast(U32)
        wuk_u = wuk_s.bitcast(U32)
        wuv_u = wuv_s.bitcast(U32)

        lane = _iota((128, 128), 1)
        row = _iota((128, 128), 0)
        E4 = jnp.where(row % 4 == lane // 32, 1.0, 0.0).astype(BF16)
        A_mask = _iota((32, 128), 1) // 4 == _iota((32, 128), 0)
        ls = _iota((16, 128), 0)
        lj = _iota((16, 128), 1) % 32
        M32 = jnp.where(lj == 2 * ls, jnp.uint32(0x0000FFFF), jnp.where(lj == 2 * ls + 1, jnp.uint32(0xFFFF0000), jnp.uint32(0)))

        def ln_parts(x):
            mean = _xsum(x) * (1.0 / M)
            xc = x - mean
            var = _xsum(xc * xc) * (1.0 / M)
            return xc, lax.rsqrt(var + EPS)

        def dup_bf16(v):
            u = pltpu.bitcast(v.astype(BF16).astype(F32), U32)
            return u | (u >> 16)

        def masked_lhs_matmul(nrows, get_tile):
            acc = None
            G = 8
            for t0 in range(0, nrows, G):
                lhs = []
                rhs = []
                for t in range(t0, t0 + G):
                    vrow = jnp.broadcast_to(v_s[pl.ds(t, 1), :], (16, 128))
                    lhs.append(pltpu.bitcast(vrow & M32, BF16))
                    rhs.append(get_tile(t))
                o = _dot(jnp.concatenate(lhs, axis=1), jnp.concatenate(rhs, axis=0))
                acc = o if acc is None else acc + o
            return acc

        def gather(wu, hp, x0, n):
            return jnp.concatenate([wu[pl.ds((x0 + 8 * r) * 16 + hp, 8, stride=16), :] for r in range(n // 8)], axis=0)

        def gather_b(blk, hp):
            return jnp.concatenate([blk[pl.ds(128 * r + hp, 8, stride=16), :] for r in range(16)], axis=0)

        def prep_heads(wu, nt, Wv, Wm, m_transposed, NV):
            def body(t, c):
                blk = wu.at[pl.ds(pl.multiple_of(t * 2048, 2048), 2048)]
                for hp in range(16):
                    g = gather_b(blk, hp)
                    tt = g.T if (2 * hp < NV or m_transposed) else None
                    for half, f in ((0, _lo), (1, _hi)):
                        h = 2 * hp + half
                        if h < NV:
                            Wv[h, t] = f(tt)
                        else:
                            Wm[h - NV, t] = pltpu.bitcast(f(tt if m_transposed else g).astype(BF16), U32)
                return c + (t >> 10)
            return lax.fori_loop(0, nt, body, 0)

        W = dict(WQm=WQm, WKm=WKm, WVm=WVm, WOm=WOm, WQv=WQv, WKv=WKv, WVv=WVv, WOv=WOv, ckvT=ckvT, ckvN=ckvN,
                 WGm=WGm, WUm=WUm, WDm=WDm, WGv=WGv, WUv=WUv, WDv=WDv)

        zz = [0]

        def dyn(base, mult):
            return pl.multiple_of(zz[0] * mult + base, mult)

        def attn1(x):
            xc, rstd = ln_parts(x)
            xn = xc * rstd
            for kt in range(5):
                xr = jnp.broadcast_to(xn[0:1, 128 * kt:128 * (kt + 1)], (32, 128))
                A = jnp.where(A_mask, xr, 0.0).astype(BF16)
                V = _dot(A, E4)
                v_s[pl.ds(32 * kt, 32), :] = dup_bf16(V)
            wait("wq")
            q = masked_lhs_matmul(160, lambda t: wq_s[pl.ds(128 * t, 128), :])
            qb = q.astype(BF16)
            if not opt.get("noprep"): zz[0] = prep_heads(wq_u, 5, WQv, WQm, False, NV1)
            wait("wuk")
            hsel = (_iota((8, 128), 1) % 32) // 8
            rsel = _iota((8, 128), 1) % 8
            srow = _iota((8, 128), 0)
            vblocks = []
            for b0 in range(0, 128, 8):
                rhs = []
                for b in range(b0, b0 + 8):
                    for cl in range(4):
                        rhs.append(wuk_s[pl.ds(32 * (128 * cl + b), 32), :])
                o = lax.dot_general(qb, jnp.concatenate(rhs, axis=0), NT, preferred_element_type=F32)
                vb = None
                for i in range(8):
                    ob = o[:, 128 * i:128 * (i + 1)]
                    u = jnp.where(hsel == 0, ob[0:8], jnp.where(hsel == 1, ob[8:16], jnp.where(hsel == 2, ob[16:24], ob[24:32])))
                    u = jnp.where(srow == rsel, u, 0.0)
                    r_ = jnp.broadcast_to(jnp.sum(u, axis=0, keepdims=True), (8, 128))
                    vb = r_ if vb is None else jnp.where(srow == i, r_, vb)
                vblocks.append(vb)
            Qt = jnp.concatenate(vblocks, axis=0).T
            qa = jnp.concatenate([Qt[32 * cl:32 * (cl + 1)] for cl in range(4)], axis=1)
            qab = qa.astype(BF16)
            if not opt.get("noprep"): prep_heads(wuk_u, 4, WKv, WKm, True, NV1)
            if opt.get("defer3"):
                for th in stage_BC(jnp.ones((8, M), F32), W, u_s, NV1, opt["BC"], qb_s, dyn):
                    th()
            scale = D ** -0.5
            wait("ckv")
            KC = 512
            mx = None
            for kc in range(SK // KC):
                s = lax.dot_general(qab, ckv_s[pl.ds(kc * KC, KC), :], NT, preferred_element_type=F32) * scale
                s_s[:, pl.ds(kc * KC, KC)] = s
                for j in range(KC // 128):
                    sj = s[:, 128 * j:128 * (j + 1)]
                    mx = sj if mx is None else jnp.maximum(mx, sj)
            mx = jnp.max(mx, axis=1, keepdims=True)
            l = None
            o = None
            for kc in range(SK // KC):
                p = jnp.exp(s_s[:, pl.ds(kc * KC, KC)] - mx)
                for j in range(KC // 128):
                    pj = p[:, 128 * j:128 * (j + 1)]
                    l = pj if l is None else l + pj
                oc = _dot(p.astype(BF16), ckv_s[pl.ds(kc * KC, KC), :])
                o = oc if o is None else o + oc
            l = _xsum(l)
            o = o * (1.0 / l)
            def ckv_body(i, c):
                for j in range(2):
                    kt = 2 * i + j
                    for ct in range(4):
                        t = ckv_s[pl.ds(pl.multiple_of(128 * kt, 128), 128), pl.ds(128 * ct, 128)]
                        ckvT[kt, pl.ds(64 * ct, 64), :] = pltpu.bitcast(t.T, U32)
                        ckvN[kt, ct] = pltpu.bitcast(t, U32)
                return c
            if not opt.get("noprep"): lax.fori_loop(0, 16, ckv_body, 0)
            Obig = jnp.concatenate([o[:, 128 * cl:128 * (cl + 1)] for cl in range(4)], axis=0)
            v_s[pl.ds(0, 128), :] = dup_bf16(Obig.T)
            wait("wuv")
            ctx = masked_lhs_matmul(128, lambda b: jnp.concatenate([wuv_s[pl.ds(32 * (128 * cl + b), 32), :] for cl in range(4)], axis=0))
            ctxb = ctx.astype(BF16)
            if not opt.get("noprep"): prep_heads(wuv_u, 4, WVv, WVm, False, NV2)
            wait("wo")
            r16 = _iota((16, 128), 0)
            acc = None
            for g in range(2):
                cg = ctxb[16 * g:16 * (g + 1)]
                for h0 in range(0, 16, 4):
                    lhs = [jnp.where(r16 == h, cg, jnp.zeros_like(cg)) for h in range(h0, h0 + 4)]
                    rhs = wo_s[pl.ds(128 * (16 * g + h0), 512), :]
                    oo = _dot(jnp.concatenate(lhs, axis=1), rhs)
                    acc = oo if acc is None else acc + oo
            out = jnp.sum(acc, axis=0, keepdims=True)
            xo = x + out

            def wo_v(h, c):
                for mt in range(5):
                    WOv[h, mt] = wo_s[pl.ds(pl.multiple_of(128 * h, 128), 128), pl.ds(128 * mt, 128)].astype(F32)
                return c
            if not opt.get("noprep"): lax.fori_loop(0, NV2, wo_v, 0)

            def wo_m(j, c):
                for mt in range(5):
                    WOm[j, mt] = pltpu.bitcast(wo_s[pl.ds(pl.multiple_of(128 * (j + NV2), 128), 128), pl.ds(128 * mt, 128)], U32)
                return c
            if not opt.get("noprep"): lax.fori_loop(0, H - NV2, wo_m, 0)
            return xo

        def prep_gu(w_s, Wm, Wv):
            if opt.get("noprep"): return
            nb = FV // 32
            for ft in range(FT):
                for mt in range(5):
                    t = w_s[pl.ds(FV + 128 * ft, 128), pl.ds(128 * mt, 128)]
                    Wm[ft, mt] = pltpu.bitcast(t.T, U32)
                for b in range(ft * nb // FT, (ft + 1) * nb // FT):
                    for mt in range(5):
                        Wv[mt, pl.ds(32 * b, 32), :] = w_s[pl.ds(32 * b, 32), pl.ds(128 * mt, 128)].astype(F32)

        def prep_v(w_s, Wv):
            if opt.get("noprep"): return
            def body(i, c):
                for j in range(2):
                    f0 = pl.multiple_of(FV // 2 * i + FV // 4 * j, 16)
                    for mt in range(5):
                        Wv[mt, pl.ds(f0, FV // 4), :] = w_s[pl.ds(f0, FV // 4), pl.ds(128 * mt, 128)].astype(F32)
                return c
            lax.fori_loop(0, 2, body, 0)

        def router(xn):
            wr = wr_s[...].astype(F32).reshape(1, M)
            return jax.nn.sigmoid(_xsum(xn * wr))

        def ffn1(x):
            xc, rstd = ln_parts(x)
            xn = xc * rstd
            rs = router(xn)
            xb = jnp.concatenate([xn, jnp.ones((8, M), F32)], axis=0).astype(BF16)

            def gate_up(w_s, which):
                r = [lax.dot_general(xb, w_s[pl.ds(a, n), :], NT, preferred_element_type=F32) for a, n in ((0, FV), (FV, FM))]
                if opt.get("defer4"):
                    for ft in range(FT):
                        csm_s[which, ft] = r[1][8:16, 128 * ft:128 * (ft + 1)]
                    for j in range((8 * LB + 127) // 128):
                        cs = jnp.broadcast_to(r[0][8:9, 128 * j:128 * (j + 1)], (128, 128))
                        csv_s[which, pl.ds(128 * j, 128), :] = cs.T
                return [v[0:8] for v in r]
            wait("wg")
            g = gate_up(wg_s, 0)
            prep_gu(wg_s, WGm, WGv)
            wait("wu")
            u = gate_up(wu_s, 1)
            hb = []
            for gg, uu in zip(g, u):
                hh = gg * jax.nn.sigmoid(gg) * uu
                hb.append(jnp.broadcast_to(hh[0:1], (16, hh.shape[1])).astype(BF16))
            if TV:
                hb_s[...] = jnp.broadcast_to(hh[0:1, FM - 128:FM], (128, 128)).T
            prep_gu(wu_s, WUm, WUv)
            y = None
            yv = None
            for i, (a, n) in enumerate(WD_CH):
                wait(f"wd{i}")
                if TV and i >= NMX:
                    for r0 in range(a, a + n, 16):
                        hc = hb_s[pl.ds(r0 - (FF - 128), 16), :]
                        part = [wd_s[pl.ds(r0, 16), pl.ds(128 * mt, 128)].astype(F32) * hc for mt in range(5)]
                        yv = part if yv is None else [p + q for p, q in zip(yv, part)]
                    continue
                lhs = hb[0] if i == 0 else hb[1][:, a - FV:a - FV + n]
                yc = _dot(lhs, wd_s[pl.ds(a, n), :])[0:8]
                y = yc if y is None else y + yc
                if i == 0:
                    prep_v(wd_s, WDv)
            if yv is not None:
                y = y + jnp.concatenate([jnp.sum(p, axis=0, keepdims=True) for p in yv], axis=1)
            upd = xn * 0.0 + y * rs
            return x + (xn + upd)

        def stats(x):
            mu = _xsum(x) * (1.0 / M)
            var = jnp.maximum(_xsum(x * x) * (1.0 / M) - mu * mu, 0.0)
            return mu, lax.rsqrt(var + EPS)

        def attn2(x):
            mu, rstd = stats(x)
            late = stage_BC(x, W, qa_s, NV1, opt["BC"], qb_s, dyn)
            for ft in range(FT):
                for mt in range(5):
                    WDm[ft, mt] = pltpu.bitcast(wd_s[pl.ds(FV + 128 * ft, 128), pl.ds(128 * mt, 128)], U32)

            def pin(v):
                qb_s[pl.ds(dyn(NV1 * 128, 8), 8), :] = v
            eg = (lambda O0, O1: early_g_thunks(O0, O1, W, NV2, a_s, dyn)) if opt.get("earlyg") else None
            O = stage_DF(qa_s, rstd[0:1] * (D ** -0.5 * LOG2E), W, s_s, opt["DF"], (u_s, mu[0:1]), late, eg, pin)
            out = stage_GH(O, W, NV2, opt["GH"], a_s if opt.get("earlyg") else None)
            return x + jnp.concatenate(out, axis=1)

        def ffn2(x):
            if opt.get("defer4"):
                mu, rstd = stats(x)
                xn = (x - mu) * rstd
                out = stage_IJ(x, rstd, W, FT, opt["IJ"], (mu, csm_s, csv_s, LB))
            else:
                xc, rstd = ln_parts(x)
                xn = xc * rstd
                out = stage_IJ(xc, rstd, W, FT, opt["IJ"])
            rs = router(xn)
            upd = xn * 0.0 + jnp.concatenate(out, axis=1) * (rs * rstd)
            return x + (xn + upd)

        wait("x")
        wait("wr")
        x = jnp.broadcast_to(x_s[0].astype(F32), (8, M))
        x = attn1(x)
        x = ffn1(x)
        if not opt.get("skip2"):
            x = attn2(x)
            if not opt.get("stop"): x = ffn2(x)
        o_ref[0] = x[0:1].astype(BF16)

    def run(A_x, A_c_kv, A_w_q, A_w_uk, A_w_uv, A_w_o, B_x, B_w_r, B_w_gate, B_w_up, B_w_down):
        anyspec = pl.BlockSpec(memory_space=pl.ANY)
        vm = pl.BlockSpec(memory_space=pltpu.VMEM)
        return pl.pallas_call(
            _kernel,
            out_shape=jax.ShapeDtypeStruct((1, 1, M), BF16),
            in_specs=[anyspec] * 10,
            out_specs=vm,
            scratch_shapes=[
                pltpu.VMEM((1, 1, M), BF16), pltpu.VMEM((M,), BF16),
                pltpu.VMEM((M * H, D), BF16), pltpu.VMEM((DC * H, D), BF16), pltpu.VMEM((SK, DC), BF16),
                pltpu.VMEM((DC * H, D), BF16), pltpu.VMEM((H * D, M), BF16),
                pltpu.VMEM((FF, M), BF16), pltpu.VMEM((FF, M), BF16), pltpu.VMEM((FF, M), BF16),
                pltpu.VMEM((160, 128), U32), pltpu.VMEM((H, SK), F32), pltpu.VMEM((H, DC), F32), pltpu.VMEM((H, DC), F32),
                pltpu.VMEM((2, FT, 8, 128), F32), pltpu.VMEM((2, 256, 128), F32), pltpu.VMEM((128, 128), F32),
                pltpu.VMEM((NV1 * 128 + 8, 128), F32), pltpu.VMEM((NV2 * 128, 128), F32),
                pltpu.VMEM((H - NV1, 5, 64, 128), U32), pltpu.VMEM((H - NV1, 4, 64, 128), U32),
                pltpu.VMEM((H - NV2, 4, 64, 128), U32), pltpu.VMEM((H - NV2, 5, 64, 128), U32),
                pltpu.VMEM((NV1, 5, 128, 128), F32), pltpu.VMEM((NV1, 4, 128, 128), F32),
                pltpu.VMEM((NV2, 4, 128, 128), F32), pltpu.VMEM((NV2, 5, 128, 128), F32),
                pltpu.VMEM((32, 256, 128), U32), pltpu.VMEM((32, 4, 64, 128), U32),
                pltpu.VMEM((FT, 5, 64, 128), U32), pltpu.VMEM((FT, 5, 64, 128), U32), pltpu.VMEM((FT, 5, 64, 128), U32),
                pltpu.VMEM((5, FV, 128), F32), pltpu.VMEM((5, FV, 128), F32), pltpu.VMEM((5, FV, 128), F32),
                pltpu.SemaphoreType.DMA((14,)),
            ],
            compiler_params=pltpu.CompilerParams(vmem_limit_bytes=110 * 1024 * 1024, flags=flags, disable_semaphore_checks=bool(opt.get('nosemchk'))),
            name=f"fused_v7_{NV1}_{NV2}_{FT}{tag}",
        )(A_x, A_c_kv, A_w_q.reshape(M * H, D), A_w_uk.reshape(DC * H, D), A_w_uv.reshape(DC * H, D),
          A_w_o.reshape(H * D, M), B_w_r, B_w_gate.T, B_w_up.T, B_w_down)
    return run


OPT = dict(nosemchk=1, defer3=1, defer4=1, lb=24, tailv=128, tailb=2, c1b=256, earlyg=0,
           BC=dict(lag=3, nsw=5, dstep=8, doff=33, s0=48), DF=dict(nh=16, sweep=1, na=16),
           GH=dict(lag="sweep", dstep=8, doff=29, s0=48), IJ=dict(lag=3, dstep=8, doff=16, vlag=10, s0=24))
_run = make_kernel(16, 15, 8, OPT)


@jax.jit
def pallas_interleave_layers__compressed_kv_cla__moe_arch_mod__decode_kernel(
    A_x, A_c_kv, A_w_q, A_w_uk, A_w_uv, A_w_o, B_x, B_w_r, B_w_gate, B_w_up, B_w_down):
    return _run(A_x, A_c_kv, A_w_q, A_w_uk, A_w_uv, A_w_o, B_x, B_w_r, B_w_gate, B_w_up, B_w_down)
```

```python
import functools
import math
import jax
import jax.numpy as jnp
from jax import lax
import jax.experimental.pallas as pl
import jax.experimental.pallas.tpu as pltpu

F32 = jnp.float32
BF16 = jnp.bfloat16
U32 = jnp.uint32
M = 640
H = 32
D = 128
DC = 512
SK = 4096
FF = 1728
EPS = 1e-5
LOG2E = math.log2(math.e)

NT = (((1,), (1,)), ((), ()))


def _iota(shape, dim):
    return lax.broadcasted_iota(jnp.int32, shape, dim)


def _dot(a, b):
    return jnp.dot(a, b, preferred_element_type=F32)


def _lo(u):
    return pltpu.bitcast(u << 16, F32)


def _hi(u):
    return pltpu.bitcast(u & jnp.uint32(0xFFFF0000), F32)


def _pack16(v):
    return jnp.concatenate([v, v], axis=0).astype(BF16)


def _as_bf16(u):
    return pltpu.bitcast(u, BF16)


def _xsum(v):
    return jnp.sum(v, axis=1, keepdims=True)


def _interleave(*streams):
    items = []
    for si, s in enumerate(streams):
        n = len(s)
        for i, th in enumerate(s):
            items.append(((i + 0.5) / n, si, th))
    items.sort(key=lambda t: (t[0], t[1]))
    for _, _, th in items:
        th()


def _interleave(*streams, phi=1.0):
    items = []
    for si, s in enumerate(streams):
        n = len(s)
        for i, th in enumerate(s):
            items.append(((i + 0.5) / n * (phi if si == 1 else 1.0), si, th))
    items.sort(key=lambda t: (t[0], t[1]))
    for _, _, th in items:
        th()


def ln_parts(x):
    mean = _xsum(x) * (1.0 / M)
    xc = x - mean
    var = _xsum(xc * xc) * (1.0 / M)
    return xc, lax.rsqrt(var + EPS)

def two_step(NV, nmult, first, second, opt, fin):
    st = {}
    dstep = opt.get("dstep", 8); doff = opt.get("doff", 29)
    s0 = opt.get("s0", 0)
    zneed = set(s - doff for s in range(0, NV * 16, dstep) if s >= s0)
    def fA(i, db):
        def f():
            s = i * 16 + db
            if db % dstep == 0:
                if first.get("shared"):
                    base = st.get("m", first["mult"](i))
                else:
                    base = first["mult"](i) if db == 0 else st["m"]
                key = ("z", s - doff)
                if key in st and "pin" in first:
                    first["pin"](st.pop(key))
                    st["m"] = base
                elif key in st:
                    z = st.pop(key)
                    st["m"] = [v + z for v in base]
                else:
                    st["m"] = base
            xx = st["m"]
            a = first["init"](i, db) if "init" in first else None
            for k in range(len(xx)):
                p = first["w"](i, k, db) * xx[k]
                a = p if a is None else a + p
            st[("b", s)] = _xsum(a)
            if "keep" in first:
                first["keep"](s, st[("b", s)])
        return f
    def fB(i, db):
        def f():
            s = i * 16 + db
            b = st.pop(("b", s))
            n = second["n"]
            for k in range(n):
                p = second["w"](i, k, db) * b
                key = second["acc"](i, k)
                st[key] = p if key not in st else st[key] + p
            if s in zneed:
                acc = st[second["acc"](i, n - 1)]
                st[("z", s)] = acc if "pin" in first else acc * 0.0
            if db == 15:
                fin(i, st)
        return f
    vs = []
    for i in range(NV + 1):
        for db in range(16):
            if i < NV: vs.append(fA(i, db))
            if i >= 1: vs.append(fB(i - 1, db))
    return vs, st

def stage_BC(xc, W, qa_s, NV, opt, qb_s=None, dyn=None):
    NM = H - NV
    WQm, WKm, WQv, WKv = W["WQm"], W["WKm"], W["WQv"], W["WKv"]
    xv = [xc[:, 128 * mt:128 * (mt + 1)] for mt in range(5)]
    XL = [_pack16(v) for v in xv]
    st = {}
    ms = []
    def mB(j, mt):
        def f():
            o = _dot(XL[mt], _as_bf16(WQm[j, mt]))[0:8]
            st[("q", j)] = o if mt == 0 else st[("q", j)] + o
            if mt == 4:
                st[("qL", j)] = _pack16(st.pop(("q", j)))
        return f
    def mC(j, ct):
        def f():
            o = _dot(st[("qL", j)], _as_bf16(WKm[j, ct]))
            qa_s[pl.ds(NV + j, 1), pl.ds(128 * ct, 128)] = o[0:1]
        return f
    lag = opt.get("lag", 2)
    if lag == "sweep":
        for j in range(NM): ms += [mB(j, mt) for mt in range(5)]
        for ct in range(4): ms += [mC(j, ct) for j in range(NM)]
    elif opt.get("nsw"):
        n0 = NM - opt["nsw"]
        for j in range(NM):
            ms += [mB(j, mt) for mt in range(5)]
            if j >= lag and j - lag < n0: ms += [mC(j - lag, ct) for ct in range(4)]
        for j in range(max(NM - lag, 0), n0): ms += [mC(j, ct) for ct in range(4)]
        for ct in range(4): ms += [mC(j, ct) for j in range(n0, NM)]
    else:
        for j in range(NM + lag):
            if j < NM: ms += [mB(j, mt) for mt in range(5)]
            if j >= lag: ms += [mC(j - lag, ct) for ct in range(4)]
    if NV == 0:
        _interleave(ms); return
    NC = 2 if opt.get("split") else 4

    def fin(i, s):
        for ct in range(NC):
            qa_s[pl.ds(i, 1), pl.ds(128 * ct, 128)] = jnp.sum(s.pop(("c", i, ct)), axis=0, keepdims=True)
    first = dict(shared=1, mult=lambda i: xv, w=lambda i, k, db: WQv[i, k, pl.ds(8 * db, 8), :])
    if opt.get("pin") and dyn is not None:
        def pinq(v):
            WQv[NV + dyn(0, 1), 0, pl.ds(0, 8), :] = v
        first["pin"] = pinq
    if NC < 4:
        def keep(s, b):
            qb_s[pl.ds(dyn(8 * s, 8), 8), :] = jnp.broadcast_to(b, (8, 128))
        first["keep"] = keep
    vs, _ = two_step(NV, 5, first,
        dict(n=NC, w=lambda i, k, db: WKv[i, k, pl.ds(8 * db, 8), :], acc=lambda i, k: ("c", i, k)), opt, fin)
    _interleave(ms, vs, phi=opt.get("phi", 1.0))
    if NC == 4:
        return []
    sd = {}

    def late(i, db):
        def f():
            qb = qb_s[pl.ds(8 * (16 * i + db), 8), :]
            for ct in range(NC, 4):
                p = WKv[i, ct, pl.ds(8 * db, 8), :] * qb
                sd[ct] = p if db == 0 else sd[ct] + p
            if db == 15:
                for ct in range(NC, 4):
                    qa_s[pl.ds(i, 1), pl.ds(128 * ct, 128)] = jnp.sum(sd[ct], axis=0, keepdims=True)
        return f
    return [late(i, db) for i in range(NV) for db in range(16)]

def stage_DF(qa_s, scale, W, s_s, opt, corr=None, late=(), early_g=None, pin=None, shadow=()):
    ckvT, ckvN = W["ckvT"], W["ckvN"]
    u_s, mu = corr
    ms_ = mu * scale

    def QLf(ct):
        return (qa_s[:, pl.ds(128 * ct, 128)] * scale - u_s[:, pl.ds(128 * ct, 128)] * ms_).astype(BF16)
    NH = opt.get("nh", 16)

    def Dt(q, kt, ct):
        return _dot(q, _as_bf16(ckvT[kt, pl.ds(64 * ct, 64), :]))
    mx = [None, None]
    shadow = list(shadow)
    sh_n = opt.get("shn", 48)
    sh_i = [0]

    def tick():
        k = sh_i[0]
        sh_i[0] += 1
        if k < sh_n:
            for th in shadow[k * len(shadow) // sh_n:(k + 1) * len(shadow) // sh_n]:
                th()
    if late:
        QL = [QLf(0), QLf(1)]

        def dA(kt):
            def f():
                sa = Dt(QL[0], kt, 0) + Dt(QL[1], kt, 1)
                s_s[:, pl.ds(128 * kt, 128)] = sa
                if kt % opt.get("pin", 1) == 0:
                    pin(sa[0:8])
            return f
        _interleave([dA(kt) for kt in range(32)], list(late), phi=opt.get("phid", 0.8))
        QL += [QLf(2), QLf(3)]
        for kt in range(32):
            sc = s_s[:, pl.ds(128 * kt, 128)] + Dt(QL[2], kt, 2) + Dt(QL[3], kt, 3)
            s_s[:, pl.ds(128 * kt, 128)] = sc
            hf = int(kt >= NH)
            mx[hf] = sc if mx[hf] is None else jnp.maximum(mx[hf], sc)
            tick()
    else:
        QL = [QLf(ct) for ct in range(4)]
        NA = opt.get("na", 0)
        for kt in range(NA):
            s_s[:, pl.ds(128 * kt, 128)] = Dt(QL[0], kt, 0)
        for kt in range(32):
            if kt < NA:
                sc = s_s[:, pl.ds(128 * kt, 128)]
                for ct in range(1, 4): sc = sc + Dt(QL[ct], kt, ct)
            else:
                sc = Dt(QL[0], kt, 0)
                for ct in range(1, 4): sc = sc + Dt(QL[ct], kt, ct)
            s_s[:, pl.ds(128 * kt, 128)] = sc
            hf = int(kt >= NH)
            mx[hf] = sc if mx[hf] is None else jnp.maximum(mx[hf], sc)
            tick()
    m0 = jnp.max(mx[0], axis=1, keepdims=True)
    m1 = jnp.maximum(m0, jnp.max(mx[1], axis=1, keepdims=True))
    alpha = jnp.exp2(m0 - m1)
    l = None; O = [None] * 4

    def Ft(pb, kt, ct):
        o = _dot(pb, _as_bf16(ckvN[kt, ct]))
        O[ct] = o if O[ct] is None else O[ct] + o
    P = {}

    def mkP(kt, m):
        nonlocal l
        p = jnp.exp2(s_s[:, pl.ds(128 * kt, 128)] - m)
        l = p if l is None else l + p
        P[kt] = p.astype(BF16)
    if early_g is None:
        for kt in range(NH):
            mkP(kt, m0)
            for ct in range(4): Ft(P[kt], kt, ct)
            tick()
        l = l * alpha
        if opt.get("sweep", 1):
            for ct in range(4):
                O[ct] = O[ct] * alpha
                for kt in range(NH, 32):
                    if ct == 0: mkP(kt, m1)
                    Ft(P[kt], kt, ct)
                    if kt % 4 == 3: tick()
        else:
            for ct in range(4):
                O[ct] = O[ct] * alpha
            for kt in range(NH, 32):
                mkP(kt, m1)
                for ct in range(4): Ft(P[kt], kt, ct)
                tick()
        assert sh_i[0] >= sh_n or not shadow
        ls = _xsum(l)
        r0 = pl.reciprocal(ls, approx=True)
        inv = r0 * (2.0 - ls * r0)
        return [o * inv for o in O]
    for kt in range(NH):
        mkP(kt, m0)
        for ct in (0, 1): Ft(P[kt], kt, ct)
    l = l * alpha
    for ct in (0, 1): O[ct] = O[ct] * alpha
    for kt in range(NH, 32):
        mkP(kt, m1)
        for ct in (0, 1): Ft(P[kt], kt, ct)
    ls = _xsum(l)
    r0 = pl.reciprocal(ls, approx=True)
    inv = r0 * (2.0 - ls * r0)
    O[0] = O[0] * inv
    O[1] = O[1] * inv

    def f2(kt):
        def f():
            if kt == NH:
                for ct in (2, 3): O[ct] = O[ct] * alpha
            for ct in (2, 3): Ft(P[kt], kt, ct)
        return f
    _interleave([f2(kt) for kt in range(32)], early_g(O[0], O[1]), phi=opt.get("phif", 0.9))
    O[2] = O[2] * inv
    O[3] = O[3] * inv
    return O


def early_g_thunks(O0, O1, W, NV, a_s, dyn):
    WVv = W["WVv"]
    sd = {}

    def step(i, db):
        def f():
            if db == 0:
                sd["r"] = [jnp.broadcast_to(O[i:i + 1], (8, 128)) for O in (O0, O1)]
            a_s[pl.ds(dyn(8 * (16 * i + db), 8), 8), :] = (WVv[i, 0, pl.ds(8 * db, 8), :] * sd["r"][0]
                                                    + WVv[i, 1, pl.ds(8 * db, 8), :] * sd["r"][1])
        return f
    return [step(i, db) for i in range(NV) for db in range(16)]


def stage_GH(O, W, NV, opt, a_s=None, dyn=None):
    NM = H - NV
    WVm, WOm, WVv, WOv = W["WVm"], W["WOm"], W["WVv"], W["WOv"]
    st = {}
    ms = []
    def mG(j, ct):
        def f():
            h = NV + j
            OL = jnp.broadcast_to(O[ct][h:h + 1], (16, 128)).astype(BF16)
            o = _dot(OL, _as_bf16(WVm[j, ct]))[0:8]
            st[("x", j)] = o if ct == 0 else st[("x", j)] + o
            if ct == 3:
                st[("cL", j)] = _pack16(st.pop(("x", j)))
        return f
    def mH(j, mt):
        def f():
            o = _dot(st[("cL", j)], _as_bf16(WOm[j, mt]))[0:8]
            st[("hm", mt)] = o if j == 0 else st[("hm", mt)] + o
        return f
    lag = opt.get("lag", 2)
    if lag == "sweep":
        for ct in range(4): ms += [mG(j, ct) for j in range(NM)]
        for j in range(NM): ms += [mH(j, mt) for mt in range(5)]
    elif opt.get("nsw"):
        n0 = opt["nsw"]
        for ct in range(4): ms += [mG(j, ct) for j in range(n0)]
        hq = list(range(NM)); hi = 0
        for j in range(n0, NM):
            ms += [mG(j, ct) for ct in range(4)]
            if j - n0 >= lag:
                ms += [mH(hq[hi], mt) for mt in range(5)]; hi += 1
        for j in hq[hi:]: ms += [mH(j, mt) for mt in range(5)]
    else:
        for j in range(NM + lag):
            if j < NM: ms += [mG(j, ct) for ct in range(4)]
            if j >= lag: ms += [mH(j - lag, mt) for mt in range(5)]
    if a_s is None:
        first = dict(mult=lambda i: [jnp.broadcast_to(O[ct][i:i + 1], (8, 128)) for ct in range(4)],
                     w=lambda i, k, db: WVv[i, k, pl.ds(8 * db, 8), :])
    else:
        first = dict(mult=lambda i: [jnp.broadcast_to(O[ct][i:i + 1], (8, 128)) for ct in (2, 3)],
                     w=lambda i, k, db: WVv[i, k + 2, pl.ds(8 * db, 8), :],
                     init=lambda i, db: a_s[pl.ds(8 * (16 * i + db), 8), :])
    if opt.get("pin") and dyn is not None:
        def pinv(v):
            WVv[NV + dyn(0, 1), 0, pl.ds(0, 8), :] = v
        first["pin"] = pinv
    vs, sv = two_step(NV, 4, first,
        dict(n=5, w=lambda i, k, db: WOv[i, k, pl.ds(8 * db, 8), :], acc=lambda i, k: ("hv", k)), opt, lambda i, s: None)
    _interleave(ms, vs, phi=opt.get("phi", 1.0))
    return [st[("hm", mt)] + jnp.sum(sv[("hv", mt)], axis=0, keepdims=True) for mt in range(5)]

def stage_IJ(xc, rstd, W, FT, opt, defer=None, dyn=None):
    FV = FF - 128 * FT
    _tanh = (lambda t: t * t) if opt.get("notanh") else jnp.tanh
    WGm, WUm, WDm, WGv, WUv, WDv = (W[k] for k in ("WGm", "WUm", "WDm", "WGv", "WUv", "WDv"))
    xv = [xc[:, 128 * mt:128 * (mt + 1)] for mt in range(5)]
    XL = [_pack16(v) for v in xv]
    hs = jnp.broadcast_to(0.5 * rstd, (8, 128))
    if defer is not None:
        mu, csm_s, csv_s, LB = defer
        mub = jnp.broadcast_to(mu, (8, 128))
    st = {}
    ms = []
    def mI(ft, which, mt):
        def f():
            Wm = WGm if which == 0 else WUm
            o = _dot(XL[mt], _as_bf16(Wm[ft, mt]))[0:8]
            st[("g", ft, which)] = o if mt == 0 else st[("g", ft, which)] + o
            if which == 1 and mt == 4:
                g, u = st.pop(("g", ft, 0)), st.pop(("g", ft, 1))
                if defer is not None:
                    g = g - mub * csm_s[0, ft]
                    u = u - mub * csm_s[1, ft]
                t = g * hs
                hh = (t * u) * (1.0 + _tanh(t))
                st[("hL", ft)] = _pack16(hh)
        return f
    def mJ(ft, mt):
        def f():
            o = _dot(st[("hL", ft)], _as_bf16(WDm[ft, mt]))[0:8]
            st[("ym", mt)] = o if ft == 0 else st[("ym", mt)] + o
        return f
    lag = opt.get("lag", 1)
    for ft in range(FT + lag):
        if ft < FT: ms += [mI(ft, w, mt) for w in range(2) for mt in range(5)]
        if ft >= lag: ms += [mJ(ft - lag, mt) for mt in range(5)]
    vs = []
    NB = FV // 8
    dstep = opt.get("dstep", 8); doff = opt.get("doff", 16)
    LAG = opt.get("vlag", 8)
    zneed = set(s - doff for s in range(0, NB, dstep) if s >= opt.get("s0", 0))
    def vI(fb, which):
        def f():
            if defer is not None and which == 0 and fb == LB:
                st["xv"] = [v - mub for v in st.get("xv", xv)]
            if which == 0 and fb % dstep == 0:
                key = ("z", fb - doff)
                if key in st and opt.get("pin"):
                    z = st.pop(key)
                    WGv[0, pl.ds(dyn(FV, 8), 8), :] = z
                    WUv[0, pl.ds(dyn(FV, 8), 8), :] = z
                    st["xv"] = st.get("xv", xv)
                elif key in st:
                    z = st.pop(key)
                    st["xv"] = [v + z for v in st.get("xv", xv)]
                else:
                    st["xv"] = st.get("xv", xv)
            Wv = WGv if which == 0 else WUv
            a = None
            for mt in range(5):
                p = Wv[mt, pl.ds(8 * fb, 8), :] * st["xv"][mt]
                a = p if a is None else a + p
            st[("gb", fb, which)] = jnp.broadcast_to(_xsum(a), (8, 128))
        return f
    def vJ(fb):
        def f():
            g, u = st.pop(("gb", fb, 0)), st.pop(("gb", fb, 1))
            if defer is not None and fb < LB:
                g = g - mub * csv_s[0, pl.ds(8 * fb, 8), :]
                u = u - mub * csv_s[1, pl.ds(8 * fb, 8), :]
            t = g * hs
            hh = (t * u) * (1.0 + _tanh(t))
            for mt in range(5):
                p = WDv[mt, pl.ds(8 * fb, 8), :] * hh
                st[("yv", mt)] = p if fb == 0 else st[("yv", mt)] + p
            if fb in zneed:
                st[("z", fb)] = st[("yv", 4)] if opt.get("pin") else st[("yv", 4)] * 0.0
        return f
    for fb in range(NB + LAG):
        if fb < NB: vs += [vI(fb, 0), vI(fb, 1)]
        if fb >= LAG: vs.append(vJ(fb - LAG))
    if opt.get("nomxu"):
        _interleave(vs)
        return [jnp.broadcast_to(jnp.sum(st[("yv", mt)], axis=0, keepdims=True), (8, 128)) for mt in range(5)]
    if opt.get("novpu"):
        _interleave(ms)
        return [st[("ym", mt)] for mt in range(5)]
    _interleave(ms, vs, phi=opt.get("phi", 1.0))
    return [st[("ym", mt)] + jnp.sum(st[("yv", mt)], axis=0, keepdims=True) for mt in range(5)]


def make_kernel(NV1, NV2, FT, opt, flags=None, tag=''):
    FM = 128 * FT
    FV = FF - FM
    TV = opt.get("tailv", 0)
    if TV:
        nb = opt.get("tailb", 1)
        c1b = opt.get("c1b", 0)
        WD_CH = [(0, FV), (FV, FM - 128 - c1b)] + ([(FF - 128 - c1b, c1b)] if c1b else [])
        NMX = len(WD_CH)
        WD_CH += [(FF - 128 + j * (128 // nb), 128 // nb) for j in range(nb)]
    else:
        WD_CH = [(0, FV), (FV, FM - 256), (FF - 256, 256)]
    LB = opt.get("lb", 0)

    def _kernel(x_hbm, ckv_hbm, wq_hbm, wuk_hbm, wuv_hbm, wo_hbm, wr_hbm, wg_hbm, wu_hbm, wd_hbm,
                o_ref,
                x_s, wr_s, wq_s, wuk_s, ckv_s, wuv_s, wo_s, wg_s, wu_s, wd_s,
                v_s, s_s, qa_s, u_s, csm_s, csv_s, hb_s, qb_s, a_s,
                WQm, WKm, WVm, WOm, WQv, WKv, WVv, WOv, ckvT, ckvN, WGm, WUm, WDm, WGv, WUv, WDv,
                sems):
        cps = {}
        k = 0

        def mk(name, src, dst):
            nonlocal k
            cps[name] = pltpu.make_async_copy(src, dst, sems.at[k])
            k += 1
        mk("x", x_hbm, x_s)
        mk("wr", wr_hbm, wr_s)
        mk("wq", wq_hbm, wq_s)
        mk("wuk", wuk_hbm, wuk_s)
        mk("ckv", ckv_hbm.at[0], ckv_s)
        mk("wuv", wuv_hbm, wuv_s)
        mk("wo", wo_hbm, wo_s)
        mk("wg", wg_hbm, wg_s)
        mk("wu", wu_hbm, wu_s)
        for i, (a, n) in enumerate(WD_CH):
            mk(f"wd{i}", wd_hbm.at[pl.ds(a, n)], wd_s.at[pl.ds(a, n)])
        order = list(cps)
        if opt.get("order") == 1:
            order = ["wq", "x"] + [n for n in order if n not in ("wq", "x")]
        elif opt.get("order") == 2:
            order = ["wq", "x", "wuk", "ckv", "wuv", "wo", "wr"] + [n for n in order if n not in ("wq", "x", "wuk", "ckv", "wuv", "wo", "wr")]
        elif opt.get("order") == 3:
            order = ["x", "wq", "wuk", "ckv", "wuv", "wo", "wr"] + [n for n in order if n not in ("wq", "x", "wuk", "ckv", "wuv", "wo", "wr")]
        for n in order:
            cps[n].start()

        def wait(name):
            cps[name].wait()

        wq_u = wq_s.bitcast(U32)
        wuk_u = wuk_s.bitcast(U32)
        wuv_u = wuv_s.bitcast(U32)

        lane = _iota((128, 128), 1)
        row = _iota((128, 128), 0)
        E4 = jnp.where(row % 4 == lane // 32, 1.0, 0.0).astype(BF16)
        A_mask = _iota((32, 128), 1) // 4 == _iota((32, 128), 0)
        ls = _iota((16, 128), 0)
        lj = _iota((16, 128), 1) % 32
        M32 = jnp.where(lj == 2 * ls, jnp.uint32(0x0000FFFF), jnp.where(lj == 2 * ls + 1, jnp.uint32(0xFFFF0000), jnp.uint32(0)))

        def ln_parts(x):
            mean = _xsum(x) * (1.0 / M)
            xc = x - mean
            var = _xsum(xc * xc) * (1.0 / M)
            return xc, lax.rsqrt(var + EPS)

        def dup_bf16(v):
            u = pltpu.bitcast(v.astype(BF16).astype(F32), U32)
            return u | (u >> 16)

        def masked_lhs_matmul(nrows, get_tile):
            acc = None
            G = 8
            for t0 in range(0, nrows, G):
                lhs = []
                rhs = []
                for t in range(t0, t0 + G):
                    vrow = jnp.broadcast_to(v_s[pl.ds(t, 1), :], (16, 128))
                    lhs.append(pltpu.bitcast(vrow & M32, BF16))
                    rhs.append(get_tile(t))
                o = _dot(jnp.concatenate(lhs, axis=1), jnp.concatenate(rhs, axis=0))
                acc = o if acc is None else acc + o
            return acc

        def gather(wu, hp, x0, n):
            return jnp.concatenate([wu[pl.ds((x0 + 8 * r) * 16 + hp, 8, stride=16), :] for r in range(n // 8)], axis=0)

        def gather_b(blk, hp):
            return jnp.concatenate([blk[pl.ds(128 * r + hp, 8, stride=16), :] for r in range(16)], axis=0)

        def prep_heads(wu, nt, Wv, Wm, m_transposed, NV):
            def body(t, c):
                blk = wu.at[pl.ds(pl.multiple_of(t * 2048, 2048), 2048)]
                for hp in range(16):
                    g = gather_b(blk, hp)
                    tt = g.T if (2 * hp < NV or m_transposed) else None
                    for half, f in ((0, _lo), (1, _hi)):
                        h = 2 * hp + half
                        if h < NV:
                            Wv[h, t] = f(tt)
                        else:
                            Wm[h - NV, t] = pltpu.bitcast(f(tt if m_transposed else g).astype(BF16), U32)
                return c + (t >> 10)
            return lax.fori_loop(0, nt, body, 0)

        W = dict(WQm=WQm, WKm=WKm, WVm=WVm, WOm=WOm, WQv=WQv, WKv=WKv, WVv=WVv, WOv=WOv, ckvT=ckvT, ckvN=ckvN,
                 WGm=WGm, WUm=WUm, WDm=WDm, WGv=WGv, WUv=WUv, WDv=WDv)

        zz = [0]

        def dyn(base, mult):
            return pl.multiple_of(zz[0] * mult + base, mult)

        def attn1(x):
            xc, rstd = ln_parts(x)
            xn = xc * rstd
            for kt in range(5):
                xr = jnp.broadcast_to(xn[0:1, 128 * kt:128 * (kt + 1)], (32, 128))
                A = jnp.where(A_mask, xr, 0.0).astype(BF16)
                V = _dot(A, E4)
                v_s[pl.ds(32 * kt, 32), :] = dup_bf16(V)
            wait("wq")
            q = masked_lhs_matmul(160, lambda t: wq_s[pl.ds(128 * t, 128), :])
            qb = q.astype(BF16)
            if not opt.get("noprep"): zz[0] = prep_heads(wq_u, 5, WQv, WQm, False, NV1)
            wait("wuk")
            hsel = (_iota((8, 128), 1) % 32) // 8
            rsel = _iota((8, 128), 1) % 8
            srow = _iota((8, 128), 0)
            vblocks = []
            for b0 in range(0, 128, 8):
                rhs = []
                for b in range(b0, b0 + 8):
                    for cl in range(4):
                        rhs.append(wuk_s[pl.ds(32 * (128 * cl + b), 32), :])
                o = lax.dot_general(qb, jnp.concatenate(rhs, axis=0), NT, preferred_element_type=F32)
                vb = None
                for i in range(8):
                    ob = o[:, 128 * i:128 * (i + 1)]
                    u = jnp.where(hsel == 0, ob[0:8], jnp.where(hsel == 1, ob[8:16], jnp.where(hsel == 2, ob[16:24], ob[24:32])))
                    u = jnp.where(srow == rsel, u, 0.0)
                    r_ = jnp.broadcast_to(jnp.sum(u, axis=0, keepdims=True), (8, 128))
                    vb = r_ if vb is None else jnp.where(srow == i, r_, vb)
                vblocks.append(vb)
            Qt = jnp.concatenate(vblocks, axis=0).T
            qa = jnp.concatenate([Qt[32 * cl:32 * (cl + 1)] for cl in range(4)], axis=1)
            qab = qa.astype(BF16)
            if not opt.get("noprep"): prep_heads(wuk_u, 4, WKv, WKm, True, NV1)
            if opt.get("defer3"):
                for th in stage_BC(jnp.ones((8, M), F32), W, u_s, NV1, opt["BC"], qb_s, dyn):
                    th()
            scale = D ** -0.5
            wait("ckv")
            KC = 512
            mx = None
            for kc in range(SK // KC):
                s = lax.dot_general(qab, ckv_s[pl.ds(kc * KC, KC), :], NT, preferred_element_type=F32) * scale
                s_s[:, pl.ds(kc * KC, KC)] = s
                for j in range(KC // 128):
                    sj = s[:, 128 * j:128 * (j + 1)]
                    mx = sj if mx is None else jnp.maximum(mx, sj)
            mx = jnp.max(mx, axis=1, keepdims=True)
            l = None
            o = None
            for kc in range(SK // KC):
                p = jnp.exp(s_s[:, pl.ds(kc * KC, KC)] - mx)
                for j in range(KC // 128):
                    pj = p[:, 128 * j:128 * (j + 1)]
                    l = pj if l is None else l + pj
                oc = _dot(p.astype(BF16), ckv_s[pl.ds(kc * KC, KC), :])
                o = oc if o is None else o + oc
            l = _xsum(l)
            o = o * (1.0 / l)
            def ckv_body(i, c):
                for j in range(2):
                    kt = 2 * i + j
                    for ct in range(4):
                        t = ckv_s[pl.ds(pl.multiple_of(128 * kt, 128), 128), pl.ds(128 * ct, 128)]
                        ckvT[kt, pl.ds(64 * ct, 64), :] = pltpu.bitcast(t.T, U32)
                        ckvN[kt, ct] = pltpu.bitcast(t, U32)
                return c
            if not opt.get("noprep"): lax.fori_loop(0, 16, ckv_body, 0)
            Obig = jnp.concatenate([o[:, 128 * cl:128 * (cl + 1)] for cl in range(4)], axis=0)
            v_s[pl.ds(0, 128), :] = dup_bf16(Obig.T)
            wait("wuv")
            ctx = masked_lhs_matmul(128, lambda b: jnp.concatenate([wuv_s[pl.ds(32 * (128 * cl + b), 32), :] for cl in range(4)], axis=0))
            ctxb = ctx.astype(BF16)
            if not opt.get("noprep"): prep_heads(wuv_u, 4, WVv, WVm, False, NV2)
            wait("wo")
            r16 = _iota((16, 128), 0)
            acc = None
            for g in range(2):
                cg = ctxb[16 * g:16 * (g + 1)]
                for h0 in range(0, 16, 4):
                    lhs = [jnp.where(r16 == h, cg, jnp.zeros_like(cg)) for h in range(h0, h0 + 4)]
                    rhs = wo_s[pl.ds(128 * (16 * g + h0), 512), :]
                    oo = _dot(jnp.concatenate(lhs, axis=1), rhs)
                    acc = oo if acc is None else acc + oo
            out = jnp.sum(acc, axis=0, keepdims=True)
            xo = x + out

            def wo_v(h, c):
                for mt in range(5):
                    WOv[h, mt] = wo_s[pl.ds(pl.multiple_of(128 * h, 128), 128), pl.ds(128 * mt, 128)].astype(F32)
                return c
            if not opt.get("noprep"): lax.fori_loop(0, NV2, wo_v, 0)

            def wo_m(j, c):
                for mt in range(5):
                    WOm[j, mt] = pltpu.bitcast(wo_s[pl.ds(pl.multiple_of(128 * (j + NV2), 128), 128), pl.ds(128 * mt, 128)], U32)
                return c
            if not opt.get("noprep"): lax.fori_loop(0, H - NV2, wo_m, 0)
            return xo

        def prep_gu(w_s, Wm, Wv, do_v=True):
            if opt.get("noprep") or opt.get("noprep_gu"): return
            nb = FV // 32
            for ft in range(FT):
                for mt in range(5):
                    t = w_s[pl.ds(FV + 128 * ft, 128), pl.ds(128 * mt, 128)]
                    Wm[ft, mt] = pltpu.bitcast(t.T, U32)
                for b in (range(ft * nb // FT, (ft + 1) * nb // FT) if do_v else ()):
                    for mt in range(5):
                        Wv[mt, pl.ds(32 * b, 32), :] = w_s[pl.ds(32 * b, 32), pl.ds(128 * mt, 128)].astype(F32)

        def prep_v(w_s, Wv):
            if opt.get("noprep") or opt.get("noprep_v"): return
            def body(i, c):
                for j in range(2):
                    f0 = pl.multiple_of(FV // 2 * i + FV // 4 * j, 16)
                    for mt in range(5):
                        Wv[mt, pl.ds(f0, FV // 4), :] = w_s[pl.ds(f0, FV // 4), pl.ds(128 * mt, 128)].astype(F32)
                return c
            lax.fori_loop(0, 2, body, 0)

        def router(xn):
            wr = wr_s[...].astype(F32).reshape(1, M)
            return jax.nn.sigmoid(_xsum(xn * wr))

        def ffn1(x):
            xc, rstd = ln_parts(x)
            xn = xc * rstd
            wait("wr")
            rs = router(xn)
            xb = jnp.concatenate([xn, jnp.ones((8, M), F32)], axis=0).astype(BF16)

            def gate_up(w_s, which):
                r = [lax.dot_general(xb, w_s[pl.ds(a, n), :], NT, preferred_element_type=F32) for a, n in ((0, FV), (FV, FM))]
                if opt.get("defer4"):
                    for ft in range(FT):
                        csm_s[which, ft] = r[1][8:16, 128 * ft:128 * (ft + 1)]
                    for j in range((8 * LB + 127) // 128):
                        cs = jnp.broadcast_to(r[0][8:9, 128 * j:128 * (j + 1)], (128, 128))
                        csv_s[which, pl.ds(128 * j, 128), :] = cs.T
                return [v[0:8] for v in r]
            wait("wg")
            g = gate_up(wg_s, 0)
            prep_gu(wg_s, WGm, WGv, 'g' not in opt.get('shadow', ''))
            wait("wu")
            u = gate_up(wu_s, 1)
            hb = []
            for gg, uu in zip(g, u):
                hh = gg * jax.nn.sigmoid(gg) * uu
                hb.append(jnp.broadcast_to(hh[0:1], (16, hh.shape[1])).astype(BF16))
            if TV:
                hb_s[...] = jnp.broadcast_to(hh[0:1, FM - 128:FM], (128, 128)).T
            prep_gu(wu_s, WUm, WUv, 'u' not in opt.get('shadow', ''))
            y = None
            yv = None

            def keep_tile(ft, t_of_mt):
                for mt in range(5):
                    WDm[ft, mt] = pltpu.bitcast(t_of_mt[mt], U32)
            for i, (a, n) in enumerate(WD_CH):
                if TV and i == NMX and opt.get("wdm1") and not opt.get("nofence"):
                    def fence(j, c):
                        v_s[pl.ds(pl.multiple_of(8 * j, 8), 8), :] = jnp.zeros((8, 128), U32)
                        return c
                    lax.fori_loop(0, 2, fence, 0)
                wait(f"wd{i}")
                if TV and i >= NMX:
                    for r0 in range(a, a + n, 16):
                        hc = hb_s[pl.ds(r0 - (FF - 128), 16), :]
                        raw = [wd_s[pl.ds(r0, 16), pl.ds(128 * mt, 128)] for mt in range(5)]
                        part = [t.astype(F32) * hc for t in raw]
                        yv = part if yv is None else [p + q for p, q in zip(yv, part)]
                        if opt.get("wdm1"):
                            for mt in range(5):
                                WDm[FT - 1, mt, pl.ds((r0 - (FF - 128)) // 2, 8), :] = pltpu.bitcast(raw[mt], U32)
                    continue
                if i == 0 or not opt.get("wdm1"):
                    lhs = hb[0] if i == 0 else hb[1][:, a - FV:a - FV + n]
                    yc = _dot(lhs, wd_s[pl.ds(a, n), :])[0:8]
                else:
                    ycs = None
                    for ft in range((a - FV) // 128, (a - FV + n) // 128):
                        raw = [wd_s[pl.ds(FV + 128 * ft, 128), pl.ds(128 * mt, 128)] for mt in range(5)]
                        keep_tile(ft, raw)
                        o = [_dot(hb[1][:, 128 * ft:128 * (ft + 1)], raw[mt])[0:8] for mt in range(5)]
                        ycs = o if ycs is None else [p + q for p, q in zip(ycs, o)]
                    yc = jnp.concatenate(ycs, axis=1)
                y = yc if y is None else y + yc
                if i == 0:
                    if opt.get("wdm1") and not opt.get("vloop"):
                        for r0 in range(0, FV, 32):
                            for mt in range(5):
                                WDv[mt, pl.ds(r0, 32), :] = wd_s[pl.ds(r0, 32), pl.ds(128 * mt, 128)].astype(F32)
                    elif 'd' not in opt.get('shadow', ''):
                        prep_v(wd_s, WDv)
            if yv is not None:
                y = y + jnp.concatenate([jnp.sum(p, axis=0, keepdims=True) for p in yv], axis=1)
            upd = xn * 0.0 + y * rs
            return x + (xn + upd)

        def stats(x):
            mu = _xsum(x) * (1.0 / M)
            var = jnp.maximum(_xsum(x * x) * (1.0 / M) - mu * mu, 0.0)
            return mu, lax.rsqrt(var + EPS)

        def attn2(x):
            mu, rstd = stats(x)
            late = stage_BC(x, W, qa_s, NV1, opt["BC"], qb_s, dyn)
            for ft in range(FT if not opt.get("wdm1") else 0):
                for mt in range(5):
                    WDm[ft, mt] = pltpu.bitcast(wd_s[pl.ds(FV + 128 * ft, 128), pl.ds(128 * mt, 128)], U32)

            def pin(v):
                qb_s[pl.ds(dyn(NV1 * 128, 8), 8), :] = v
            shadow = []

            def vprep(w_s, Wv, r0, nr):
                def f():
                    for mt in range(5):
                        Wv[mt, pl.ds(dyn(r0, 16), nr), :] = w_s[pl.ds(r0, nr), pl.ds(128 * mt, 128)].astype(F32)
                return f
            for nm, w_s, Wv in (("g", wg_s, WGv), ("u", wu_s, WUv), ("d", wd_s, WDv)):
                if nm in opt.get("shadow", ""):
                    shadow += [vprep(w_s, Wv, r0, 16) for r0 in range(0, FV, 16)]
            eg = (lambda O0, O1: early_g_thunks(O0, O1, W, NV2, a_s, dyn)) if opt.get("earlyg") else None
            O = stage_DF(qa_s, rstd[0:1] * (D ** -0.5 * LOG2E), W, s_s, opt["DF"], (u_s, mu[0:1]), late, eg, pin, shadow)
            out = stage_GH(O, W, NV2, opt["GH"], a_s if opt.get("earlyg") else None, dyn)
            return x + jnp.concatenate(out, axis=1)

        def ffn2(x):
            if opt.get("defer4"):
                mu, rstd = stats(x)
                xn = (x - mu) * rstd
                out = stage_IJ(x, rstd, W, FT, opt["IJ"], (mu, csm_s, csv_s, LB), dyn)
            else:
                xc, rstd = ln_parts(x)
                xn = xc * rstd
                out = stage_IJ(xc, rstd, W, FT, opt["IJ"])
            rs = router(xn)
            upd = xn * 0.0 + jnp.concatenate(out, axis=1) * (rs * rstd)
            return x + (xn + upd)

        wait("x")
        x = jnp.broadcast_to(x_s[0].astype(F32), (8, M))
        x = attn1(x)
        x = ffn1(x)
        if not opt.get("skip2"):
            x = attn2(x)
            if not opt.get("stop"): x = ffn2(x)
        o_ref[0] = x[0:1].astype(BF16)

    def run(A_x, A_c_kv, A_w_q, A_w_uk, A_w_uv, A_w_o, B_x, B_w_r, B_w_gate, B_w_up, B_w_down):
        anyspec = pl.BlockSpec(memory_space=pl.ANY)
        vm = pl.BlockSpec(memory_space=pltpu.VMEM)
        return pl.pallas_call(
            _kernel,
            out_shape=jax.ShapeDtypeStruct((1, 1, M), BF16),
            in_specs=[anyspec] * 10,
            out_specs=vm,
            scratch_shapes=[
                pltpu.VMEM((1, 1, M), BF16), pltpu.VMEM((M,), BF16),
                pltpu.VMEM((M * H, D), BF16), pltpu.VMEM((DC * H, D), BF16), pltpu.VMEM((SK, DC), BF16),
                pltpu.VMEM((DC * H, D), BF16), pltpu.VMEM((H * D, M), BF16),
                pltpu.VMEM((FF, M), BF16), pltpu.VMEM((FF, M), BF16), pltpu.VMEM((FF, M), BF16),
                pltpu.VMEM((160, 128), U32), pltpu.VMEM((H, SK), F32), pltpu.VMEM((H, DC), F32), pltpu.VMEM((H, DC), F32),
                pltpu.VMEM((2, FT, 8, 128), F32), pltpu.VMEM((2, 256, 128), F32), pltpu.VMEM((128, 128), F32),
                pltpu.VMEM((NV1 * 128 + 8, 128), F32), pltpu.VMEM((NV2 * 128, 128), F32),
                pltpu.VMEM((H - NV1, 5, 64, 128), U32), pltpu.VMEM((H - NV1, 4, 64, 128), U32),
                pltpu.VMEM((H - NV2, 4, 64, 128), U32), pltpu.VMEM((H - NV2, 5, 64, 128), U32),
                pltpu.VMEM((NV1 + 1, 5, 128, 128), F32), pltpu.VMEM((NV1, 4, 128, 128), F32),
                pltpu.VMEM((NV2 + 1, 4, 128, 128), F32), pltpu.VMEM((NV2, 5, 128, 128), F32),
                pltpu.VMEM((32, 256, 128), U32), pltpu.VMEM((32, 4, 64, 128), U32),
                pltpu.VMEM((FT, 5, 64, 128), U32), pltpu.VMEM((FT, 5, 64, 128), U32), pltpu.VMEM((FT, 5, 64, 128), U32),
                pltpu.VMEM((5, FV + 8, 128), F32), pltpu.VMEM((5, FV + 8, 128), F32), pltpu.VMEM((5, FV, 128), F32),
                pltpu.SemaphoreType.DMA((14,)),
            ],
            compiler_params=pltpu.CompilerParams(vmem_limit_bytes=110 * 1024 * 1024, flags=flags, disable_semaphore_checks=bool(opt.get('nosemchk'))),
            name=f"fused_v8_{NV1}_{NV2}_{FT}{tag}",
        )(A_x, A_c_kv, A_w_q.reshape(M * H, D), A_w_uk.reshape(DC * H, D), A_w_uv.reshape(DC * H, D),
          A_w_o.reshape(H * D, M), B_w_r, B_w_gate.T, B_w_up.T, B_w_down)
    return run


OPT = {'nosemchk': 1, 'defer3': 1, 'defer4': 1, 'lb': 16, 'tailv': 128, 'tailb': 2, 'c1b': 256, 'order': 2, 'earlyg': 0, 'BC': {'lag': 3, 'nsw': 5, 'dstep': 8, 'doff': 37, 's0': 48, 'split': 1, 'phi': 1.1}, 'DF': {'nh': 16, 'sweep': 1, 'na': 12, 'phid': 0.6, 'pin': 1}, 'GH': {'lag': 3, 'dstep': 16, 'doff': 33, 's0': 64, 'nsw': 8}, 'IJ': {'lag': 4, 'dstep': 8, 'doff': 12, 'vlag': 10, 's0': 24}, 'wdm1': 1, 'nofence': 1}
_run = make_kernel(17, 16, 8, OPT, flags={'XLA_TPU_FORCE_LP_LLO_SCHEDULER': True})


@jax.jit
def pallas_interleave_layers__compressed_kv_cla__moe_arch_mod__decode_kernel(
    A_x, A_c_kv, A_w_q, A_w_uk, A_w_uv, A_w_o, B_x, B_w_r, B_w_gate, B_w_up, B_w_down):
    return _run(A_x, A_c_kv, A_w_q, A_w_uk, A_w_uv, A_w_o, B_x, B_w_r, B_w_gate, B_w_up, B_w_down)
```

```python
import math

import jax
import jax.numpy as jnp
from jax import lax
import jax.experimental.pallas as pl
import jax.experimental.pallas.tpu as pltpu

F32 = jnp.float32
BF16 = jnp.bfloat16
U32 = jnp.uint32

M = 640
H = 32
D = 128
DC = 512
SK = 4096
FF = 1728
EPS = 1e-5
LOG2E = math.log2(math.e)
NT = (((1,), (1,)), ((), ()))

NV1 = 16
NV2 = 16
FT = 8
FM = 128 * FT
FV = FF - FM
LB = 16
WD_MXU = [(0, FV), (FV, FM - 384), (FF - 384, 256)]
WD_VPU = [(FF - 128, 64), (FF - 64, 64)]


def _iota(shape, dim):
    return lax.broadcasted_iota(jnp.int32, shape, dim)


def _dot(a, b):
    return jnp.dot(a, b, preferred_element_type=F32)


def _lo(u):
    return pltpu.bitcast(u << 16, F32)


def _hi(u):
    return pltpu.bitcast(u & jnp.uint32(0xFFFF0000), F32)


def _pack16(v):
    return jnp.concatenate([v, v], axis=0).astype(BF16)


def _as_bf16(u):
    return pltpu.bitcast(u, BF16)


def _xsum(v):
    return jnp.sum(v, axis=1, keepdims=True)


def _interleave(a, b, phi=1.0):
    items = [((i + 0.5) / len(a), 0, th) for i, th in enumerate(a)]
    items += [((i + 0.5) / len(b) * phi, 1, th) for i, th in enumerate(b)]
    items.sort(key=lambda t: (t[0], t[1]))
    for _, _, th in items:
        th()


def _vpu_chain(nv, mult, shared, w_first, w_second, n_second, acc_key, fin, keep, dstep, doff, s0):
    st = {}
    zneed = set(s - doff for s in range(0, nv * 16, dstep) if s >= s0)

    def first(i, db):
        def f():
            s = i * 16 + db
            if db % dstep == 0:
                if shared:
                    base = st.get("m", mult(i))
                else:
                    base = mult(i) if db == 0 else st["m"]
                if ("z", s - doff) in st:
                    z = st.pop(("z", s - doff))
                    st["m"] = [v + z for v in base]
                else:
                    st["m"] = base
            a = None
            for k, x in enumerate(st["m"]):
                p = w_first(i, k, db) * x
                a = p if a is None else a + p
            st[("b", s)] = _xsum(a)
            if keep is not None:
                keep(s, st[("b", s)])
        return f

    def second(i, db):
        def f():
            s = i * 16 + db
            b = st.pop(("b", s))
            for k in range(n_second):
                p = w_second(i, k, db) * b
                key = acc_key(i, k)
                st[key] = p if key not in st else st[key] + p
            if s in zneed:
                st[("z", s)] = st[acc_key(i, n_second - 1)] * 0.0
            if db == 15:
                fin(i, st)
        return f

    steps = []
    for i in range(nv + 1):
        for db in range(16):
            if i < nv:
                steps.append(first(i, db))
            if i >= 1:
                steps.append(second(i - 1, db))
    return steps, st


def _stage_query(x, W, dst, qb_s, dyn):
    WQm, WKm, WQv, WKv = W["WQm"], W["WKm"], W["WQv"], W["WKv"]
    nm = H - NV1
    xv = [x[:, 128 * mt:128 * (mt + 1)] for mt in range(5)]
    XL = [_pack16(v) for v in xv]
    st = {}

    def m_q(j, mt):
        def f():
            o = _dot(XL[mt], _as_bf16(WQm[j, mt]))[0:8]
            st[("q", j)] = o if mt == 0 else st[("q", j)] + o
            if mt == 4:
                st[("qL", j)] = _pack16(st.pop(("q", j)))
        return f

    def m_k(j, ct):
        def f():
            o = _dot(st[("qL", j)], _as_bf16(WKm[j, ct]))
            dst[pl.ds(NV1 + j, 1), pl.ds(128 * ct, 128)] = o[0:1]
        return f
    mxu = [m_q(j, mt) for j in range(nm) for mt in range(5)]
    mxu += [m_k(j, ct) for ct in range(4) for j in range(nm)]

    def fin(i, s):
        for ct in range(2):
            dst[pl.ds(i, 1), pl.ds(128 * ct, 128)] = jnp.sum(s.pop(("c", i, ct)), axis=0, keepdims=True)

    def keep(s, b):
        qb_s[pl.ds(dyn(8 * s), 8), :] = jnp.broadcast_to(b, (8, 128))
    vpu, _ = _vpu_chain(
        NV1, lambda i: xv, True,
        lambda i, k, db: WQv[i, k, pl.ds(8 * db, 8), :],
        lambda i, k, db: WKv[i, k, pl.ds(8 * db, 8), :], 2,
        lambda i, k: ("c", i, k), fin, keep, dstep=8, doff=37, s0=0)
    _interleave(mxu, vpu, phi=1.05)

    sd = {}

    def late(i, db):
        def f():
            qb = qb_s[pl.ds(8 * (16 * i + db), 8), :]
            for ct in (2, 3):
                p = WKv[i, ct, pl.ds(8 * db, 8), :] * qb
                sd[ct] = p if db == 0 else sd[ct] + p
            if db == 15:
                for ct in (2, 3):
                    dst[pl.ds(i, 1), pl.ds(128 * ct, 128)] = jnp.sum(sd[ct], axis=0, keepdims=True)
        return f
    return [late(i, db) for i in range(NV1) for db in range(16)]


def _stage_attention(qa_s, u_s, mu, scale, W, s_s, late, pin):
    ckvT, ckvN = W["ckvT"], W["ckvN"]
    mscale = mu * scale

    def q_left(ct):
        return (qa_s[:, pl.ds(128 * ct, 128)] * scale - u_s[:, pl.ds(128 * ct, 128)] * mscale).astype(BF16)

    def score(q, kt, ct):
        return _dot(q, _as_bf16(ckvT[kt, pl.ds(64 * ct, 64), :]))

    q0, q1 = q_left(0), q_left(1)

    def first_half(kt):
        def f():
            s = score(q0, kt, 0) + score(q1, kt, 1)
            s_s[:, pl.ds(128 * kt, 128)] = s
            pin(s[0:8])
        return f
    _interleave([first_half(kt) for kt in range(32)], late, phi=0.6)
    q2, q3 = q_left(2), q_left(3)
    mx = [None, None]
    for kt in range(32):
        s = s_s[:, pl.ds(128 * kt, 128)]
        s = s + score(q2, kt, 2)
        s = s + score(q3, kt, 3)
        s_s[:, pl.ds(128 * kt, 128)] = s
        seg = kt // 16
        mx[seg] = s if mx[seg] is None else jnp.maximum(mx[seg], s)
    m0 = jnp.max(mx[0], axis=1, keepdims=True)
    m1 = jnp.maximum(m0, jnp.max(mx[1], axis=1, keepdims=True))
    alpha = jnp.exp2(m0 - m1)
    O = [None] * 4
    P = {}
    l = None

    def probs(kt, m):
        nonlocal l
        p = jnp.exp2(s_s[:, pl.ds(128 * kt, 128)] - m)
        l = p if l is None else l + p
        P[kt] = p.astype(BF16)

    def pv(kt, ct):
        o = _dot(P[kt], _as_bf16(ckvN[kt, ct]))
        O[ct] = o if O[ct] is None else O[ct] + o
    for kt in range(16):
        probs(kt, m0)
        for ct in range(4):
            pv(kt, ct)
    l = l * alpha
    for ct in range(4):
        O[ct] = O[ct] * alpha
        for kt in range(16, 32):
            if ct == 0:
                probs(kt, m1)
            pv(kt, ct)
    ls = _xsum(l)
    r0 = pl.reciprocal(ls, approx=True)
    inv = r0 * (2.0 - ls * r0)
    return [o * inv for o in O]


def _stage_output(O, W):
    WVm, WOm, WVv, WOv = W["WVm"], W["WOm"], W["WVv"], W["WOv"]
    nm = H - NV2
    nsw, lag = 8, 3
    st = {}

    def m_v(j, ct):
        def f():
            h = NV2 + j
            left = jnp.broadcast_to(O[ct][h:h + 1], (16, 128)).astype(BF16)
            o = _dot(left, _as_bf16(WVm[j, ct]))[0:8]
            st[("x", j)] = o if ct == 0 else st[("x", j)] + o
            if ct == 3:
                st[("cL", j)] = _pack16(st.pop(("x", j)))
        return f

    def m_o(j, mt):
        def f():
            o = _dot(st[("cL", j)], _as_bf16(WOm[j, mt]))[0:8]
            st[("hm", mt)] = o if j == 0 else st[("hm", mt)] + o
        return f
    mxu = [m_v(j, ct) for ct in range(4) for j in range(nsw)]
    done = 0
    for j in range(nsw, nm):
        mxu += [m_v(j, ct) for ct in range(4)]
        if j - nsw >= lag:
            mxu += [m_o(done, mt) for mt in range(5)]
            done += 1
    mxu += [m_o(j, mt) for j in range(done, nm) for mt in range(5)]
    vpu, sv = _vpu_chain(
        NV2, lambda i: [jnp.broadcast_to(O[ct][i:i + 1], (8, 128)) for ct in range(4)], False,
        lambda i, k, db: WVv[i, k, pl.ds(8 * db, 8), :],
        lambda i, k, db: WOv[i, k, pl.ds(8 * db, 8), :], 5,
        lambda i, k: ("hv", k), lambda i, s: None, None, dstep=16, doff=33, s0=64)
    _interleave(mxu, vpu)
    return [st[("hm", mt)] + jnp.sum(sv[("hv", mt)], axis=0, keepdims=True) for mt in range(5)]


def _swiglu(g, u, half_rstd):
    t = g * half_rstd
    return (t * u) * (1.0 + jnp.tanh(t))


def _stage_ffn(x, mu, rstd, W, csm_s, csv_s):
    WGm, WUm, WDm, WGv, WUv, WDv = (W[k] for k in ("WGm", "WUm", "WDm", "WGv", "WUv", "WDv"))
    xv = [x[:, 128 * mt:128 * (mt + 1)] for mt in range(5)]
    XL = [_pack16(v) for v in xv]
    hs = jnp.broadcast_to(0.5 * rstd, (8, 128))
    mub = jnp.broadcast_to(mu, (8, 128))
    st = {}

    def m_in(ft, which, mt):
        def f():
            o = _dot(XL[mt], _as_bf16((WGm, WUm)[which][ft, mt]))[0:8]
            st[("g", ft, which)] = o if mt == 0 else st[("g", ft, which)] + o
            if which == 1 and mt == 4:
                g, u = st.pop(("g", ft, 0)), st.pop(("g", ft, 1))
                g = g - mub * csm_s[0, ft]
                u = u - mub * csm_s[1, ft]
                st[("hL", ft)] = _pack16(_swiglu(g, u, hs))
        return f

    def m_out(ft, mt):
        def f():
            o = _dot(st[("hL", ft)], _as_bf16(WDm[ft, mt]))[0:8]
            st[("ym", mt)] = o if ft == 0 else st[("ym", mt)] + o
        return f
    mxu = [m_in(ft, w, mt) for ft in range(FT) for w in range(2) for mt in range(5)]
    mxu += [m_out(ft, mt) for ft in range(FT) for mt in range(5)]

    nb = FV // 8
    dstep, doff, vlag, s0 = 8, 12, 10, 32
    zneed = set(s - doff for s in range(0, nb, dstep) if s >= s0)

    def v_in(fb, which):
        def f():
            if which == 0 and fb == LB:
                st["xv"] = [v - mub for v in st.get("xv", xv)]
            if which == 0 and fb % dstep == 0:
                if ("z", fb - doff) in st:
                    z = st.pop(("z", fb - doff))
                    st["xv"] = [v + z for v in st.get("xv", xv)]
                else:
                    st["xv"] = st.get("xv", xv)
            a = None
            for mt in range(5):
                p = (WGv, WUv)[which][mt, pl.ds(8 * fb, 8), :] * st["xv"][mt]
                a = p if a is None else a + p
            st[("gb", fb, which)] = jnp.broadcast_to(_xsum(a), (8, 128))
        return f

    def v_out(fb):
        def f():
            g, u = st.pop(("gb", fb, 0)), st.pop(("gb", fb, 1))
            if fb < LB:
                g = g - mub * csv_s[0, pl.ds(8 * fb, 8), :]
                u = u - mub * csv_s[1, pl.ds(8 * fb, 8), :]
            hh = _swiglu(g, u, hs)
            for mt in range(5):
                p = WDv[mt, pl.ds(8 * fb, 8), :] * hh
                st[("yv", mt)] = p if fb == 0 else st[("yv", mt)] + p
            if fb in zneed:
                st[("z", fb)] = st[("yv", 4)] * 0.0
        return f
    vpu = []
    for fb in range(nb + vlag):
        if fb < nb:
            vpu += [v_in(fb, 0), v_in(fb, 1)]
        if fb >= vlag:
            vpu.append(v_out(fb - vlag))
    _interleave(mxu, vpu, phi=0.9)
    return [st[("ym", mt)] + jnp.sum(st[("yv", mt)], axis=0, keepdims=True) for mt in range(5)]


def _kernel(x_hbm, ckv_hbm, wq_hbm, wuk_hbm, wuv_hbm, wo_hbm, wr_hbm, wg_hbm, wu_hbm, wd_hbm,
            o_ref,
            x_s, wr_s, wq_s, wuk_s, ckv_s, wuv_s, wo_s, wg_s, wu_s, wd_s,
            v_s, s_s, qa_s, u_s, csm_s, csv_s, hb_s, qb_s,
            WQm, WKm, WVm, WOm, WQv, WKv, WVv, WOv, ckvT, ckvN, WGm, WUm, WDm, WGv, WUv, WDv,
            sems):
    W = dict(WQm=WQm, WKm=WKm, WVm=WVm, WOm=WOm, WQv=WQv, WKv=WKv, WVv=WVv, WOv=WOv, ckvT=ckvT, ckvN=ckvN,
             WGm=WGm, WUm=WUm, WDm=WDm, WGv=WGv, WUv=WUv, WDv=WDv)

    queue = [("wq", wq_hbm, wq_s), ("x", x_hbm, x_s), ("wuk", wuk_hbm, wuk_s), ("ckv", ckv_hbm.at[0], ckv_s),
             ("wuv", wuv_hbm, wuv_s), ("wo", wo_hbm, wo_s), ("wr", wr_hbm, wr_s), ("wg", wg_hbm, wg_s),
             ("wu", wu_hbm, wu_s)]
    for i, (r0, n) in enumerate(WD_MXU + WD_VPU):
        queue.append((f"wd{i}", wd_hbm.at[pl.ds(r0, n)], wd_s.at[pl.ds(r0, n)]))
    copies = {name: pltpu.make_async_copy(src, dst, sems.at[i]) for i, (name, src, dst) in enumerate(queue)}
    for c in copies.values():
        c.start()

    def wait(name):
        copies[name].wait()

    zero = [0]

    def dyn(base):
        return pl.multiple_of(zero[0] * 8 + base, 8)

    def ln_parts(x):
        mean = _xsum(x) * (1.0 / M)
        xc = x - mean
        var = _xsum(xc * xc) * (1.0 / M)
        return xc, lax.rsqrt(var + EPS)

    def ln_stats(x):
        mu = _xsum(x) * (1.0 / M)
        var = jnp.maximum(_xsum(x * x) * (1.0 / M) - mu * mu, 0.0)
        return mu, lax.rsqrt(var + EPS)

    def router(xn):
        wr = wr_s[...].astype(F32).reshape(1, M)
        return jax.nn.sigmoid(_xsum(xn * wr))

    E4 = jnp.where(_iota((128, 128), 0) % 4 == _iota((128, 128), 1) // 32, 1.0, 0.0).astype(BF16)
    A_mask = _iota((32, 128), 1) // 4 == _iota((32, 128), 0)
    hr, hl = _iota((16, 128), 0), _iota((16, 128), 1) % 32
    M32 = jnp.where(hl == 2 * hr, jnp.uint32(0x0000FFFF),
                    jnp.where(hl == 2 * hr + 1, jnp.uint32(0xFFFF0000), jnp.uint32(0)))

    def dup_bf16(v):
        u = pltpu.bitcast(v.astype(BF16).astype(F32), U32)
        return u | (u >> 16)

    def per_head_matmul(ntiles, get_tile):
        acc = None
        for t0 in range(0, ntiles, 8):
            lhs, rhs = [], []
            for t in range(t0, t0 + 8):
                vrow = jnp.broadcast_to(v_s[pl.ds(t, 1), :], (16, 128))
                lhs.append(pltpu.bitcast(vrow & M32, BF16))
                rhs.append(get_tile(t))
            o = _dot(jnp.concatenate(lhs, axis=1), jnp.concatenate(rhs, axis=0))
            acc = o if acc is None else acc + o
        return acc

    def relayout_heads(w_s, ntiles, Wv, Wm, mxu_transposed, nv):
        wu = w_s.bitcast(U32)

        def body(t, c):
            blk = wu.at[pl.ds(pl.multiple_of(t * 2048, 2048), 2048)]
            for hp in range(16):
                g = jnp.concatenate([blk[pl.ds(128 * r + hp, 8, stride=16), :] for r in range(16)], axis=0)
                gt = g.T if (2 * hp < nv or mxu_transposed) else None
                for half, f in ((0, _lo), (1, _hi)):
                    h = 2 * hp + half
                    if h < nv:
                        Wv[h, t] = f(gt)
                    else:
                        Wm[h - nv, t] = pltpu.bitcast(f(gt if mxu_transposed else g).astype(BF16), U32)
            return c + (t >> 10)
        return lax.fori_loop(0, ntiles, body, 0)

    def attention_1(x):
        xc, rstd = ln_parts(x)
        xn = xc * rstd
        for kt in range(5):
            xr = jnp.broadcast_to(xn[0:1, 128 * kt:128 * (kt + 1)], (32, 128))
            V = _dot(jnp.where(A_mask, xr, 0.0).astype(BF16), E4)
            v_s[pl.ds(32 * kt, 32), :] = dup_bf16(V)
        wait("wq")
        qb = per_head_matmul(160, lambda t: wq_s[pl.ds(128 * t, 128), :]).astype(BF16)
        zero[0] = relayout_heads(wq_s, 5, WQv, WQm, False, NV1)
        wait("wuk")
        hsel = (_iota((8, 128), 1) % 32) // 8
        rsel = _iota((8, 128), 1) % 8
        srow = _iota((8, 128), 0)
        vblocks = []
        for b0 in range(0, 128, 8):
            rhs = [wuk_s[pl.ds(32 * (128 * cl + b), 32), :] for b in range(b0, b0 + 8) for cl in range(4)]
            o = lax.dot_general(qb, jnp.concatenate(rhs, axis=0), NT, preferred_element_type=F32)
            vb = None
            for i in range(8):
                ob = o[:, 128 * i:128 * (i + 1)]
                u = jnp.where(hsel == 0, ob[0:8],
                              jnp.where(hsel == 1, ob[8:16], jnp.where(hsel == 2, ob[16:24], ob[24:32])))
                u = jnp.where(srow == rsel, u, 0.0)
                r_ = jnp.broadcast_to(jnp.sum(u, axis=0, keepdims=True), (8, 128))
                vb = r_ if vb is None else jnp.where(srow == i, r_, vb)
            vblocks.append(vb)
        qt = jnp.concatenate(vblocks, axis=0).T
        qab = jnp.concatenate([qt[32 * cl:32 * (cl + 1)] for cl in range(4)], axis=1).astype(BF16)
        relayout_heads(wuk_s, 4, WKv, WKm, True, NV1)
        for th in _stage_query(jnp.ones((8, M), F32), W, u_s, qb_s, dyn):
            th()
        wait("ckv")
        kc = 512
        mx = None
        for c in range(SK // kc):
            s = lax.dot_general(qab, ckv_s[pl.ds(c * kc, kc), :], NT, preferred_element_type=F32) * (D ** -0.5)
            s_s[:, pl.ds(c * kc, kc)] = s
            for j in range(kc // 128):
                sj = s[:, 128 * j:128 * (j + 1)]
                mx = sj if mx is None else jnp.maximum(mx, sj)
        mx = jnp.max(mx, axis=1, keepdims=True)
        l = o = None
        for c in range(SK // kc):
            p = jnp.exp(s_s[:, pl.ds(c * kc, kc)] - mx)
            for j in range(kc // 128):
                pj = p[:, 128 * j:128 * (j + 1)]
                l = pj if l is None else l + pj
            oc = _dot(p.astype(BF16), ckv_s[pl.ds(c * kc, kc), :])
            o = oc if o is None else o + oc
        o = o * (1.0 / _xsum(l))

        def ckv_body(i, c):
            for j in range(2):
                kt = 2 * i + j
                for ct in range(4):
                    t = ckv_s[pl.ds(pl.multiple_of(128 * kt, 128), 128), pl.ds(128 * ct, 128)]
                    ckvT[kt, pl.ds(64 * ct, 64), :] = pltpu.bitcast(t.T, U32)
                    ckvN[kt, ct] = pltpu.bitcast(t, U32)
            return c
        lax.fori_loop(0, 16, ckv_body, 0)
        obig = jnp.concatenate([o[:, 128 * cl:128 * (cl + 1)] for cl in range(4)], axis=0)
        v_s[pl.ds(0, 128), :] = dup_bf16(obig.T)
        wait("wuv")
        ctxb = per_head_matmul(128, lambda b: jnp.concatenate(
            [wuv_s[pl.ds(32 * (128 * cl + b), 32), :] for cl in range(4)], axis=0)).astype(BF16)
        relayout_heads(wuv_s, 4, WVv, WVm, False, NV2)
        wait("wo")
        r16 = _iota((16, 128), 0)
        acc = None
        for g in range(2):
            cg = ctxb[16 * g:16 * (g + 1)]
            for h0 in range(0, 16, 4):
                lhs = [jnp.where(r16 == h, cg, jnp.zeros_like(cg)) for h in range(h0, h0 + 4)]
                oo = _dot(jnp.concatenate(lhs, axis=1), wo_s[pl.ds(128 * (16 * g + h0), 512), :])
                acc = oo if acc is None else acc + oo
        xo = x + jnp.sum(acc, axis=0, keepdims=True)

        def wo_v(h, c):
            for mt in range(5):
                WOv[h, mt] = wo_s[pl.ds(pl.multiple_of(128 * h, 128), 128), pl.ds(128 * mt, 128)].astype(F32)
            return c
        lax.fori_loop(0, NV2, wo_v, 0)

        def wo_m(j, c):
            for mt in range(5):
                t = wo_s[pl.ds(pl.multiple_of(128 * (j + NV2), 128), 128), pl.ds(128 * mt, 128)]
                WOm[j, mt] = pltpu.bitcast(t, U32)
            return c
        lax.fori_loop(0, H - NV2, wo_m, 0)
        return xo

    def ffn_1(x):
        xc, rstd = ln_parts(x)
        xn = xc * rstd
        wait("wr")
        rs = router(xn)
        xb = jnp.concatenate([xn, jnp.ones((8, M), F32)], axis=0).astype(BF16)

        def gate_up(w_s, which, Wm, Wv):
            r = [lax.dot_general(xb, w_s[pl.ds(a, n), :], NT, preferred_element_type=F32)
                 for a, n in ((0, FV), (FV, FM))]
            for ft in range(FT):
                csm_s[which, ft] = r[1][8:16, 128 * ft:128 * (ft + 1)]
            for j in range((8 * LB + 127) // 128):
                cs = jnp.broadcast_to(r[0][8:9, 128 * j:128 * (j + 1)], (128, 128))
                csv_s[which, pl.ds(128 * j, 128), :] = cs.T
            return [v[0:8] for v in r]

        def relayout(w_s, Wm, Wv):
            nb = FV // 32
            for ft in range(FT):
                for mt in range(5):
                    t = w_s[pl.ds(FV + 128 * ft, 128), pl.ds(128 * mt, 128)]
                    Wm[ft, mt] = pltpu.bitcast(t.T, U32)
                for b in range(ft * nb // FT, (ft + 1) * nb // FT):
                    for mt in range(5):
                        Wv[mt, pl.ds(32 * b, 32), :] = w_s[pl.ds(32 * b, 32), pl.ds(128 * mt, 128)].astype(F32)
        wait("wg")
        g = gate_up(wg_s, 0, WGm, WGv)
        relayout(wg_s, WGm, WGv)
        wait("wu")
        u = gate_up(wu_s, 1, WUm, WUv)
        hb = []
        for gg, uu in zip(g, u):
            hh = gg * jax.nn.sigmoid(gg) * uu
            hb.append(jnp.broadcast_to(hh[0:1], (16, hh.shape[1])).astype(BF16))
        hb_s[...] = jnp.broadcast_to(hh[0:1, FM - 128:FM], (128, 128)).T
        relayout(wu_s, WUm, WUv)

        y = None
        for i, (a, n) in enumerate(WD_MXU):
            wait(f"wd{i}")
            if i == 0:
                y = _dot(hb[0], wd_s[pl.ds(0, FV), :])[0:8]
                for r0 in range(0, FV, 32):
                    for mt in range(5):
                        WDv[mt, pl.ds(r0, 32), :] = wd_s[pl.ds(r0, 32), pl.ds(128 * mt, 128)].astype(F32)
                continue
            acc = None
            for ft in range((a - FV) // 128, (a - FV + n) // 128):
                raw = [wd_s[pl.ds(FV + 128 * ft, 128), pl.ds(128 * mt, 128)] for mt in range(5)]
                for mt in range(5):
                    WDm[ft, mt] = pltpu.bitcast(raw[mt], U32)
                o = [_dot(hb[1][:, 128 * ft:128 * (ft + 1)], raw[mt])[0:8] for mt in range(5)]
                acc = o if acc is None else [p + q for p, q in zip(acc, o)]
            y = y + jnp.concatenate(acc, axis=1)
        yv = None
        for i, (a, n) in enumerate(WD_VPU):
            wait(f"wd{len(WD_MXU) + i}")
            for r0 in range(a, a + n, 16):
                hc = hb_s[pl.ds(r0 - (FF - 128), 16), :]
                raw = [wd_s[pl.ds(r0, 16), pl.ds(128 * mt, 128)] for mt in range(5)]
                part = [t.astype(F32) * hc for t in raw]
                yv = part if yv is None else [p + q for p, q in zip(yv, part)]
                for mt in range(5):
                    WDm[FT - 1, mt, pl.ds((r0 - (FF - 128)) // 2, 8), :] = pltpu.bitcast(raw[mt], U32)
        y = y + jnp.concatenate([jnp.sum(p, axis=0, keepdims=True) for p in yv], axis=1)
        return x + (xn + (xn * 0.0 + y * rs))

    def attention_2(x):
        mu, rstd = ln_stats(x)
        late = _stage_query(x, W, qa_s, qb_s, dyn)

        def pin(v):
            qb_s[pl.ds(dyn(NV1 * 128), 8), :] = v
        O = _stage_attention(qa_s, u_s, mu[0:1], rstd[0:1] * (D ** -0.5 * LOG2E), W, s_s, late, pin)
        return x + jnp.concatenate(_stage_output(O, W), axis=1)

    def ffn_2(x):
        mu, rstd = ln_stats(x)
        xn = (x - mu) * rstd
        y = jnp.concatenate(_stage_ffn(x, mu, rstd, W, csm_s, csv_s), axis=1)
        rs = router(xn)
        return x + (xn + (xn * 0.0 + y * (rs * rstd)))

    wait("x")
    x = jnp.broadcast_to(x_s[0].astype(F32), (8, M))
    x = attention_1(x)
    x = ffn_1(x)
    x = attention_2(x)
    x = ffn_2(x)
    o_ref[0] = x[0:1].astype(BF16)


def _run(A_x, A_c_kv, A_w_q, A_w_uk, A_w_uv, A_w_o, B_x, B_w_r, B_w_gate, B_w_up, B_w_down, name="fused_layers"):
    del B_x
    hbm = pl.BlockSpec(memory_space=pl.ANY)
    ncopies = 9 + len(WD_MXU) + len(WD_VPU)
    scratch = [
        pltpu.VMEM((1, 1, M), BF16), pltpu.VMEM((M,), BF16),
        pltpu.VMEM((M * H, D), BF16), pltpu.VMEM((DC * H, D), BF16), pltpu.VMEM((SK, DC), BF16),
        pltpu.VMEM((DC * H, D), BF16), pltpu.VMEM((H * D, M), BF16),
        pltpu.VMEM((FF, M), BF16), pltpu.VMEM((FF, M), BF16), pltpu.VMEM((FF, M), BF16),
        pltpu.VMEM((160, 128), U32), pltpu.VMEM((H, SK), F32), pltpu.VMEM((H, DC), F32), pltpu.VMEM((H, DC), F32),
        pltpu.VMEM((2, FT, 8, 128), F32), pltpu.VMEM((2, 256, 128), F32), pltpu.VMEM((128, 128), F32),
        pltpu.VMEM((NV1 * 128 + 8, 128), F32),
        pltpu.VMEM((H - NV1, 5, 64, 128), U32), pltpu.VMEM((H - NV1, 4, 64, 128), U32),
        pltpu.VMEM((H - NV2, 4, 64, 128), U32), pltpu.VMEM((H - NV2, 5, 64, 128), U32),
        pltpu.VMEM((NV1, 5, 128, 128), F32), pltpu.VMEM((NV1, 4, 128, 128), F32),
        pltpu.VMEM((NV2, 4, 128, 128), F32), pltpu.VMEM((NV2, 5, 128, 128), F32),
        pltpu.VMEM((32, 256, 128), U32), pltpu.VMEM((32, 4, 64, 128), U32),
        pltpu.VMEM((FT, 5, 64, 128), U32), pltpu.VMEM((FT, 5, 64, 128), U32), pltpu.VMEM((FT, 5, 64, 128), U32),
        pltpu.VMEM((5, FV, 128), F32), pltpu.VMEM((5, FV, 128), F32), pltpu.VMEM((5, FV, 128), F32),
        pltpu.SemaphoreType.DMA((ncopies,)),
    ]
    return pl.pallas_call(
        _kernel,
        out_shape=jax.ShapeDtypeStruct((1, 1, M), BF16),
        in_specs=[hbm] * 10,
        out_specs=pl.BlockSpec(memory_space=pltpu.VMEM),
        scratch_shapes=scratch,
        compiler_params=pltpu.CompilerParams(
            vmem_limit_bytes=110 * 1024 * 1024,
            disable_semaphore_checks=True,
            flags={"XLA_TPU_FORCE_LP_LLO_SCHEDULER": True}),
        name=name,
    )(A_x, A_c_kv,
      A_w_q.reshape(M * H, D), A_w_uk.reshape(DC * H, D), A_w_uv.reshape(DC * H, D), A_w_o.reshape(H * D, M),
      B_w_r, B_w_gate.T, B_w_up.T, B_w_down)


@jax.jit
def pallas_interleave_layers__compressed_kv_cla__moe_arch_mod__decode_kernel(
        A_x, A_c_kv, A_w_q, A_w_uk, A_w_uv, A_w_o, B_x, B_w_r, B_w_gate, B_w_up, B_w_down):
    return _run(A_x, A_c_kv, A_w_q, A_w_uk, A_w_uv, A_w_o, B_x, B_w_r, B_w_gate, B_w_up, B_w_down)
```
